```python
import jax
import jax.numpy as jnp

def _softmax(x, axis=-1):
    return jax.nn.softmax(x, axis=axis)
def _gelu(x):
    return jax.nn.gelu(x, approximate=True)
def _silu(x):
    return jax.nn.silu(x)
def _sigmoid(x):
    return jax.nn.sigmoid(x)
def _layernorm(x, axis=-1, eps=1e-5):
    m = jnp.mean(x, axis=axis, keepdims=True)
    v = jnp.var(x, axis=axis, keepdims=True)
    return (x - m) / jnp.sqrt(v + eps)
def _scatter_add(tgt, idx, src, axis=0):
    return tgt.at[idx].add(src)
def _segment_sum(src, seg, n):
    return jax.ops.segment_sum(src, seg, n)
class _Rng:
    def __init__(self, key):
        self._k = key
    def _next(self):
        self._k, sub = jax.random.split(self._k)
        return sub
    def normal(self, shape):
        return jax.random.normal(self._next(), shape, dtype=jnp.bfloat16)
    def randint(self, lo, hi, shape):
        return jax.random.randint(self._next(), shape, lo, hi, dtype=jnp.int32)
    def uniform(self, shape, lo=0.0, hi=1.0):
        return jax.random.uniform(self._next(), shape, jnp.bfloat16, lo, hi)
    def permutation(self, n):
        return jax.random.permutation(self._next(), n)


kernel_name = 'gated_mix__sliding_local_dilated__ssm_conv_s4__prompt'

def setup_inputs():
    _rng = _Rng(jax.random.key(int.from_bytes(__import__("os").urandom(4), "little")))
    _w = (lambda a: (lambda t: t.astype(jnp.bfloat16) if jnp.issubdtype(t.dtype, jnp.floating) else t)(jnp.asarray(a)))
    def _A_setup():
        B, S, D = 1, 2048, 640
        return {
            "x": _w((lambda *s: _rng.normal(s) * 0.05)(B, S, D)),
            "wqkv": _w((lambda *s: _rng.normal(s) * 0.05)(D, 3 * D)),
            "wo": _w((lambda *s: _rng.normal(s) * 0.05)(D, D)),
        }
    _A_in = _A_setup()

    def _B_setup():
        B, L, D, N = 1, 2048, 640, 192
        A_re = -jnp.exp((lambda *s: _rng.normal(s) * 0.05)(D, N))
        A_im = jnp.pi * (lambda *s: _rng.normal(s) * 0.05)(D, N)
        B_re = (lambda *s: _rng.normal(s) * 0.05)(D, N)
        B_im = (lambda *s: _rng.normal(s) * 0.05)(D, N)
        C_re = (lambda *s: _rng.normal(s) * 0.05)(D, N)
        C_im = (lambda *s: _rng.normal(s) * 0.05)(D, N)
        log_dt = (lambda *s: _rng.normal(s) * 0.05)(D) * 0.5 - 4.0
        Dskip = (lambda *s: _rng.normal(s) * 0.05)(D)
        return {
            "u": _w((lambda *s: _rng.normal(s) * 0.05)(B, L, D)),
            "A_re": _w(A_re),
            "A_im": _w(A_im),
            "B_re": _w(B_re),
            "B_im": _w(B_im),
            "C_re": _w(C_re),
            "C_im": _w(C_im),
            "log_dt": _w(log_dt),
            "Dskip": _w(Dskip),
        }
    _B_in = _B_setup()

    return {
        "A_x": _A_in["x"],
        "A_wqkv": _A_in["wqkv"],
        "A_wo": _A_in["wo"],
        "B_u": _B_in["u"],
        "B_A_re": _B_in["A_re"],
        "B_A_im": _B_in["A_im"],
        "B_B_re": _B_in["B_re"],
        "B_B_im": _B_in["B_im"],
        "B_C_re": _B_in["C_re"],
        "B_C_im": _B_in["C_im"],
        "B_log_dt": _B_in["log_dt"],
        "B_Dskip": _B_in["Dskip"],
        "gate_w": _w((lambda *s: _rng.normal(s) * 0.05)(640)),
    }

def reference(A_x, A_wqkv, A_wo, B_u, B_A_re, B_A_im, B_B_re, B_B_im, B_C_re, B_C_im, B_log_dt, B_Dskip, gate_w):
    def _A_ref(x, wqkv, wo):
        B, S, D = x.shape
        H = 32; Dh = D // H
        W, dil = 8, 2
        qkv = (lambda x, *d: x.transpose(*d))((x @ wqkv).reshape(B, S, 3, H, Dh), 2, 0, 3, 1, 4)
        q, k, v = qkv[0], qkv[1], qkv[2]
        scale = Dh ** -0.5
        pos = jnp.arange(S)
        off = jnp.arange(W) * dil
        idx = pos[:, None] - off[None, :]
        mask = idx >= 0
        idx_c = jnp.where(mask, idx, 0).reshape(-1)
        kg = k[:, :, idx_c, :].reshape(B, H, S, W, Dh)
        vg = v[:, :, idx_c, :].reshape(B, H, S, W, Dh)
        logits = jnp.einsum("bhsd,bhswd->bhsw", q, kg) * scale
        logits = jnp.where(mask[None, None, :, :], logits, -1e9)
        attn = _softmax(logits, axis=-1)
        o = jnp.einsum("bhsw,bhswd->bhsd", attn, vg)
        return (lambda x, *d: x.transpose(*d))(o, 0, 2, 1, 3).reshape(B, S, D) @ wo

    def _B_ref(u, A_re, A_im, B_re, B_im, C_re, C_im, log_dt, Dskip):
        Bsz, L, D = u.shape
        dt = jnp.exp(log_dt)[:, None]
        A = A_re + 1j * A_im
        Bc = B_re + 1j * B_im
        Cc = C_re + 1j * C_im
        logdA = dt * A
        dB = dt * Bc
        l = (lambda x, dt: x.astype(dt))(jnp.arange(L), A_re.dtype)
        P = jnp.exp(logdA[:, :, None] * l[None, None, :])
        K = jnp.einsum("dn,dnl,dn->dl", Cc, P, dB).real
        L2 = 2 * L
        Kp = jnp.pad(K, ((0, 0), (0, L)))
        up = (lambda x, *d: x.transpose(*d))(u, 0, 2, 1)
        up = jnp.pad(up, ((0, 0), (0, 0), (0, L)))
        Kf = (lambda x, axes=(-2,-1): jnp.fft.rfft2(x.astype(jnp.float32), axes=axes))(Kp[:, None, :], axes=(-2, -1))
        Uf = (lambda x, axes=(-2,-1): jnp.fft.rfft2(x.astype(jnp.float32), axes=axes))(up[:, :, None, :], axes=(-2, -1))
        Yf = Uf * Kf[None, :, :, :]
        y = (lambda x, s, axes=(-2,-1): jnp.fft.irfft2(x, s=s, axes=axes).astype(jnp.bfloat16))(Yf, (1, L2), axes=(-2, -1))[:, :, 0, :L]
        y = (lambda x, *d: x.transpose(*d))(y, 0, 2, 1) + u * Dskip[None, None, :]
        return y

    x = A_x
    g = _sigmoid((x * gate_w).sum(-1, keepdims=True))
    a = _A_ref(x, A_wqkv, A_wo)
    b = _B_ref(x, B_A_re, B_A_im, B_B_re, B_B_im, B_C_re, B_C_im, B_log_dt, B_Dskip)
    return g * a + (1 - g) * b
```

```python
import jax
import jax.numpy as jnp
import numpy as np
import jax.experimental.pallas as pl
import jax.experimental.pallas.tpu as pltpu

S, D, H, DH, N = 2048, 640, 32, 20, 192
WIN, DIL = 8, 2
T = 128
NT = D // T
NB = S // T
HALO = 16
NU, NV = 10, 16
F32, BF16, U32 = jnp.float32, jnp.bfloat16, jnp.uint32

_BASES = [0, 1, 2, 3, 4, 5, 6, 7, 256, 258, 260, 262, 512, 516, 768, 772,
          1024, 1280, 1536, 1792]


def _constants():
    om = 2.0 * np.pi * (np.arange(T) + 0.25) / T
    ph = np.exp(-1j * om[:, None] * np.arange(T)[None, :])
    fx = np.concatenate([ph.real, ph.imag], 0)
    g = np.stack([ph.real.T, ph.imag.T], -1).reshape(T, 2 * T) / T
    lag = np.arange(S).astype(np.float32).astype(BF16).astype(np.float32).astype(np.int64)
    lane = np.arange(T)
    off = 8 * (2 * (lane // 8) + lane % 2)
    tiles = [np.array(_BASES[4 * t:4 * t + 4])[(lane % 8) // 2] + off for t in range(5)]
    lo = lane < T // 2
    vals = {0: np.where(lo, tiles[0], np.roll(tiles[1], T // 2)),
            1: np.where(lo, np.roll(tiles[0], T // 2), tiles[1])}
    for m in range(2, NB):
        vals[m] = tiles[2 if m < 4 else 3 if m < 8 else 4].copy()
    vals[3][0], vals[7][0], vals[15][0] = 512, 1024, S
    fk = np.zeros((NB, 2 * T, T))
    for m in range(NB):
        blk = lag[m * T:(m + 1) * T]
        e = (blk[:, None] == vals[m][None, :]).astype(np.float64)
        assert (e.sum(1) == 1).all()
        c = ph @ e
        fk[m] = np.concatenate([c.real, c.imag], 0)
    cast = lambda a: a.astype(np.float32).astype(BF16)
    return cast(fx), cast(g), cast(fk)


def _cmul(a, b):
    return a[0] * b[0] - a[1] * b[1], a[0] * b[1] + a[1] * b[0]


def _csq(a):
    t = a[0] * a[1]
    return a[0] * a[0] - a[1] * a[1], t + t


def _pack(a, b):
    return pltpu.pack_elementwise([a, b], packed_dtype=BF16)


def _dot(a, b):
    return jnp.dot(a, b, preferred_element_type=F32)


def _dot_nt(a, b):
    return jax.lax.dot_general(a, b, (((1,), (1,)), ((), ())), preferred_element_type=F32)


def _kernel(x_ref, wqkv_ref, wo_ref, are_ref, aim_ref, bre_ref, bim_ref, cre_ref, cim_ref,
            ldt_ref, dsk_ref, gw_ref, fx_ref, g_ref, fk_ref, o_ref,
            wt_s, wp_s, wop_s, par_s, us_s, vs_s, kend_s, ko_s, kt_s, kh_s, xh_s, yh_s, y_s,
            q_s, k_s, v_s):
    lane = jax.lax.broadcasted_iota(jnp.int32, (8, T), 1)
    lo = lane < T // 2

    def w_transpose(c, _):
        c0 = pl.multiple_of(c * T, T)
        for kt in range(NT):
            wt_s[kt, pl.ds(c0, T), :] = wqkv_ref[kt * T:(kt + 1) * T, pl.ds(c0, T)].astype(F32).T
        return _
    jax.lax.fori_loop(0, 3 * NT, w_transpose, None)
    for s in range(3):
        for t in range(NT):
            for kt in range(NT):
                rows = [wt_s[kt, pl.ds(s * D + 4 * t + i, H, stride=DH), :] for i in range(4)]
                wp_s[t, s * T:(s + 1) * T, kt * T:(kt + 1) * T] = jnp.concatenate(rows, 0).astype(BF16)
    for ct in range(NT):
        wt_s[ct, 0:D, :] = wo_ref[:, ct * T:(ct + 1) * T].astype(F32)
        for t in range(NT):
            rows = [wt_s[ct, pl.ds(4 * t + i, H, stride=DH), :] for i in range(4)]
            wop_s[t * T:(t + 1) * T, ct * T:(ct + 1) * T] = jnp.concatenate(rows, 0).astype(BF16)

    for t in range(NT):
        k_s[t, 0:HALO, :] = jnp.zeros((HALO, T), F32)
        v_s[t, 0:HALO, :] = jnp.zeros((HALO, T), F32)

    def prep(j):
        r0 = pl.multiple_of(j * T, T)
        dt = jnp.exp(ldt_ref[:, pl.ds(r0, T)].astype(F32)).astype(BF16).astype(F32)
        dt = jnp.broadcast_to(dt, (T, T)).T
        lo_h = jax.lax.broadcasted_iota(jnp.int32, (T // 2, T), 1) < T // 2
        dt = jnp.concatenate([dt, jnp.where(lo_h, dt[:T // 2], dt[T // 2:])], 0)

        def load(ref):
            hi = ref[pl.ds(r0, T), T:N].astype(F32)
            hi = jnp.concatenate([hi[:T // 2], hi[T // 2:]], 1)
            return jnp.concatenate([ref[pl.ds(r0, T), 0:T].astype(F32), hi], 0)
        mag = jnp.exp(dt * load(are_ref))
        ang = dt * load(aim_ref)
        par_s[0] = mag * jnp.cos(ang)
        par_s[1] = mag * jnp.sin(ang)
        w = _cmul((load(cre_ref), load(cim_ref)), (dt * load(bre_ref), dt * load(bim_ref)))
        par_s[2] = w[0]
        par_s[3] = w[1]

    def powers(r0):
        p = (par_s[0, pl.ds(r0, 8), :], par_s[1, pl.ds(r0, 8), :])
        w = (par_s[2, pl.ds(r0, 8), :], -par_s[3, pl.ds(r0, 8), :])
        p2 = _csq(p)
        p4 = _csq(p2)
        q = _csq(p4)
        v = [(jnp.ones_like(q[0]), jnp.zeros_like(q[0])), q]
        step = q
        while len(v) < 2 * NV:
            step = _csq(step)
            v = v + [step] + [_cmul(a, step) for a in v[1:]]
        conj = lambda a: (a[0], -a[1])
        b1 = conj(_csq(step))
        b2 = _csq(b1)
        b4 = _csq(b2)
        u = [w, _cmul(w, conj(p))]
        u += [_cmul(a, conj(p2)) for a in u]
        u += [_cmul(a, conj(p4)) for a in u]
        u += [_cmul(a, b1) for a in u[0:8:2]]
        u += [_cmul(a, b2) for a in (u[0], u[4], u[8], u[10])]
        u += [_cmul(a, b4) for a in (u[0], u[8], u[12], u[14])]
        last = u[16][0] * b4[0] - u[16][1] * b4[1]
        pk = lambda xs: [(_pack(a[0], b[0]), _pack(a[1], b[1])) for a, b in zip(xs[0::2], xs[1::2])]
        return pk(u), pk(v), last

    def gen_lo(r, _):
        r0 = pl.multiple_of(r * 8, 8)
        u, v, last = powers(r0)
        for dst, xs in ((us_s, u), (vs_s, v)):
            for i, a in enumerate(xs):
                dst[0, pl.ds(i * T + r0, 8), :] = a[0]
                dst[1, pl.ds(i * T + r0, 8), :] = a[1]
        kend_s[0, pl.ds(r0, 8), :] = last
        return _

    def gen_hi(r, _):
        r0 = pl.multiple_of(r * 8, 8)
        u, v, last = powers(T + r0)
        for dst, xs in ((us_s, u), (vs_s, v)):
            for i, a in enumerate(xs):
                t = pltpu.roll(jnp.where(lo, a[1], a[0]), T // 2, 1)
                dst[2, pl.ds(i * T + r0, 8), :] = jnp.where(lo, a[0], t)
                dst[2, pl.ds(i * T + T // 2 + r0, 8), :] = jnp.where(lo, t, a[1])
        kend_s[1, pl.ds(r0, 8), :] = jnp.where(lo, last, 0.0)
        kend_s[1, pl.ds(T // 2 + r0, 8), :] = jnp.where(lo, 0.0, last)
        return _

    def kmat(g, _):
        u = jnp.concatenate([pltpu.bitcast(us_s[t, pl.ds(g, 4 * NU, stride=32), :], BF16)
                             for t in range(3)], 1)
        v = jnp.concatenate([pltpu.bitcast(vs_s[t, pl.ds(g, 4 * NV, stride=32), :], BF16)
                             for t in range(3)], 1)
        ko_s[pl.ds(pl.multiple_of(g * 8 * NU, 8), 8 * NU), :] = _dot_nt(u, v)
        return _

    def shuffle():
        lane32 = jax.lax.broadcasted_iota(jnp.int32, (32, T), 1)
        slot = (lane32 % 8) // 2
        tiles = []
        for t in range(5):
            parts = []
            for c in range(4):
                acc = None
                for jj in range(4):
                    k = 4 * t + jj
                    a = ko_s[pl.ds((k // 2) * 8 + 2 * c + k % 2, 32, stride=8 * NU), :]
                    if jj != c:
                        a = pltpu.roll(a, (2 * (jj - c)) % T, 1)
                    acc = a if acc is None else jnp.where(slot == jj, a, acc)
                parts.append(acc)
            tiles.append(jnp.concatenate(parts, 0))
        lane_t = jax.lax.broadcasted_iota(jnp.int32, (T, T), 1)
        lo_t, first = lane_t < T // 2, lane_t == 0
        x = pltpu.roll(jnp.where(lo_t, tiles[1], tiles[0]), T // 2, 1)
        kend = jnp.sum(kend_s[0] + kend_s[1], axis=1, keepdims=True)
        outs = [jnp.where(lo_t, tiles[0], x), jnp.where(lo_t, x, tiles[1]),
                tiles[2], jnp.where(first, tiles[3], tiles[2]),
                tiles[3], jnp.where(first, tiles[4], tiles[3]),
                tiles[4], jnp.where(first, kend, tiles[4])]
        for i, a in enumerate(outs):
            kt_s[i] = a.astype(BF16)

    ksel = [0, 1, 2, 3, 4, 4, 4, 5] + [6] * 7 + [7]

    def forward(j):
        c0 = pl.multiple_of(j * T, T)
        for m in range(NB):
            kh_s[m] = _dot_nt(fk_ref[m], kt_s[ksel[m]])
            xh_s[m] = _dot(fx_ref[...], x_ref[m * T:(m + 1) * T, pl.ds(c0, T)])

    def pointwise(i, _):
        r0 = pl.multiple_of(i * 8, 8)
        kk, xx, prev = [], [], None
        for m in range(NB):
            a = (kh_s[m, pl.ds(r0, 8), :], kh_s[m, pl.ds(T + r0, 8), :])
            kk.append(a + (a[0] + a[1],))
            b = (xh_s[m, pl.ds(r0, 8), :], xh_s[m, pl.ds(T + r0, 8), :])
            c = b if prev is None else (b[0] - prev[1], b[1] + prev[0])
            xx.append(c + (c[0] + c[1],))
            prev = b
        for p in range(NB):
            s = []
            for c in range(3):
                acc = kk[0][c] * xx[p][c]
                for m in range(1, p + 1):
                    acc = acc + kk[m][c] * xx[p - m][c]
                s.append(acc)
            yh_s[p, pl.ds(r0, 8), :] = _pack(s[0] - s[1], s[2] - s[0] - s[1])
        return _

    def inverse(j):
        for p in range(NB):
            y_s[j, p * T:(p + 1) * T, :] = _dot(g_ref[...], pltpu.bitcast(yh_s[p], BF16))

    qscale = float(DH ** -0.5 * np.log2(np.e))

    def qkv(j):
        def body(i, _):
            r0 = pl.multiple_of(i * 256, 256)
            r = _dot_nt(x_ref[pl.ds(r0, 256), :], wp_s[j])
            q_s[j, pl.ds(r0, 256), :] = r[:, 0:T] * qscale
            k_s[j, pl.ds(HALO + r0, 256), :] = r[:, T:2 * T]
            v_s[j, pl.ds(HALO + r0, 256), :] = r[:, 2 * T:3 * T]
            return _
        jax.lax.fori_loop(0, S // 256, body, None)

    def tile(j, _):
        prep(j)
        jax.lax.fori_loop(0, 16, gen_lo, None)
        jax.lax.fori_loop(0, 8, gen_hi, None)
        jax.lax.fori_loop(0, 32, kmat, None)
        shuffle()
        forward(j)
        jax.lax.fori_loop(0, 16, pointwise, None)
        inverse(j)
        qkv(j)
        return _
    jax.lax.fori_loop(0, NT, tile, None)

    R, RC = 128, 16

    def attend(r0, masked):
        qs = [q_s[t, pl.ds(r0, RC), :] for t in range(NT)]
        ls = []
        for w in range(WIN):
            a = qs[0] * k_s[0, pl.ds(r0 + HALO - DIL * w, RC), :]
            for t in range(1, NT):
                a = a + qs[t] * k_s[t, pl.ds(r0 + HALO - DIL * w, RC), :]
            a = a + pltpu.roll(a, 64, 1)
            a = a + pltpu.roll(a, 32, 1)
            if masked:
                row = jax.lax.broadcasted_iota(jnp.int32, (RC, T), 0) + r0
                a = jnp.where(row >= DIL * w, a, -1e9)
            ls.append(a)
        mx = ls[0]
        for a in ls[1:]:
            mx = jnp.maximum(mx, a)
        es = [jnp.exp2(a - mx) for a in ls]
        den = es[0]
        for e in es[1:]:
            den = den + e
        inv = 1.0 / den
        outs = []
        for t in range(NT):
            a = es[0] * v_s[t, pl.ds(r0 + HALO, RC), :]
            for w in range(1, WIN):
                a = a + es[w] * v_s[t, pl.ds(r0 + HALO - DIL * w, RC), :]
            outs.append((a * inv).astype(BF16))
        return jnp.concatenate(outs, 1)

    def rows(i, _):
        r0 = pl.multiple_of(i * R, R)
        o = jnp.concatenate([attend(r0 + c * RC, c == 0) for c in range(R // RC)], 0)
        a = _dot(o, wop_s[...])
        x = x_ref[pl.ds(r0, R), :].astype(F32)
        gate = jax.nn.sigmoid(jnp.sum(x * gw_ref[...].astype(F32), axis=1, keepdims=True))
        y = jnp.concatenate([y_s[t, pl.ds(r0, R), :] for t in range(NT)], 1)
        b = y + x * dsk_ref[...].astype(F32)
        o_ref[pl.ds(r0, R), :] = (b + gate * (a - b)).astype(BF16)
        return _
    jax.lax.fori_loop(0, S // R, rows, None)


@jax.jit
def pallas_gated_mix__sliding_local_dilated__ssm_conv_s4__prompt_kernel(
    A_x: jax.Array,
    A_wqkv: jax.Array,
    A_wo: jax.Array,
    B_u: jax.Array,
    B_A_re: jax.Array,
    B_A_im: jax.Array,
    B_B_re: jax.Array,
    B_B_im: jax.Array,
    B_C_re: jax.Array,
    B_C_im: jax.Array,
    B_log_dt: jax.Array,
    B_Dskip: jax.Array,
    gate_w: jax.Array,
):
    del B_u
    fx, g, fk = _constants()
    vm = pltpu.VMEM
    out = pl.pallas_call(
        _kernel,
        out_shape=jax.ShapeDtypeStruct((S, D), BF16),
        scratch_shapes=[
            vm((NT, 3 * D, T), F32), vm((NT, 3 * T, D), BF16), vm((D, D), BF16),
            vm((4, N, T), F32), vm((3, NU * T, T), U32), vm((3, NV * T, T), U32),
            vm((2, T, T), F32), vm((32 * 8 * NU, T), F32), vm((8, T, T), BF16),
            vm((NB, 2 * T, T), F32), vm((NB, 2 * T, T), F32), vm((NB, T, T), U32),
            vm((NT, S, T), F32),
            vm((NT, S, T), F32), vm((NT, S + HALO, T), F32), vm((NT, S + HALO, T), F32),
        ],
        compiler_params=pltpu.CompilerParams(vmem_limit_bytes=100 * 1024 * 1024),
    )(A_x.reshape(S, D), A_wqkv, A_wo, B_A_re, B_A_im, B_B_re, B_B_im, B_C_re, B_C_im,
      B_log_dt.reshape(1, D), B_Dskip.reshape(1, D), gate_w.reshape(1, D), fx, g, fk)
    return out.reshape(1, S, D)
```

```python
import jax
import jax.numpy as jnp
import numpy as np
import jax.experimental.pallas as pl
import jax.experimental.pallas.tpu as pltpu

S, D, H, DH, N = 2048, 640, 32, 20, 192
WIN, DIL = 8, 2
T = 128
NT = D // T
NB = S // T
HALO = 16
SINCOS_MAX = 8192.0
LEAD, LAST = 0.15, 1.0
NU, NV = 10, 16
GS = 36
KS = 84
O_PAR = 0
O_KH = O_PAR + 4 * N
O_XH = O_KH + NB * 2 * T
O_SSM = O_XH + NT * NB * 2 * T
O_Q = 0
O_K = O_Q + NT * S
O_V = O_K + NT * (S + HALO)
O_END = O_V + NT * (S + HALO)
F32, BF16, U32 = jnp.float32, jnp.bfloat16, jnp.uint32

_BASES = [0, 1, 2, 3, 4, 5, 6, 7, 256, 258, 260, 262, 512, 516, 768, 772,
          1024, 1280, 1536, 1792]


def _pack_rows(a):
    b = a.astype(np.float32).astype(BF16).view(np.uint16).astype(np.uint32)
    return b[..., 0::2, :] | (b[..., 1::2, :] << 16)


def _constants():
    om = 2.0 * np.pi * (np.arange(T) + 0.25) / T
    ph = np.exp(-1j * om[:, None] * np.arange(T)[None, :])
    fx = np.concatenate([ph.real, ph.imag], 0)
    g = np.stack([ph.real.T, ph.imag.T], -1).reshape(T, 2 * T) / T
    lag = np.arange(S).astype(np.float32).astype(BF16).astype(np.float32).astype(np.int64)
    lane = np.arange(T)
    off = 8 * (2 * (lane // 8) + lane % 2)
    tiles = [np.array(_BASES[4 * t:4 * t + 4])[(lane % 8) // 2] + off for t in range(5)]
    lo = lane < T // 2
    vals = {0: np.where(lo, tiles[0], np.roll(tiles[1], T // 2)),
            1: np.where(lo, np.roll(tiles[0], T // 2), tiles[1])}
    for m in range(2, NB):
        vals[m] = tiles[2 if m < 4 else 3 if m < 8 else 4].copy()
    vals[3][0], vals[7][0], vals[15][0] = 512, 1024, S
    fk = np.zeros((NB, 2 * T, T))
    for m in range(NB):
        blk = lag[m * T:(m + 1) * T]
        e = (blk[:, None] == vals[m][None, :]).astype(np.float64)
        assert (e.sum(1) == 1).all()
        c = ph @ e
        fk[m] = np.concatenate([c.real, c.imag], 0)
    g = np.stack([g[:, :T], g[:, T:]])
    return _pack_rows(fx), _pack_rows(g), _pack_rows(fk)


def _cmul(a, b):
    return a[0] * b[0] - a[1] * b[1], a[0] * b[1] + a[1] * b[0]


def _csq(a):
    t = a[0] * a[1]
    return a[0] * a[0] - a[1] * a[1], t + t


def _tree(op, xs):
    while len(xs) > 1:
        xs = [op(a, b) for a, b in zip(xs[0::2], xs[1::2])]
    return xs[0]


def _pack(a, b):
    return pltpu.pack_elementwise([a, b], packed_dtype=BF16)


def _words(a):
    return pltpu.bitcast(a.astype(BF16), U32)


def _halves(a):
    return pltpu.bitcast(a, BF16)


def _dot(a, b):
    return jnp.dot(a, b, preferred_element_type=F32)


def _dot_nt(a, b):
    return jax.lax.dot_general(a, b, (((1,), (1,)), ((), ())), preferred_element_type=F32)


def _sincos(x):
    k = jnp.floor(x * (2.0 / np.pi) + 0.5)
    r = ((x - k * 1.5703125) - k * 4.837512969970703125e-4) - k * 7.54978995489188216e-8
    z = r * r
    s = r + r * z * (-1.6666654611e-1 + z * (8.3321608736e-3 + z * -1.9515295891e-4))
    c = 1.0 + z * (-0.5 + z * (4.166664568298827e-2
                               + z * (-1.388731625493765e-3 + z * 2.443315711809948e-5)))
    n = k.astype(jnp.int32)
    odd = (n & 1) == 1
    s, c = jnp.where(odd, c, s), jnp.where(odd, s, c)
    return jnp.where((n & 2) == 2, -s, s), jnp.where(((n + 1) & 2) == 2, -c, c)


def _loop(n, body):
    jax.lax.fori_loop(0, n, lambda i, c: body(i), None)


def _interleave(*streams):
    done = [0] * len(streams)
    live = list(range(len(streams)))
    while live:
        i = min(live, key=lambda n: streams[n][2]
                + (streams[n][3] - streams[n][2]) * done[n] / streams[n][1])
        if next(streams[i][0], None) is None:
            live.remove(i)
        done[i] += 1


def _chain(gens):
    for g in gens:
        yield from g


def _kernel(x_hbm, wqkv_hbm, wo_hbm, are_hbm, aim_hbm, bre_hbm, bim_hbm, cre_hbm, cim_hbm,
            ldt_ref, dsk_ref, gw_ref, fx_hbm, g_hbm, fk_hbm, o_hbm,
            x_ref, wqkv_ref, wo_ref, ssm_ref, fx_ref, g_ref, fk_ref, o_ref,
            xs_s, gate_s, wt_s, wp_s, wop_s, ar_s, at_in, us_s, vs_s, kend_s, ko_s, yh_s, tmp_s, at_a, at_b,
            sems, osem):
    lane = jax.lax.broadcasted_iota(jnp.int32, (8, T), 1)
    lo = lane < T // 2

    ssm_hbm = (are_hbm, aim_hbm, bre_hbm, bim_hbm, cre_hbm, cim_hbm)
    pairs = [(h.at[:, 0:T], ssm_ref.at[i, :, 0:T]) for i, h in enumerate(ssm_hbm)]
    pairs += [(x_hbm, x_ref), (fx_hbm, fx_ref)]
    pairs += [(wqkv_hbm.at[:, s * D:(s + 1) * D], wqkv_ref.at[:, s * D:(s + 1) * D]) for s in range(3)]
    pairs += [(h.at[:, T:D], ssm_ref.at[i, :, T:D]) for i, h in enumerate(ssm_hbm)]
    pairs += [(fk_hbm, fk_ref), (wo_hbm, wo_ref), (g_hbm, g_ref)]
    copies = [pltpu.make_async_copy(a, b, sems.at[i]) for i, (a, b) in enumerate(pairs)]
    cp_ssm0, cp_x, cp_w, cp_ssm1, cp_rest = (
        copies[0:6], copies[6:8], copies[8:11], copies[11:17], copies[17:20])
    for c in cp_ssm0 + cp_x:
        c.start()

    tokens, always = [], []

    def post(a, every):
        tokens.extend(a[r - 8:r] for r in range(every, a.shape[0] + 1, every))

    def pace(x):
        if not tokens:
            return x
        return jnp.where(always[0], x, tokens.pop(0))

    def x_repack(i):
        r0 = pl.multiple_of(i * T, T)
        h0 = pl.multiple_of(i * (T // 2), T // 2)
        acc = None
        for t in range(NT):
            x = x_ref[pl.ds(r0, T), t * T:(t + 1) * T]
            xs_s[t, pl.ds(h0, T // 2), :] = pltpu.bitcast(x, U32)
            xg = x.astype(F32) * gw_ref[:, t * T:(t + 1) * T].astype(F32)
            acc = xg if acc is None else acc + xg
        gate = jax.nn.sigmoid(jnp.sum(acc, axis=1, keepdims=True))
        gate_s[pl.ds(r0, T), :] = jnp.broadcast_to(gate, (T, T))

    def w_qkv(s):
        for c in range(NT):
            for kt in range(NT):
                w = wqkv_ref[kt * T:(kt + 1) * T, pl.ds(pl.multiple_of(s * D + c * T, T), T)]
                wt_s[kt, c * T:(c + 1) * T, :] = w.astype(F32).T
                yield 1
        for t in range(NT):
            for kt in range(NT):
                rows = [wt_s[kt, pl.ds(4 * t + i, H, stride=DH), :] for i in range(4)]
                wp_s[t, kt, pl.ds(pl.multiple_of(s * (T // 2), T // 2), T // 2), :] = _words(
                    jnp.concatenate(rows, 0))
                yield 1

    def w_out():
        for ct in range(NT):
            wt_s[ct] = wo_ref[:, ct * T:(ct + 1) * T].astype(F32)
            for t in range(NT):
                rows = [wt_s[ct, pl.ds(4 * t + i, H, stride=DH), :] for i in range(4)]
                wop_s[ct, t * (T // 2):(t + 1) * (T // 2), :] = _words(jnp.concatenate(rows, 0))

    def put_par(i, a):
        ar_s[O_PAR + i * N:O_PAR + i * N + T, :] = a[0:T].T
        hi = a[T:N]
        ar_s[O_PAR + i * N + T:O_PAR + (i + 1) * N, :] = jnp.concatenate(
            [hi, pltpu.roll(hi, T // 2, 1)], 0).T[0:T // 2]

    def discretize(j):
        c0 = pl.multiple_of(j * T, T)
        dt = jnp.exp(ldt_ref[:, pl.ds(c0, T)].astype(F32)).astype(BF16).astype(F32)
        load = lambda i: ssm_ref[i, :, pl.ds(c0, T)].astype(F32)
        return dt, load, jnp.exp(dt * load(0)), dt * load(1)

    def prep(j):
        dt, load, mag, ang = discretize(j)
        sin, cos = _sincos(ang)
        w = _cmul((load(4), load(5)), (dt * load(2), dt * load(3)))
        for i, a in enumerate((mag * cos, mag * sin, w[0], -w[1])):
            put_par(i, a)
        return jnp.max(jnp.abs(ang))

    def prep_wide(j, ang_max):
        def redo(_):
            _, _, mag, ang = discretize(j)
            put_par(0, mag * jnp.cos(ang))
            put_par(1, mag * jnp.sin(ang))
        _loop(jnp.where(ang_max <= SINCOS_MAX, 0, 1), redo)

    GEN_STEPS = 28

    def gen(r, hi):
        r0 = pl.multiple_of(r * 8, 8)
        d0 = (r // 4) * GS + (r % 4) * 8
        s0 = T + r0 if hi else r0

        def put(dst, i, a, b):
            re, im = _pack(a[0], b[0]), _pack(a[1], b[1])
            if hi:
                t = pltpu.roll(jnp.where(lo, im, re), T // 2, 1)
                dst[2, pl.ds(i * 4 * GS + d0, 8), :] = jnp.where(lo, re, t)
                dst[2, pl.ds(i * 4 * GS + 2 * GS + d0, 8), :] = jnp.where(lo, t, im)
            else:
                dst[0, pl.ds(i * 4 * GS + d0, 8), :] = re
                dst[1, pl.ds(i * 4 * GS + d0, 8), :] = im

        conj = lambda a: (a[0], -a[1])
        p = (ar_s[pl.ds(O_PAR + 0 * N + s0, 8), :], ar_s[pl.ds(O_PAR + 1 * N + s0, 8), :])
        p2 = _csq(p)
        p4 = _csq(p2)
        q = _csq(p4)
        q2 = _csq(q)
        q4 = _csq(q2)
        yield 1
        v = [(jnp.ones_like(q[0]), jnp.zeros_like(q[0])), q, q2, _cmul(q, q2)]
        for i in range(NV // 2):
            put(vs_s, 2 * i, v[0], v[1])
            yield 1
            put(vs_s, 2 * i + 1, v[2], v[3])
            if i == 0:
                v = [q4] + [_cmul(a, q4) for a in v[1:]]
            elif i < NV // 2 - 1:
                v = [_cmul((pace(a[0]), a[1]), q4) for a in v[:1]] + [_cmul(a, q4) for a in v[1:]]
            yield 1
        b1 = conj(_cmul(v[0], q4))
        u = [(ar_s[pl.ds(O_PAR + 2 * N + s0, 8), :], ar_s[pl.ds(O_PAR + 3 * N + s0, 8), :])]
        u += [_cmul(u[0], conj(p))]
        put(us_s, 0, u[0], u[1])
        yield 1
        u += [_cmul(a, conj(p2)) for a in u]
        put(us_s, 1, u[2], u[3])
        yield 1
        u += [_cmul(a, conj(p4)) for a in u[0:2]]
        put(us_s, 2, u[4], u[5])
        yield 1
        u += [_cmul(a, conj(p4)) for a in u[2:4]]
        put(us_s, 3, u[6], u[7])
        yield 1
        b2 = _csq(b1)
        b4 = _csq(b2)
        for i, (a, b, f) in enumerate(((0, 2, b1), (4, 6, b1), (0, 4, b2), (8, 10, b2),
                                       (0, 8, b4), (12, 14, b4))):
            u += [_cmul((pace(u[a][0]), u[a][1]), f), _cmul(u[b], f)]
            put(us_s, 4 + i, u[-2], u[-1])
            yield 1
        last = u[16][0] * b4[0] - u[16][1] * b4[1]
        if hi:
            kend_s[1, pl.ds(r0, 8), :] = jnp.where(lo, last, 0.0)
            kend_s[1, pl.ds(T // 2 + r0, 8), :] = jnp.where(lo, 0.0, last)
        else:
            kend_s[0, pl.ds(r0, 8), :] = last
        yield 1

    def kmat(g):
        u = jnp.concatenate([_halves(us_s[t, pl.ds(g, 4 * NU, stride=GS), :]) for t in range(3)], 1)
        v = jnp.concatenate([_halves(vs_s[t, pl.ds(g, 4 * NV, stride=GS), :]) for t in range(3)], 1)
        ko_s[pl.ds(g * KS, 8 * NU), :] = _dot_nt(u, v)

    def spectrum_k(j):
        lane32 = jax.lax.broadcasted_iota(jnp.int32, (32, T), 1)
        slot = (lane32 % 8) // 2

        def gather(t):
            parts = []
            for c in range(4):
                acc = None
                for jj in range(4):
                    k = 4 * t + jj
                    a = ko_s[pl.ds((k // 2) * 8 + 2 * c + k % 2, 32, stride=KS), :]
                    if jj != c:
                        a = pltpu.roll(a, (2 * (jj - c)) % T, 1)
                    acc = a if acc is None else jnp.where(slot == jj, a, acc)
                parts.append(acc)
            return jnp.concatenate(parts, 0)

        def emit(ms, taps):
            taps = taps.astype(BF16)
            for m in ms:
                ar_s[O_KH + m * 2 * T:O_KH + (m + 1) * 2 * T, :] = _dot_nt(_halves(fk_ref[m]), taps)

        lane_t = jax.lax.broadcasted_iota(jnp.int32, (T, T), 1)
        lo_t, first = lane_t < T // 2, lane_t == 0
        t4 = gather(4)
        emit(range(8, 15), t4)
        kend = jnp.sum(kend_s[0] + kend_s[1], axis=1, keepdims=True)
        emit([15], jnp.where(first, kend, t4))
        t3 = gather(3)
        emit(range(4, 7), t3)
        emit([7], jnp.where(first, t4, t3))
        t2 = gather(2)
        emit([2], t2)
        emit([3], jnp.where(first, t3, t2))
        t1, t0 = gather(1), gather(0)
        x = pltpu.roll(jnp.where(lo_t, t1, t0), T // 2, 1)
        emit([1], jnp.where(lo_t, x, t1))
        skip = dsk_ref[:, pl.ds(pl.multiple_of(j * T, T), T)].astype(F32)
        skip = jnp.broadcast_to(skip, (T, T)).T
        emit([0], jnp.where(lo_t, t0, x) + jnp.where(first, skip, 0.0))

    def spectrum_x(j):
        for m in range(NB):
            r = _dot(_halves(fx_ref[...]), _halves(xs_s[j, m * (T // 2):(m + 1) * (T // 2), :]))
            ar_s[pl.ds(pl.multiple_of(O_XH + (j * NB + m) * 2 * T, 2 * T), 2 * T), :] = r
            yield 1

    PW_STEPS = 30

    def pointwise(j, i):
        r0 = pl.multiple_of(i * 8, 8)
        kh_s, xh_s = O_KH, O_XH + j * NB * 2 * T
        re = lambda o, m: ar_s[pl.ds(o + m * 2 * T + r0, 8), :]
        im = lambda o, m: ar_s[pl.ds(o + m * 2 * T + T + r0, 8), :]
        xr = lambda m: re(xh_s, m) - im(xh_s, m - 1) if m else re(xh_s, m)
        xi = lambda m: im(xh_s, m) + re(xh_s, m - 1) if m else im(xh_s, m)
        acc = None
        for c in range(3):
            xs = [(xr(m), xi(m), xr(m) + xi(m))[c] for m in range(NB)]
            work = 0
            for m in range(NB):
                k = re(kh_s, m) if c == 0 else im(kh_s, m) if c == 1 else re(kh_s, m) + im(kh_s, m)
                if work < NB - m:
                    k = pace(k)
                if m == 0:
                    acc = [k * a for a in xs] if c < 2 else [k * a - b for a, b in zip(xs, acc)]
                else:
                    acc = acc[:m] + [acc[p] + k * xs[p - m] for p in range(m, NB)]
                work += NB - m
                if work >= 12:
                    work -= 12
                    yield 1
            if c == 0:
                for p in range(NB):
                    tmp_s[p] = acc[p]
            elif c == 1:
                for p in range(NB):
                    s0 = tmp_s[p]
                    tmp_s[NB + p] = s0 - acc[p]
                    acc[p] = s0 + acc[p]
            else:
                for p in range(NB):
                    yh_s[j, p, pl.ds(r0, 8), :] = _pack(tmp_s[NB + p], acc[p])

    qscale = float(DH ** -0.5 * np.log2(np.e))
    QR = 128

    def qkv(j, i, every):
        r0 = pl.multiple_of(i * QR, QR)
        h0 = pl.multiple_of(i * (QR // 2), QR // 2)
        for s in range(3):
            x = jnp.concatenate([_halves(xs_s[t, pl.ds(h0, QR // 2), :]) for t in range(NT)], 1)
            w = jnp.concatenate([_halves(wp_s[j, t, s * (T // 2):(s + 1) * (T // 2), :])
                                 for t in range(NT)], 1)
            acc = _dot_nt(x, w)
            if s == 0:
                at_in[pl.ds(O_Q + j * S + r0, QR), :] = acc * qscale
            else:
                at_in[pl.ds((O_K, O_V)[s - 1] + j * (S + HALO) + HALO + r0, QR), :] = acc
            post(acc, every)
            yield 1

    def window(r0, masked):
        qs = [at_in[pl.ds(O_Q + t * S + r0, 8), :] for t in range(NT)]
        ls = []
        for w in range(WIN):
            a = None
            for t in range(NT):
                k = at_in[pl.ds(O_K + t * (S + HALO) + r0 + HALO - DIL * w, 8), :]
                kq = qs[t] * (pace(k) if t == 0 and w % 4 == 0 else k)
                a = kq if a is None else a + kq
            ls.append((a, pltpu.roll(a, 64, 1)))
        yield None
        ls = [a + b for a, b in ls]
        ls = [(a, pltpu.roll(a, 32, 1)) for a in ls]
        yield None
        ls = [a + b for a, b in ls]
        if masked:
            row = jax.lax.broadcasted_iota(jnp.int32, (8, T), 0) + r0
            ls = [jnp.where(row >= DIL * w, a, -1e9 * np.log2(np.e)) for w, a in enumerate(ls)]
        mx = _tree(jnp.maximum, ls)
        es = [jnp.exp2(a - mx) for a in ls]
        yield None
        inv = gate_s[pl.ds(r0, 8), :] * pl.reciprocal(_tree(jnp.add, es), full_range=False)
        outs = []
        for t in range(NT):
            a = None
            for w in range(WIN):
                v = at_in[pl.ds(O_V + t * (S + HALO) + r0 + HALO - DIL * w, 8), :]
                pv = es[w] * (pace(v) if w == 0 and t % 2 == 0 else v)
                a = pv if a is None else a + pv
            outs.append(a)
        yield [a * inv for a in outs]

    def attend(i, dst, first):
        r0 = pl.multiple_of(i * T, T)
        n = T // 8
        gens = [window(r0 + 8 * c, first and 8 * c < HALO) for c in range(n)]
        for step in range(n + 3):
            for c in range(step, step - 4, -1):
                if 0 <= c < n:
                    out = next(gens[c])
                    if out is not None:
                        if c % 2:
                            for t in range(NT):
                                dst[t, (c // 2) * 8:(c // 2 + 1) * 8, :] = _words(
                                    jnp.concatenate([top[t], out[t]], 0))
                        top = out
            yield 1

    def out_copy(i):
        r0 = pl.multiple_of(i * T, T)
        return pltpu.make_async_copy(o_ref.at[pl.ds(r0, T), :], o_hbm.at[pl.ds(r0, T), :], osem)

    def mix(i, src):
        r0 = pl.multiple_of(i * T, T)
        for ct in range(NT):
            y = _dot(jnp.concatenate([_halves(g_ref[h]) for h in range(2)], 1), _halves(yh_s[ct, i]))
            a = _dot(jnp.concatenate([_halves(src[t]) for t in range(NT)], 1), _halves(wop_s[ct]))
            acc = a + (1.0 - gate_s[pl.ds(r0, T), :]) * y
            o_ref[pl.ds(r0, T), ct * T:(ct + 1) * T] = acc.astype(BF16)
            post(acc, 8)
            yield 1

    def gen_streams(i):
        return [(_chain([gen(4 * i + 2 * u, False), gen(4 * i + 2 * u + 1, False), gen(2 * i + u, True)]),
                 3 * GEN_STEPS, 0.0, 1.0) for u in range(2)]

    def qkv_stream(j, i0, n, every):
        return (_chain([qkv(j, i0 + u, every) for u in range(n)]), n * 3, LEAD, LAST)

    def overlap(*streams):
        always.append(at_in[O_K:O_K + 8, :] == 0.0)
        _interleave(*streams)
        tokens.clear()
        always.clear()

    def kmats(i):
        for u in range(16):
            kmat(16 * i + u)

    for t in range(NT):
        at_in[pl.ds(O_K + t * (S + HALO), HALO), :] = jnp.zeros((HALO, T), F32)
        at_in[pl.ds(O_V + t * (S + HALO), HALO), :] = jnp.zeros((HALO, T), F32)
    for c in cp_ssm0:
        c.wait()
    cp_w[0].start()
    prep_wide(0, prep(0))
    _loop(4, lambda i: _interleave(*gen_streams(i)))
    for c in cp_w[1:]:
        c.start()
    _loop(2, kmats)
    for c in cp_x:
        c.wait()
    for c in cp_rest[:1] + cp_ssm1 + cp_rest[1:]:
        c.start()
    _loop(NB, x_repack)
    _interleave((_chain([spectrum_x(0), spectrum_x(1)]), 2 * NB, 0.0, 1.0))
    for s in range(3):
        cp_w[s].wait()
        _interleave((spectrum_x(2 + s), NB, 0.0, 1.0), (w_qkv(s), 2 * NT * NT, 0.0, 1.0))
    for c in cp_rest[:1] + cp_ssm1:
        c.wait()

    nq = S // QR // 8

    def conv_qkv(j, i, i0, n):
        pw = (_chain([pointwise(j, 4 * i + u) for u in range(4)]), 4 * PW_STEPS, 0.0, 1.0)
        overlap(qkv_stream(j, i0, n, 8 * n // nq), pw)

    def tile(j):
        spectrum_k(j)
        prep_wide(j + 1, prep(j + 1))
        _loop(4, lambda i: conv_qkv(j, i, nq * i, nq))
        _loop(4, lambda i: overlap(qkv_stream(j, nq * (4 + i), nq, 16), *gen_streams(i)))
        _loop(2, kmats)
    _loop(NT - 1, tile)
    for c in cp_rest[1:]:
        c.wait()
    spectrum_k(NT - 1)
    w_out()
    _loop(4, lambda i: conv_qkv(NT - 1, i, 2 * nq * i, 2 * nq))

    overlap((attend(0, at_a, True), 19, 0.0, 1.0))

    def rows(i, src, dst):
        overlap((mix(i - 1, src), NT, LEAD, LAST), (attend(i, dst, False), 19, 0.0, 1.0))
        out_copy(i - 1).start()

    def rows2(i):
        rows(2 * i + 1, at_a, at_b)
        rows(2 * i + 2, at_b, at_a)
    _loop(NB // 2 - 1, rows2)
    rows(NB - 1, at_a, at_b)
    overlap((mix(NB - 1, at_b), NT, 0.0, 1.0))
    out_copy(NB - 1).start()
    for i in range(NB):
        out_copy(i).wait()


@jax.jit
def pallas_gated_mix__sliding_local_dilated__ssm_conv_s4__prompt_kernel(
    A_x: jax.Array,
    A_wqkv: jax.Array,
    A_wo: jax.Array,
    B_u: jax.Array,
    B_A_re: jax.Array,
    B_A_im: jax.Array,
    B_B_re: jax.Array,
    B_B_im: jax.Array,
    B_C_re: jax.Array,
    B_C_im: jax.Array,
    B_log_dt: jax.Array,
    B_Dskip: jax.Array,
    gate_w: jax.Array,
):
    del B_u
    fx, g, fk = _constants()
    vm = pltpu.VMEM
    hbm = pl.BlockSpec(memory_space=pl.ANY)
    small = pl.BlockSpec(memory_space=vm)
    out = pl.pallas_call(
        _kernel,
        out_shape=jax.ShapeDtypeStruct((S, D), BF16),
        in_specs=[hbm] * 9 + [small] * 3 + [hbm] * 3,
        out_specs=hbm,
        scratch_shapes=[
            vm((S, D), BF16), vm((D, 3 * D), BF16), vm((D, D), BF16), vm((6, N, D), BF16),
            vm(fx.shape, U32), vm(g.shape, U32), vm(fk.shape, U32), vm((S, D), BF16),
            vm((NT, S // 2, T), U32), vm((S, T), F32),
            vm((NT, D, T), F32), vm((NT, NT, 3 * T // 2, T), U32), vm((NT, D // 2, T), U32),
            vm((O_SSM, T), F32), vm((O_END, T), F32),
            vm((3, NU * 4 * GS, T), U32), vm((3, NV * 4 * GS, T), U32),
            vm((2, T, T), F32), vm((32 * KS, T), F32), vm((NT, NB, T, T), U32),
            vm((2 * NB, 8, T), F32), vm((NT, T // 2, T), U32), vm((NT, T // 2, T), U32),
            pltpu.SemaphoreType.DMA((20,)), pltpu.SemaphoreType.DMA(()),
        ],
        compiler_params=pltpu.CompilerParams(vmem_limit_bytes=100 * 1024 * 1024),
    )(A_x.reshape(S, D), A_wqkv, A_wo, B_A_re.T, B_A_im.T, B_B_re.T, B_B_im.T, B_C_re.T, B_C_im.T,
      B_log_dt.reshape(1, D), B_Dskip.reshape(1, D), gate_w.reshape(1, D), fx, g, fk)
    return out.reshape(1, S, D)
```

```python
import jax
import jax.numpy as jnp
import numpy as np
import jax.experimental.pallas as pl
import jax.experimental.pallas.tpu as pltpu

S, D, H, DH, N = 2048, 640, 32, 20, 192
WIN, DIL = 8, 2
T = 128
NT = D // T
NB = S // T
HALO = 16
N_COPIES = 26
SINCOS_MAX = 8192.0
LEAD = 0.15
LEAD2 = 0.04
NC = 4
HEAD = 4
EARLY = 8
PER_ROW = 16
FK_EVERY = 64
KMAT_EVERY = 24
X_LAG = 4
W_LAST = 0.85
LAST = 1.0
QR = 128
PW_EVERY = 8
GEN_EVERY = 16
MR = 64
MIX_EVERY = 8
MIX_LEAD = 0.15
MIX_LAST = 1.0
PACE_K = ()
PACE_V = ()
NU, NV = 10, 16
GS = 36
KS = 84
F32, BF16, U32 = jnp.float32, jnp.bfloat16, jnp.uint32

_BASES = [0, 1, 2, 3, 4, 5, 6, 7, 256, 258, 260, 262, 512, 516, 768, 772,
          1024, 1280, 1536, 1792]


_TAPS = {2: (2, 0, None), 3: (2, 0, 0),
         4: (3, 0, None), 5: (3, 0, None), 6: (3, T - 4, None), 7: (3, T - 4, 4)}
_TAPS.update({m: (4, (8 - m + m % 2) % T, 2 if m == NB - 1 else None) for m in range(8, NB)})
_SLOT = [0, 1, 2, 3] + [4 + (m - 4) // 2 for m in range(4, NB)]
_SHARE = [0, 0, 1, 2, 3, 4, 3, 4] + [5, 6] * 4


def _pack_rows(a):
    b = a.astype(np.float32).astype(BF16).view(np.uint16).astype(np.uint32)
    return b[..., 0::2, :] | (b[..., 1::2, :] << 16)


def _constants():
    om = 2.0 * np.pi * (np.arange(T) + 0.25) / T
    ph = np.exp(-1j * om[:, None] * np.arange(T)[None, :])
    fx = np.concatenate([ph.real, ph.imag], 0)
    g = np.stack([ph.real.T, ph.imag.T], -1).reshape(T, 2 * T) / T
    lag = np.arange(S).astype(np.float32).astype(BF16).astype(np.float32).astype(np.int64)
    lane = np.arange(T)
    off = 8 * (2 * (lane // 8) + lane % 2)
    tiles = [np.array(_BASES[4 * t:4 * t + 4])[(lane % 8) // 2] + off for t in range(5)]
    lo = lane < T // 2
    vals = [np.where(lo, tiles[0], np.roll(tiles[1], T // 2)),
            np.where(lo, np.roll(tiles[0], T // 2), tiles[1])]
    for m in range(2, NB):
        t, shift, end = _TAPS[m]
        v = np.roll(tiles[t], shift)
        vals.append(v if end is None else np.where(lane == end, (m + 1) * T, v))
    fk = np.zeros((max(_SHARE) + 1, 2 * T, T))
    for m in range(NB):
        blk = lag[m * T:(m + 1) * T]
        e = (blk[:, None] == vals[m][None, :]).astype(np.float64)
        assert (e.sum(1) == 1).all()
        c = np.concatenate([(ph @ e).real, (ph @ e).imag], 0)
        assert _SHARE.index(_SHARE[m]) == m or np.array_equal(fk[_SHARE[m]], c)
        fk[_SHARE[m]] = c
    g = np.stack([g[:, :T], g[:, T:]])
    return _pack_rows(fx), _pack_rows(g), _pack_rows(fk)


def _cmul(a, b):
    return a[0] * b[0] - a[1] * b[1], a[0] * b[1] + a[1] * b[0]


def _csq(a):
    t = a[0] * a[1]
    return a[0] * a[0] - a[1] * a[1], t + t


def _tree(op, xs):
    while len(xs) > 1:
        xs = [op(a, b) for a, b in zip(xs[0::2], xs[1::2])]
    return xs[0]


def _pack(a, b):
    return pltpu.pack_elementwise([a, b], packed_dtype=BF16)


def _words(a):
    return pltpu.bitcast(a.astype(BF16), U32)


def _halves(a):
    return pltpu.bitcast(a, BF16)


def _dot(a, b):
    return jnp.dot(a, b, preferred_element_type=F32)


def _dot_nt(a, b):
    return jax.lax.dot_general(a, b, (((1,), (1,)), ((), ())), preferred_element_type=F32)


def _sincos(x):
    k = jnp.floor(x * (2.0 / np.pi) + 0.5)
    r = ((x - k * 1.5703125) - k * 4.837512969970703125e-4) - k * 7.54978995489188216e-8
    z = r * r
    s = r + r * z * (-1.6666654611e-1 + z * (8.3321608736e-3 + z * -1.9515295891e-4))
    c = 1.0 + z * (-0.5 + z * (4.166664568298827e-2
                               + z * (-1.388731625493765e-3 + z * 2.443315711809948e-5)))
    n = k.astype(jnp.int32)
    odd = (n & 1) == 1
    s, c = jnp.where(odd, c, s), jnp.where(odd, s, c)
    return jnp.where((n & 2) == 2, -s, s), jnp.where(((n + 1) & 2) == 2, -c, c)


def _loop(n, body):
    jax.lax.fori_loop(0, n, lambda i, c: body(i), None)


def _interleave(*streams):
    done = [0] * len(streams)
    live = list(range(len(streams)))
    while live:
        i = min(live, key=lambda n: streams[n][2]
                + (streams[n][3] - streams[n][2]) * done[n] / streams[n][1])
        work = next(streams[i][0], None)
        if work is None:
            live.remove(i)
        else:
            done[i] += work


def _alternate(a, b):
    for x, y in zip(a, b):
        yield x
        yield y


def _chain(gens):
    for g in gens:
        yield from g


def _kernel(x_hbm, wqkv_hbm, wo_hbm, are_hbm, aim_hbm, bre_hbm, bim_hbm, cre_hbm, cim_hbm,
            ldt_ref, dsk_ref, gw_ref, fx_hbm, g_hbm, fk_hbm, o_hbm,
            x_ref, wqkv_ref, wo_ref, ssm_ref, fx_ref, g_ref, fk_ref, o_ref,
            xs_s, gate_s, wt_s, wp_s, wop_s, par_s, us_s, vs_s, kend_s, ko_s, kt_s,
            kh_s, xh_s, yh_s, tmp_s, q_s, k_s, v_s, at_s, cur_s, zero_s,
            sems, osem):
    lane = jax.lax.broadcasted_iota(jnp.int32, (8, T), 1)
    lo = lane < T // 2

    ssm_hbm = (are_hbm, aim_hbm, bre_hbm, bim_hbm, cre_hbm, cim_hbm)
    sem_ids = iter(range(N_COPIES))
    copy = lambda a, b: pltpu.make_async_copy(a, b, sems.at[next(sem_ids)])
    cp_ssm = [[copy(h.at[:, a:b], ssm_ref.at[i, :, a:b]) for i, h in enumerate(ssm_hbm)]
              for a, b in ((0, T), (T, 2 * T), (2 * T, D))]
    cp_x = [copy(x_hbm, x_ref), copy(fx_hbm, fx_ref)]
    cp_w = [copy(wqkv_hbm.at[:, s * D:(s + 1) * D], wqkv_ref.at[:, s * D:(s + 1) * D]) for s in range(3)]
    cp_fk = copy(fk_hbm, fk_ref)
    cp_out = [copy(wo_hbm, wo_ref), copy(g_hbm, g_ref)]
    for c in cp_ssm[0] + cp_x:
        c.start()

    tokens, always = [], []

    def post(a, every):
        tokens.extend(a[r - 8:r] for r in range(every, a.shape[0] + 1, every))

    def pace(x, lag=0):
        if len(tokens) <= lag:
            return x
        head = jnp.where(always[0], x[:8], pltpu.bitcast(tokens.pop(0), x.dtype))
        return head if x.shape[0] == 8 else jnp.concatenate([head, x[8:]], 0)

    def x_block(m):
        acc = None
        for t in range(NT):
            x = x_ref[m * T:(m + 1) * T, t * T:(t + 1) * T]
            words = pltpu.bitcast(x, U32)
            xs_s[t, m * (T // 2):(m + 1) * (T // 2), :] = words
            xh_s[t, m] = _dot(_halves(fx_ref[...]), _halves(pace(words, X_LAG)))
            xg = x.astype(F32) * gw_ref[:, t * T:(t + 1) * T].astype(F32)
            acc = xg if acc is None else acc + xg
            post(acc, T)
            yield 1
        gate = jax.nn.sigmoid(jnp.sum(acc, axis=1, keepdims=True))
        gate_s[m * T:(m + 1) * T, :] = jnp.broadcast_to(gate, (T, T))

    def regroup(src, t):
        rows = []
        for i in range(2):
            w = src[pl.ds(2 * t + i, H, stride=DH // 2), :]
            rows += [pltpu.unpack_elementwise(w, index=e, packed_dtype=BF16, unpacked_dtype=F32)
                     for e in range(2)]
        return _words(jnp.concatenate(rows, 0))

    def w_qkv(s):
        for c in range(NT):
            for kt in range(NT):
                w = wqkv_ref[kt * T:(kt + 1) * T, s * D + c * T:s * D + (c + 1) * T]
                wt_s[kt, c * (T // 2):(c + 1) * (T // 2), :] = pltpu.bitcast(w.T, U32)
                yield 1
        for t in range(NT):
            for kt in range(NT):
                w = regroup(wt_s.at[kt], t)
                wp_s[t, kt, s * (T // 2):(s + 1) * (T // 2), :] = w
                tokens[-1:] = [w[-8:]]
                yield 1

    def w_out():
        for ct in range(NT):
            wt_s[ct] = pltpu.bitcast(wo_ref[:, ct * T:(ct + 1) * T], U32)
            for t in range(NT):
                wop_s[ct, t * (T // 2):(t + 1) * (T // 2), :] = regroup(wt_s.at[ct], t)

    def put_par(i, a):
        par_s[i, 0:T, :] = a[0:T].T
        hi = a[T:N]
        par_s[i, T:N, :] = jnp.concatenate(
            [hi, pltpu.roll(hi, T // 2, 1)], 0).T[0:T // 2]

    def discretize(j):
        c0 = j * T if isinstance(j, int) else pl.multiple_of(j * T, T)
        dt = jnp.exp(ldt_ref[:, pl.ds(c0, T)].astype(F32)).astype(BF16).astype(F32)
        load = lambda i: ssm_ref[i, :, pl.ds(c0, T)].astype(F32)
        return dt, load, jnp.exp(dt * load(0)), dt * load(1)

    def prep(j):
        dt, load, mag, ang = discretize(j)
        sin, cos = _sincos(ang)
        w = _cmul((load(4), load(5)), (dt * load(2), dt * load(3)))
        for i, a in enumerate((mag * cos, mag * sin, w[0], -w[1])):
            put_par(i, a)
        return jnp.max(jnp.abs(ang))

    def prep_wide(j, ang_max):
        def redo(_):
            _, _, mag, ang = discretize(j)
            put_par(0, mag * jnp.cos(ang))
            put_par(1, mag * jnp.sin(ang))
        _loop(jnp.where(ang_max <= SINCOS_MAX, 0, 1), redo)

    GEN_STEPS = 28

    def gen(r, hi):
        r0 = r * 8 if isinstance(r, int) else pl.multiple_of(r * 8, 8)
        d0 = (r // 4) * GS + (r % 4) * 8
        s0 = T + r0 if hi else r0

        def put(dst, i, a, b):
            re, im = _pack(a[0], b[0]), _pack(a[1], b[1])
            if hi:
                t = pltpu.roll(jnp.where(lo, im, re), T // 2, 1)
                dst[2, pl.ds(i * 4 * GS + d0, 8), :] = jnp.where(lo, re, t)
                dst[2, pl.ds(i * 4 * GS + 2 * GS + d0, 8), :] = jnp.where(lo, t, im)
            else:
                dst[0, pl.ds(i * 4 * GS + d0, 8), :] = re
                dst[1, pl.ds(i * 4 * GS + d0, 8), :] = im

        conj = lambda a: (a[0], -a[1])
        p = (par_s[0, pl.ds(s0, 8), :], par_s[1, pl.ds(s0, 8), :])
        p2 = _csq(p)
        p4 = _csq(p2)
        q = _csq(p4)
        q2 = _csq(q)
        q4 = _csq(q2)
        yield 1
        v = [(jnp.ones_like(q[0]), jnp.zeros_like(q[0])), q, q2, _cmul(q, q2)]
        for i in range(NV // 2):
            put(vs_s, 2 * i, v[0], v[1])
            yield 1
            put(vs_s, 2 * i + 1, v[2], v[3])
            if i == 0:
                v = [q4] + [_cmul(a, q4) for a in v[1:]]
            elif i < NV // 2 - 1:
                v = [_cmul((pace(a[0]), a[1]), q4) for a in v[:1]] + [_cmul(a, q4) for a in v[1:]]
            yield 1
        b1 = conj(_cmul(v[0], q4))
        u = [(par_s[2, pl.ds(s0, 8), :], par_s[3, pl.ds(s0, 8), :])]
        u += [_cmul(u[0], conj(p))]
        put(us_s, 0, u[0], u[1])
        yield 1
        u += [_cmul(a, conj(p2)) for a in u]
        put(us_s, 1, u[2], u[3])
        yield 1
        u += [_cmul(a, conj(p4)) for a in u[0:2]]
        put(us_s, 2, u[4], u[5])
        yield 1
        u += [_cmul(a, conj(p4)) for a in u[2:4]]
        put(us_s, 3, u[6], u[7])
        yield 1
        b2 = _csq(b1)
        b4 = _csq(b2)
        for i, (a, b, f) in enumerate(((0, 2, b1), (4, 6, b1), (0, 4, b2), (8, 10, b2),
                                       (0, 8, b4), (12, 14, b4))):
            u += [_cmul((pace(u[a][0]), u[a][1]), f), _cmul(u[b], f)]
            put(us_s, 4 + i, u[-2], u[-1])
            yield 1
        last = u[16][0] * b4[0] - u[16][1] * b4[1]
        if hi:
            kend_s[1, pl.ds(r0, 8), :] = jnp.where(lo, last, 0.0)
            kend_s[1, pl.ds(T // 2 + r0, 8), :] = jnp.where(lo, 0.0, last)
        else:
            kend_s[0, pl.ds(r0, 8), :] = last
        yield 1

    def kmat(g):
        u = jnp.concatenate([_halves(us_s[t, pl.ds(g, 4 * NU, stride=GS), :]) for t in range(3)], 1)
        v = jnp.concatenate([_halves(vs_s[t, pl.ds(g, 4 * NV, stride=GS), :]) for t in range(3)], 1)
        r = _dot_nt(u, v)
        ko_s[pl.ds(g * KS, 8 * NU), :] = r
        post(r, KMAT_EVERY)

    def taps(j):
        lane32 = jax.lax.broadcasted_iota(jnp.int32, (32, T), 1)
        slot = (lane32 % 8) // 2

        def gather(t):
            parts = []
            for c in range(4):
                acc = None
                for jj in range(4):
                    k = 4 * t + jj
                    a = ko_s[pl.ds((k // 2) * 8 + 2 * c + k % 2, 32, stride=KS), :]
                    if jj != c:
                        a = pltpu.roll(a, (2 * (jj - c)) % T, 1)
                    acc = a if acc is None else jnp.where(slot == jj, a, acc)
                parts.append(acc)
            return jnp.concatenate(parts, 0)

        def emit(ms, taps):
            kt_s[_SLOT[ms[0]]] = _words(taps)

        lane_t = jax.lax.broadcasted_iota(jnp.int32, (T, T), 1)
        lo_t, first = lane_t < T // 2, lane_t == 0
        t4 = gather(4)
        emit([8, 9], t4)
        for m in (10, 12):
            emit([m, m + 1], pltpu.roll(t4, _TAPS[m][1], 1))
        kend = jnp.sum(kend_s[0] + kend_s[1], axis=1, keepdims=True)
        emit([14, 15], jnp.where(lane_t == 2, kend, pltpu.roll(t4, _TAPS[14][1], 1)))
        yield 1
        t3 = gather(3)
        emit([4, 5], t3)
        emit([6, 7], jnp.where(lane_t == 4, pltpu.roll(t4, 4, 1), pltpu.roll(t3, _TAPS[6][1], 1)))
        yield 1
        t2 = gather(2)
        emit([2], t2)
        emit([3], jnp.where(first, t3, t2))
        yield 1
        t1 = gather(1)
        yield 1
        t0 = gather(0)
        x = pltpu.roll(jnp.where(lo_t, t1, t0), T // 2, 1)
        emit([1], jnp.where(lo_t, x, t1))
        skip = dsk_ref[:, pl.ds(j * T if isinstance(j, int) else pl.multiple_of(j * T, T), T)].astype(F32)
        skip = jnp.broadcast_to(skip, (T, T)).T
        emit([0], jnp.where(lo_t, t0, x) + jnp.where(first, skip, 0.0))
        yield 1

    def spectrum_k():
        for m in range(NB):
            r = _dot_nt(_halves(fk_ref[_SHARE[m]]), _halves(kt_s[_SLOT[m]]))
            kh_s[m] = r
            post(r, FK_EVERY)
            yield 64

    PW_STEPS = 30

    def pointwise(j, i):
        r0 = pl.multiple_of(i * 8, 8)
        xj = xh_s.at[j]
        re = lambda ref, m: ref[m, pl.ds(r0, 8), :]
        im = lambda ref, m: ref[m, pl.ds(T + r0, 8), :]
        xr = lambda m: re(xj, m) - im(xj, m - 1) if m else re(xj, m)
        xi = lambda m: im(xj, m) + re(xj, m - 1) if m else im(xj, m)
        acc = None
        for c in range(3):
            xs = [(xr(m), xi(m), xr(m) + xi(m))[c] for m in range(NB)]
            work = 0
            for m in range(NB):
                k = re(kh_s, m) if c == 0 else im(kh_s, m) if c == 1 else re(kh_s, m) + im(kh_s, m)
                if work < NB - m:
                    k = pace(k)
                if m == 0:
                    acc = [k * a for a in xs] if c < 2 else [k * a - b for a, b in zip(xs, acc)]
                else:
                    acc = acc[:m] + [acc[p] + k * xs[p - m] for p in range(m, NB)]
                work += NB - m
                if work >= 12:
                    work -= 12
                    yield 1
            if c == 0:
                for p in range(NB):
                    tmp_s[p] = acc[p]
            elif c == 1:
                for p in range(NB):
                    s0 = tmp_s[p]
                    tmp_s[NB + p] = s0 - acc[p]
                    acc[p] = s0 + acc[p]
            else:
                for p in range(NB):
                    yh_s[j, p, pl.ds(r0, 8), :] = _pack(tmp_s[NB + p], acc[p])

    qscale = float(DH ** -0.5 * np.log2(np.e))

    def qkv(j, i, every):
        r0, h0 = i * QR, i * (QR // 2)
        if not isinstance(i, int):
            r0, h0 = pl.multiple_of(r0, QR), pl.multiple_of(h0, QR // 2)
        for s in range(3):
            x = jnp.concatenate([_halves(xs_s[t, pl.ds(h0, QR // 2), :]) for t in range(NT)], 1)
            w = jnp.concatenate([_halves(wp_s[j, t, s * (T // 2):(s + 1) * (T // 2), :])
                                 for t in range(NT)], 1)
            acc = _dot_nt(x, w)
            if s == 0:
                q_s[j, pl.ds(r0, QR), :] = acc * qscale
            else:
                (k_s, v_s)[s - 1][j, pl.ds(HALO + r0, QR), :] = acc
            post(acc, every)
            yield 160

    def window(r0, masked):
        qs = [q_s[t, pl.ds(r0, 8), :] for t in range(NT)]
        ls = []
        for w in range(WIN):
            a = None
            for t in range(NT):
                k = k_s[t, pl.ds(r0 + HALO - DIL * w, 8), :]
                kq = qs[t] * (pace(k) if t == 0 and w in PACE_K else k)
                a = kq if a is None else a + kq
            ls.append((a, pltpu.roll(a, 64, 1)))
        yield None
        ls = [a + b for a, b in ls]
        ls = [(a, pltpu.roll(a, 32, 1)) for a in ls]
        yield None
        ls = [a + b for a, b in ls]
        if masked:
            row = jax.lax.broadcasted_iota(jnp.int32, (8, T), 0) + r0
            ls = [jnp.where(row >= DIL * w, a, -1e9 * np.log2(np.e)) for w, a in enumerate(ls)]
        mx = _tree(jnp.maximum, ls)
        es = [jnp.exp2(a - mx) for a in ls]
        yield None
        inv = gate_s[pl.ds(r0, 8), :] * pl.reciprocal(_tree(jnp.add, es), full_range=False)
        outs = []
        for t in range(NT):
            a = None
            for w in range(WIN):
                v = v_s[t, pl.ds(r0 + HALO - DIL * w, 8), :]
                pv = es[w] * (pace(v) if w == 0 and t in PACE_V else v)
                a = pv if a is None else a + pv
            outs.append(a)
        yield [a * inv for a in outs]

    def attend(r0, n, first=False):
        gens = [window(r0 + 8 * c, first and 8 * c < HALO) for c in range(n)]
        for step in range(n + 3):
            for c in range(step, step - 4, -1):
                if 0 <= c < n:
                    out = next(gens[c])
                    if out is not None:
                        if c % 2:
                            h0 = r0 // 2 + (c // 2) * 8
                            h0 = h0 if isinstance(h0, int) else pl.multiple_of(h0, 8)
                            for t in range(NT):
                                at_s[t, pl.ds(h0, 8), :] = _words(jnp.concatenate([top[t], out[t]], 0))
                        top = out
            yield 1

    def stage(i):
        h0 = i * (T // 2)
        cur_s[...] = at_s[:, pl.ds(h0 if isinstance(i, int) else pl.multiple_of(h0, T // 2), T // 2), :]

    def out_copy(i):
        r0 = pl.multiple_of(i * T, T)
        return pltpu.make_async_copy(o_ref.at[pl.ds(r0, T), :], o_hbm.at[pl.ds(r0, T), :], osem)

    def mix(i):
        for ct in range(NT):
            for h in range(0, T, MR):
                r0 = pl.multiple_of(i * T + h, MR)
                hs = slice(h // 2, (h + MR) // 2)
                y = _dot(jnp.concatenate([_halves(g_ref[b, hs, :]) for b in range(2)], 1),
                         _halves(yh_s[ct, i]))
                a = _dot(jnp.concatenate([_halves(cur_s[t, hs, :]) for t in range(NT)], 1),
                         _halves(wop_s[ct]))
                acc = a + (1.0 - gate_s[pl.ds(r0, MR), :]) * y
                o_ref[pl.ds(r0, MR), ct * T:(ct + 1) * T] = acc.astype(BF16)
                post(acc, MIX_EVERY)
                yield 1

    def gen_streams(i0, n):
        units = lambda i, u: [gen(4 * i + 2 * u, False), gen(4 * i + 2 * u + 1, False), gen(2 * i + u, True)]
        return [(_chain([g for i in range(n) for g in units(i0 + i, u)]), 3 * n * GEN_STEPS, 0.0, 1.0)
                for u in range(2)]

    def qkvs(j, i0, n, every):
        return _chain([qkv(j, i0 + u, every) for u in range(n)])

    def kmats(g0, n):
        for u in range(n):
            kmat(g0 + u)
            yield 60

    def overlap(*streams):
        always.append(zero_s[...] == 0.0)
        _interleave(*streams)
        tokens.clear()
        always.clear()

    for t in range(NT):
        k_s[t, 0:HALO, :] = jnp.zeros((HALO, T), F32)
        v_s[t, 0:HALO, :] = jnp.zeros((HALO, T), F32)
    zero_s[...] = jnp.zeros((8, T), F32)
    for c in cp_ssm[0]:
        c.wait()
    cp_w[0].start()
    prep_wide(0, prep(0))
    cp_w[1].start()
    _loop(4, lambda i: overlap(*gen_streams(i, 1)))
    for c in [cp_w[2], cp_fk] + cp_ssm[1]:
        c.start()
    _loop(2, lambda i: overlap((kmats(16 * i, 16), 1, 0.0, 1.0)))
    for c in cp_x:
        c.wait()
    for c in cp_ssm[2] + cp_out:
        c.start()
    for s, (m0, m1) in enumerate(((0, 6), (6, 11), (11, NB))):
        cp_w[s].wait()
        xs = (_chain([x_block(m) for m in range(m0, m1)]), NT * (m1 - m0), 0.0, 1.0)
        overlap(xs, (w_qkv(s), 2 * NT * NT, 0.0, W_LAST))
    for c in [cp_fk] + cp_ssm[1]:
        c.wait()

    def pws(j, i0, n):
        return (_chain([pointwise(j, i0 + u) for u in range(n)]), n * PW_STEPS, 0.0, 1.0)

    def tile(j):
        @pl.when(j == 1)
        def _():
            for c in cp_ssm[2]:
                c.wait()
        overlap((qkvs(j, 0, 2, T), 960, 0.0, 1.0), (taps(j), 5, 0.0, 1.0))
        prep_wide(j + 1, prep(j + 1))
        mxu = _chain([spectrum_k(), qkvs(j, 2, 6, GEN_EVERY)])
        overlap((mxu, 1024 + 6 * 480, LEAD2, LAST), *gen_streams(0, 4))

        def conv(i):
            mxu = _chain([kmats(32 // NC * i, 32 // NC), qkvs(j, 8 + 8 // NC * i, 8 // NC, PW_EVERY)])
            overlap((mxu, (1920 + 8 * 480) // NC, LEAD, LAST), pws(j, 16 // NC * i, 16 // NC))
        _loop(NC, conv)
    _loop(NT - 1, tile)

    j = NT - 1
    for c in cp_out:
        c.wait()
    overlap((qkvs(j, 0, HEAD, T), 480 * HEAD, 0.0, 1.0), (taps(j), 5, 0.0, 0.5))
    w_out()
    overlap((spectrum_k(), 1024, LEAD, LAST), (attend(0, 16, True), 19, 0.0, 1.0))

    def last_conv(i):
        n = (NB - HEAD) // 4
        r0 = pl.multiple_of(T + i * (8 * EARLY), 16)
        overlap((qkvs(j, HEAD + n * i, n, PW_EVERY), 480 * n, LEAD, LAST), pws(j, 4 * i, 4), (attend(r0, EARLY), EARLY + 3, 0.0, 1.0))
    _loop(4, last_conv)

    late = (S - T) // 8 - 4 * EARLY
    n_mixed = min(late // PER_ROW, NB - 1)
    assert n_mixed * PER_ROW == late and PER_ROW % 2 == 0 and EARLY % 2 == 0
    assert 8 * 4 * EARLY <= (HEAD - 1) * T
    assert all(T + 8 * (4 * EARLY + PER_ROW * (i + 1)) >= (i + 2) * T for i in range(n_mixed))
    stage(0)

    def rows(i, mixed):
        st = [(mix(i), NT * T // MR, MIX_LEAD, MIX_LAST)]
        if mixed:
            r0 = pl.multiple_of(T + 8 * (4 * EARLY + PER_ROW * i), 16)
            st.append((attend(r0, PER_ROW), PER_ROW + 3, 0.0, 1.0))
        overlap(*st)
        stage(jnp.minimum(i + 1, NB - 1))
        out_copy(i).start()
    _loop(n_mixed, lambda i: rows(i, True))
    _loop(NB - n_mixed, lambda i: rows(n_mixed + i, False))
    for i in range(NB):
        out_copy(i).wait()


@jax.jit
def pallas_gated_mix__sliding_local_dilated__ssm_conv_s4__prompt_kernel(
    A_x: jax.Array,
    A_wqkv: jax.Array,
    A_wo: jax.Array,
    B_u: jax.Array,
    B_A_re: jax.Array,
    B_A_im: jax.Array,
    B_B_re: jax.Array,
    B_B_im: jax.Array,
    B_C_re: jax.Array,
    B_C_im: jax.Array,
    B_log_dt: jax.Array,
    B_Dskip: jax.Array,
    gate_w: jax.Array,
):
    del B_u
    fx, g, fk = _constants()
    vm = pltpu.VMEM
    hbm = pl.BlockSpec(memory_space=pl.ANY)
    small = pl.BlockSpec(memory_space=vm)
    out = pl.pallas_call(
        _kernel,
        out_shape=jax.ShapeDtypeStruct((S, D), BF16),
        in_specs=[hbm] * 9 + [small] * 3 + [hbm] * 3,
        out_specs=hbm,
        scratch_shapes=[
            vm((S, D), BF16), vm((D, 3 * D), BF16), vm((D, D), BF16), vm((6, N, D), BF16),
            vm(fx.shape, U32), vm(g.shape, U32), vm(fk.shape, U32), vm((S, D), BF16),
            vm((NT, S // 2, T), U32), vm((S, T), F32),
            vm((NT, D // 2, T), U32), vm((NT, NT, 3 * T // 2, T), U32), vm((NT, D // 2, T), U32),
            vm((4, N, T), F32), vm((3, NU * 4 * GS, T), U32), vm((3, NV * 4 * GS, T), U32),
            vm((2, T, T), F32), vm((32 * KS, T), F32), vm((max(_SLOT) + 1, T // 2, T), U32),
            vm((NB, 2 * T, T), F32), vm((NT, NB, 2 * T, T), F32), vm((NT, NB, T, T), U32),
            vm((2 * NB, 8, T), F32),
            vm((NT, S, T), F32), vm((NT, S + HALO, T), F32), vm((NT, S + HALO, T), F32),
            vm((NT, S // 2, T), U32), vm((NT, T // 2, T), U32), vm((8, T), F32),
            pltpu.SemaphoreType.DMA((N_COPIES,)), pltpu.SemaphoreType.DMA(()),
        ],
        compiler_params=pltpu.CompilerParams(vmem_limit_bytes=100 * 1024 * 1024),
    )(A_x.reshape(S, D), A_wqkv, A_wo, B_A_re.T, B_A_im.T, B_B_re.T, B_B_im.T, B_C_re.T, B_C_im.T,
      B_log_dt.reshape(1, D), B_Dskip.reshape(1, D), gate_w.reshape(1, D), fx, g, fk)
    return out.reshape(1, S, D)
```

```python
import jax
import jax.numpy as jnp
import numpy as np
import jax.experimental.pallas as pl
import jax.experimental.pallas.tpu as pltpu

S, D, H, DH, N = 2048, 640, 32, 20, 192
WIN, DIL = 8, 2
T = 128
NT = D // T
NB = S // T
HALO = 16
N_COPIES = 28
SINCOS_MAX = 8192.0
LEAD = 0.08
LEAD2 = 0.12
LAST = 0.95
LAST2 = 0.95
QR = 256
HEAD = 2
NL = 2
FIRST = 28
EARLY = 16
RB = 256
PER_ROW = 28
GEN_SERIAL = True
FK_EVERY = 256
KMAT_EVERY = 40
PW_EVERY = 16
GEN_EVERY = 8
MIX_EVERY = 64
MIX_LEAD = 0.05
MIX_LAST = 1.0
PACE_K = ()
PACE_V = (0,)
X_LAG = 8
X_SERIAL = True
X_GAP = 1
X_EVERY = 64
X_LEAD = 0.1
X_LAST = 0.95
GEN_GAP = 1
PW_GAP = 2
PW_SPLIT = 8
KEEP = 8
NG = 4
NA = 1
PA = 8
TAP_LAST = 0.8
GEN_LAG = 4
PW_LAG = 4
MIX_GAP = 1
MIX_LAG = 1
NU, NV = 10, 16
GS = 36
KS = 84
F32, BF16, U32 = jnp.float32, jnp.bfloat16, jnp.uint32

_BASES = [0, 1, 2, 3, 4, 5, 6, 7, 256, 258, 260, 262, 512, 516, 768, 772,
          1024, 1280, 1536, 1792]


_TAPS = {2: (2, 0, None), 3: (2, 0, 0),
         4: (3, 0, None), 5: (3, 0, None), 6: (3, T - 4, None), 7: (3, T - 4, 4)}
_TAPS.update({m: (4, (8 - m + m % 2) % T, 2 if m == NB - 1 else None) for m in range(8, NB)})
_SLOT = [0, 1, 2, 3] + [4 + (m - 4) // 2 for m in range(4, NB)]
_SHARE = [0, 0, 1, 2, 3, 4, 3, 4] + [5, 6] * 4


def _pack_rows(a):
    b = a.astype(np.float32).astype(BF16).view(np.uint16).astype(np.uint32)
    return b[..., 0::2, :] | (b[..., 1::2, :] << 16)


def _constants():
    om = 2.0 * np.pi * (np.arange(T) + 0.25) / T
    ph = np.exp(-1j * om[:, None] * np.arange(T)[None, :])
    fx = np.concatenate([ph.real, ph.imag], 0)
    g = np.stack([ph.real.T, ph.imag.T], -1).reshape(T, 2 * T) / T
    lag = np.arange(S).astype(np.float32).astype(BF16).astype(np.float32).astype(np.int64)
    lane = np.arange(T)
    off = 8 * (2 * (lane // 8) + lane % 2)
    tiles = [np.array(_BASES[4 * t:4 * t + 4])[(lane % 8) // 2] + off for t in range(5)]
    lo = lane < T // 2
    vals = [np.where(lo, tiles[0], np.roll(tiles[1], T // 2)),
            np.where(lo, np.roll(tiles[0], T // 2), tiles[1])]
    for m in range(2, NB):
        t, shift, end = _TAPS[m]
        v = np.roll(tiles[t], shift)
        vals.append(v if end is None else np.where(lane == end, (m + 1) * T, v))
    fk = np.zeros((max(_SHARE) + 1, 2 * T, T))
    for m in range(NB):
        blk = lag[m * T:(m + 1) * T]
        e = (blk[:, None] == vals[m][None, :]).astype(np.float64)
        assert (e.sum(1) == 1).all()
        c = np.concatenate([(ph @ e).real, (ph @ e).imag], 0)
        assert _SHARE.index(_SHARE[m]) == m or np.array_equal(fk[_SHARE[m]], c)
        fk[_SHARE[m]] = c
    g = np.stack([g[:, :T], g[:, T:]])
    return _pack_rows(fx), _pack_rows(g), _pack_rows(fk)


def _cmul(a, b):
    return a[0] * b[0] - a[1] * b[1], a[0] * b[1] + a[1] * b[0]


def _times(f, conj=False):
    dif, tot = f[1] - f[0], f[1] + f[0]

    def mul(a):
        k = f[0] * (a[0] + a[1])
        if conj:
            return k + a[1] * dif, k - a[0] * tot
        return k - a[1] * tot, k + a[0] * dif
    return mul


def _csq(a):
    t = a[0] * a[1]
    return a[0] * a[0] - a[1] * a[1], t + t


def _tree(op, xs):
    while len(xs) > 1:
        xs = [op(a, b) for a, b in zip(xs[0::2], xs[1::2])]
    return xs[0]


def _pack(a, b):
    return pltpu.pack_elementwise([a, b], packed_dtype=BF16)


def _words(a):
    return pltpu.bitcast(a.astype(BF16), U32)


def _halves(a):
    return pltpu.bitcast(a, BF16)


def _dot(a, b):
    return jnp.dot(a, b, preferred_element_type=F32)


def _dot_nt(a, b):
    return jax.lax.dot_general(a, b, (((1,), (1,)), ((), ())), preferred_element_type=F32)


def _sincos(x):
    k = jnp.floor(x * (2.0 / np.pi) + 0.5)
    r = ((x - k * 1.5703125) - k * 4.837512969970703125e-4) - k * 7.54978995489188216e-8
    z = r * r
    s = r + r * z * (-1.6666654611e-1 + z * (8.3321608736e-3 + z * -1.9515295891e-4))
    c = 1.0 + z * (-0.5 + z * (4.166664568298827e-2
                               + z * (-1.388731625493765e-3 + z * 2.443315711809948e-5)))
    n = k.astype(jnp.int32)
    odd = (n & 1) == 1
    s, c = jnp.where(odd, c, s), jnp.where(odd, s, c)
    return jnp.where((n & 2) == 2, -s, s), jnp.where(((n + 1) & 2) == 2, -c, c)


def _aligned(i, n):
    return i if isinstance(i, int) else pl.multiple_of(i, n)


def _loop(n, body):
    jax.lax.fori_loop(0, n, lambda i, c: body(i), None)


def _interleave(*streams):
    done = [0] * len(streams)
    live = list(range(len(streams)))
    while live:
        i = min(live, key=lambda n: streams[n][2]
                + (streams[n][3] - streams[n][2]) * done[n] / streams[n][1])
        work = next(streams[i][0], None)
        if work is None:
            live.remove(i)
        else:
            done[i] += work


def _chain(gens):
    for g in gens:
        yield from g


def _kernel(x_hbm, wqkv_hbm, wo_hbm, are_hbm, aim_hbm, bre_hbm, bim_hbm, cre_hbm, cim_hbm,
            ldt_hbm, dsk_hbm, gw_hbm, fx_hbm, g_hbm, fk_hbm, o_hbm,
            x_ref, wqkv_ref, wo_ref, ssm_ref, fx_ref, g_ref, fk_ref, o_ref,
            xs_s, gate_s, wt_s, wp_s, wop_s, par_s, us_s, vs_s, kend_s, ko_s, kt_s,
            kh_s, xh_s, yh_s, tmp_s, q_s, k_s, v_s, at_s, cur_s, zero_s, vec_s, ldt_in, dsk_in, gw_in,
            sems, xsems, osem):
    lane = jax.lax.broadcasted_iota(jnp.int32, (8, T), 1)
    lo = lane < T // 2

    ldt_ref, dsk_ref, gw_ref = vec_s.at[0], vec_s.at[1], vec_s.at[2]
    ssm_hbm = (are_hbm, aim_hbm, bre_hbm, bim_hbm, cre_hbm, cim_hbm)
    sem_ids = iter(range(N_COPIES))
    copy = lambda a, b: pltpu.make_async_copy(a, b, sems.at[next(sem_ids)])
    cp_ssm = [[copy(h.at[:, a:b], ssm_ref.at[i, :, a:b]) for i, h in enumerate(ssm_hbm)]
              for a, b in ((0, T), (T, 2 * T), (2 * T, D))]
    cp_fx = copy(fx_hbm, fx_ref)
    cp_vec = [copy(ldt_hbm, ldt_in), copy(dsk_hbm, dsk_in), copy(gw_hbm, gw_in)]

    def cp_x(i):
        rows = pl.ds(_aligned(i * (S // 4), S // 4), S // 4)
        return pltpu.make_async_copy(x_hbm.at[rows, :], x_ref.at[rows, :], xsems.at[i])
    cp_w = [copy(wqkv_hbm.at[:, s * D:(s + 1) * D], wqkv_ref.at[:, s * D:(s + 1) * D]) for s in range(3)]
    cp_fk = copy(fk_hbm, fk_ref)
    cp_out = [copy(wo_hbm, wo_ref), copy(g_hbm, g_ref)]
    for c in cp_vec + cp_ssm[0] + [cp_fx, cp_x(0)]:
        c.start()

    tokens, always = [], []

    def post(a, every):
        tokens[:] = tokens[-KEEP:] + [a[r - 8:r] for r in range(every, a.shape[0] + 1, every)]

    def pace(x):
        always[2] += 1
        if len(tokens) <= always[3] or always[2] < always[1]:
            return x
        always[2] = 0
        head = jnp.where(always[0], x[:8], pltpu.bitcast(tokens.pop(0), x.dtype))
        return head if x.shape[0] == 8 else jnp.concatenate([head, x[8:]], 0)

    def x_block(m):
        r0, h0 = _aligned(m * T, T), _aligned(m * (T // 2), T // 2)
        acc = None
        for t in range(NT):
            x = x_ref[pl.ds(r0, T), t * T:(t + 1) * T]
            xs_s[t, pl.ds(h0, T // 2), :] = pltpu.bitcast(x, U32)
            r = _dot(_halves(fx_ref[...]), x)
            xh_s[t, m] = r
            post(r, X_EVERY)
            xg = x.astype(F32) * gw_ref[:, t * T:(t + 1) * T]
            acc = xg if acc is None else acc + xg
            yield 1
        gate = jax.nn.sigmoid(jnp.sum(acc, axis=1, keepdims=True))
        gate_s[pl.ds(r0, T), :] = jnp.broadcast_to(gate, (T, T))

    def regroup(src, t):
        rows = []
        for i in range(2):
            w = src[pl.ds(2 * t + i, H, stride=DH // 2), :]
            w = pace(w) if i == 0 else w
            rows += [pltpu.unpack_elementwise(w, index=e, packed_dtype=BF16, unpacked_dtype=F32)
                     for e in range(2)]
        return _words(jnp.concatenate(rows, 0))

    def w_qkv(s):
        for c in range(NT):
            for kt in range(NT):
                w = wqkv_ref[kt * T:(kt + 1) * T, s * D + c * T:s * D + (c + 1) * T]
                wt_s[s, kt, c * (T // 2):(c + 1) * (T // 2), :] = pltpu.bitcast(w.T, U32)
                yield 1
        for t in range(NT):
            for kt in range(NT):
                wp_s[t, kt, s * (T // 2):(s + 1) * (T // 2), :] = regroup(wt_s.at[s, kt], t)
                yield 1

    def w_out():
        for ct in range(NT):
            wt_s[0, ct] = pltpu.bitcast(wo_ref[:, ct * T:(ct + 1) * T], U32)
            for t in range(NT):
                wop_s[ct, t * (T // 2):(t + 1) * (T // 2), :] = regroup(wt_s.at[0, ct], t)

    def put_par(i, a):
        par_s[i, 0:T, :] = a[0:T].T
        hi = a[T:N]
        par_s[i, T:N, :] = jnp.concatenate(
            [hi, pltpu.roll(hi, T // 2, 1)], 0).T[0:T // 2]

    def discretize(j):
        c0 = j * T if isinstance(j, int) else pl.multiple_of(j * T, T)
        dt = jnp.exp(ldt_ref[:, pl.ds(c0, T)].astype(F32)).astype(BF16).astype(F32)
        load = lambda i: ssm_ref[i, :, pl.ds(c0, T)].astype(F32)
        return dt, load, jnp.exp(dt * load(0)), dt * load(1)

    def prep(j):
        dt, load, mag, ang = discretize(j)
        sin, cos = _sincos(ang)
        w = _cmul((load(4), load(5)), (dt * load(2), dt * load(3)))
        for i, a in enumerate((mag * cos, mag * sin, w[0], -w[1])):
            put_par(i, a)
        return jnp.max(jnp.abs(ang))

    def prep_wide(j, ang_max):
        def redo(_):
            _, _, mag, ang = discretize(j)
            put_par(0, mag * jnp.cos(ang))
            put_par(1, mag * jnp.sin(ang))
        _loop(jnp.where(ang_max <= SINCOS_MAX, 0, 1), redo)

    GEN_STEPS = 28

    def gen(r, hi):
        r0 = r * 8 if isinstance(r, int) else pl.multiple_of(r * 8, 8)
        d0 = (r // 4) * GS + (r % 4) * 8
        s0 = T + r0 if hi else r0

        def put(dst, i, a, b):
            re, im = _pack(a[0], b[0]), _pack(a[1], b[1])
            if hi:
                t = pltpu.roll(jnp.where(lo, im, re), T // 2, 1)
                dst[2, pl.ds(i * 4 * GS + d0, 8), :] = jnp.where(lo, re, t)
                dst[2, pl.ds(i * 4 * GS + 2 * GS + d0, 8), :] = jnp.where(lo, t, im)
            else:
                dst[0, pl.ds(i * 4 * GS + d0, 8), :] = re
                dst[1, pl.ds(i * 4 * GS + d0, 8), :] = im

        p = (par_s[0, pl.ds(s0, 8), :], par_s[1, pl.ds(s0, 8), :])
        p2 = _csq(p)
        p4 = _csq(p2)
        q = _csq(p4)
        q2 = _csq(q)
        q4 = _csq(q2)
        yield 1
        v = [(jnp.ones_like(q[0]), jnp.zeros_like(q[0])), q, q2, _cmul(q, q2)]
        by_q4 = _times(q4)
        for i in range(NV // 2):
            put(vs_s, 2 * i, v[0], v[1])
            yield 1
            put(vs_s, 2 * i + 1, v[2], v[3])
            if i == 0:
                v = [q4] + [by_q4(a) for a in v[1:]]
            elif i < NV // 2 - 1:
                v = [by_q4((pace(v[0][0]), v[0][1]))] + [by_q4(a) for a in v[1:]]
            yield 1
        b1 = by_q4(v[0])
        u = [(par_s[2, pl.ds(s0, 8), :], par_s[3, pl.ds(s0, 8), :])]
        u += [_times(p, True)(u[0])]
        put(us_s, 0, u[0], u[1])
        yield 1
        fs, by = [p2, p4, b1], []
        for i, (a, b, f) in enumerate(((0, 1, 0), (0, 1, 1), (2, 3, 1), (0, 2, 2), (4, 6, 2),
                                       (0, 4, 3), (8, 10, 3), (0, 8, 4), (12, 14, 4))):
            if f == len(fs):
                fs.append(_csq(fs[-1]))
            if f == len(by):
                by.append(_times(fs[f], True))
            u += [by[f]((pace(u[a][0]), u[a][1])), by[f](u[b])]
            put(us_s, 1 + i, u[-2], u[-1])
            yield 1
        last = u[16][0] * fs[4][0] + u[16][1] * fs[4][1]
        if hi:
            kend_s[1, pl.ds(r0, 8), :] = jnp.where(lo, last, 0.0)
            kend_s[1, pl.ds(T // 2 + r0, 8), :] = jnp.where(lo, 0.0, last)
        else:
            kend_s[0, pl.ds(r0, 8), :] = last
        yield 1

    def kmat(g):
        u = jnp.concatenate([_halves(us_s[t, pl.ds(g, 4 * NU, stride=GS), :]) for t in range(3)], 1)
        v = jnp.concatenate([_halves(vs_s[t, pl.ds(g, 4 * NV, stride=GS), :]) for t in range(3)], 1)
        r = _dot_nt(u, v)
        ko_s[pl.ds(g * KS, 8 * NU), :] = r
        post(r, KMAT_EVERY)

    def taps(j):
        lane32 = jax.lax.broadcasted_iota(jnp.int32, (32, T), 1)
        slot = (lane32 % 8) // 2

        def gather(t):
            parts = []
            for c in range(4):
                acc = None
                for jj in range(4):
                    k = 4 * t + jj
                    a = ko_s[pl.ds((k // 2) * 8 + 2 * c + k % 2, 32, stride=KS), :]
                    if jj != c:
                        a = pltpu.roll(a, (2 * (jj - c)) % T, 1)
                    acc = a if acc is None else jnp.where(slot == jj, a, acc)
                parts.append(acc)
            return jnp.concatenate(parts, 0)

        def emit(ms, taps):
            kt_s[_SLOT[ms[0]]] = _words(taps)

        lane_t = jax.lax.broadcasted_iota(jnp.int32, (T, T), 1)
        lo_t, first = lane_t < T // 2, lane_t == 0
        t4 = gather(4)
        emit([8, 9], t4)
        for m in (10, 12):
            emit([m, m + 1], pltpu.roll(t4, _TAPS[m][1], 1))
        kend = jnp.sum(kend_s[0] + kend_s[1], axis=1, keepdims=True)
        emit([14, 15], jnp.where(lane_t == 2, kend, pltpu.roll(t4, _TAPS[14][1], 1)))
        yield 1
        t3 = gather(3)
        emit([4, 5], t3)
        emit([6, 7], jnp.where(lane_t == 4, pltpu.roll(t4, 4, 1), pltpu.roll(t3, _TAPS[6][1], 1)))
        yield 1
        t2 = gather(2)
        emit([2], t2)
        emit([3], jnp.where(first, t3, t2))
        yield 1
        t1 = gather(1)
        yield 1
        t0 = gather(0)
        x = pltpu.roll(jnp.where(lo_t, t1, t0), T // 2, 1)
        emit([1], jnp.where(lo_t, x, t1))
        skip = dsk_ref[:, pl.ds(j * T if isinstance(j, int) else pl.multiple_of(j * T, T), T)].astype(F32)
        skip = jnp.broadcast_to(skip, (T, T)).T
        emit([0], jnp.where(lo_t, t0, x) + jnp.where(first, skip, 0.0))
        yield 1

    def spectrum_k():
        for m in range(NB):
            r = _dot_nt(_halves(fk_ref[_SHARE[m]]), _halves(kt_s[_SLOT[m]]))
            kh_s[m] = r
            post(r, FK_EVERY)
            yield 64

    PW_STEPS = 3 * NB * (NB + 1) // 2

    def pointwise(j, i):
        r0 = _aligned(i * 8, 8)

        def part(ref, m, c):
            if c < 2:
                return ref[m, pl.ds(c * T + r0, 8), :]
            return part(ref, m, 0) + part(ref, m, 1)

        prev = None
        for c in range(3):
            for p0 in range(0, NB, PW_SPLIT):
                ps = range(p0, p0 + PW_SPLIT)
                xs, acc = {}, {}
                for m in range(p0 + PW_SPLIT):
                    k = part(kh_s, m, c)
                    if m % 2 == 0:
                        k = pace(k)
                    for p in ps:
                        if p >= m:
                            if p - m not in xs:
                                xs[p - m] = part(xh_s.at[j], p - m, c)
                            kx = k * xs[p - m]
                            acc[p] = kx + acc[p] if m else kx - tmp_s[p] if c == 2 else kx
                    yield min(p0 + PW_SPLIT - m, PW_SPLIT)
                for p in ps:
                    if c == 0:
                        tmp_s[p] = acc[p]
                    elif c == 1:
                        rr = tmp_s[p]
                        tmp_s[NB + p] = rr - acc[p]
                        tmp_s[p] = rr + acc[p]
                    else:
                        y = (tmp_s[NB + p], acc[p])
                        z = y if prev is None else (y[0] - prev[1], y[1] + prev[0])
                        yh_s[j, p, pl.ds(r0, 8), :] = _pack(*z)
                        prev = y

    qscale = float(DH ** -0.5 * np.log2(np.e))

    def qkv(j, i, every):
        r0, h0 = i * QR, i * (QR // 2)
        if not isinstance(i, int):
            r0, h0 = pl.multiple_of(r0, QR), pl.multiple_of(h0, QR // 2)
        for s in range(3):
            x = jnp.concatenate([_halves(xs_s[t, pl.ds(h0, QR // 2), :]) for t in range(NT)], 1)
            w = jnp.concatenate([_halves(wp_s[j, t, s * (T // 2):(s + 1) * (T // 2), :])
                                 for t in range(NT)], 1)
            acc = _dot_nt(x, w)
            if s == 0:
                q_s[j, pl.ds(r0, QR), :] = acc * qscale
            else:
                (k_s, v_s)[s - 1][j, pl.ds(HALO + r0, QR), :] = acc
            post(acc, every)
            yield QR * 5 // 4

    def window(r0, masked):
        qs = [q_s[t, pl.ds(r0, 8), :] for t in range(NT)]
        ls = []
        for w in range(WIN):
            a = None
            for t in range(NT):
                k = k_s[t, pl.ds(r0 + HALO - DIL * w, 8), :]
                kq = qs[t] * (pace(k) if t == 0 and w in PACE_K else k)
                a = kq if a is None else a + kq
            ls.append((a, pltpu.roll(a, 64, 1)))
        yield None
        ls = [a + b for a, b in ls]
        ls = [(a, pltpu.roll(a, 32, 1)) for a in ls]
        yield None
        ls = [a + b for a, b in ls]
        if masked:
            row = jax.lax.broadcasted_iota(jnp.int32, (8, T), 0) + r0
            ls = [jnp.where(row >= DIL * w, a, -1e9 * np.log2(np.e)) for w, a in enumerate(ls)]
        mx = _tree(jnp.maximum, ls)
        es = [jnp.exp2(a - mx) for a in ls]
        yield None
        inv = gate_s[pl.ds(r0, 8), :] * pl.reciprocal(_tree(jnp.add, es), full_range=False)
        outs = []
        for t in range(NT):
            a = None
            for w in range(WIN):
                v = v_s[t, pl.ds(r0 + HALO - DIL * w, 8), :]
                pv = es[w] * (pace(v) if w == 0 and t in PACE_V else v)
                a = pv if a is None else a + pv
            outs.append(a)
        yield [a * inv for a in outs]

    def attend(r0, n, first=False):
        gens = [window(r0 + 8 * c, first and 8 * c < HALO) for c in range(n)]
        for step in range(n + 3):
            for c in range(step, step - 4, -1):
                if 0 <= c < n:
                    out = next(gens[c])
                    if out is not None:
                        if c % 2:
                            h0 = r0 // 2 + (c // 2) * 8
                            h0 = h0 if isinstance(h0, int) else pl.multiple_of(h0, 8)
                            for t in range(NT):
                                at_s[t, pl.ds(h0, 8), :] = _words(jnp.concatenate([top[t], out[t]], 0))
                        top = out
            yield 1

    def stage(i):
        cur_s[...] = at_s[:, pl.ds(_aligned(i * (RB // 2), RB // 2), RB // 2), :]

    def out_copy(i):
        r0 = _aligned(i * RB, RB)
        return pltpu.make_async_copy(o_ref.at[pl.ds(r0, RB), :], o_hbm.at[pl.ds(r0, RB), :], osem)

    def mix(i):
        r0 = _aligned(i * RB, RB)
        for ct in range(NT):
            a = _dot(jnp.concatenate([_halves(cur_s[t]) for t in range(NT)], 1), _halves(wop_s[ct]))
            y = jnp.concatenate(
                [_dot(jnp.concatenate([_halves(g_ref[b]) for b in range(2)], 1),
                      _halves(yh_s[ct, i * (RB // T) + h])) for h in range(RB // T)], 0)
            acc = a + (1.0 - gate_s[pl.ds(r0, RB), :]) * y
            o_ref[pl.ds(r0, RB), ct * T:(ct + 1) * T] = acc.astype(BF16)
            post(acc, MIX_EVERY)
            yield 1

    def gen_streams(i0, n, serial):
        units = lambda i, u: [gen(4 * i + 2 * u, False), gen(4 * i + 2 * u + 1, False), gen(2 * i + u, True)]
        if serial:
            return [(_chain([g for i in range(n) for u in range(2) for g in units(i0 + i, u)]),
                     6 * n * GEN_STEPS, 0.0, 1.0)]
        return [(_chain([g for i in range(n) for g in units(i0 + i, u)]), 3 * n * GEN_STEPS, 0.0, 1.0)
                for u in range(2)]

    def qkvs(j, i0, n, every):
        return _chain([qkv(j, i0 + u, every) for u in range(n)])

    def kmats(g0, n):
        for u in range(n):
            kmat(g0 + u)
            yield 60

    def overlap(*streams, gap=1, lag=0):
        always[:] = [zero_s[...] == 0.0, gap, 0, lag]
        _interleave(*streams)
        tokens.clear()
        always.clear()

    for t in range(NT):
        k_s[t, 0:HALO, :] = jnp.zeros((HALO, T), F32)
        v_s[t, 0:HALO, :] = jnp.zeros((HALO, T), F32)
    zero_s[...] = jnp.zeros((8, T), F32)
    for c in cp_vec + cp_ssm[0]:
        c.wait()
    for i, ref in enumerate((ldt_in, dsk_in, gw_in)):
        vec_s[i] = ref[...].astype(F32).reshape(1, D)
    for i in range(1, 4):
        cp_x(i).start()
    prep_wide(0, prep(0))
    cp_fx.wait()

    def first(i):
        for when, cs in ((1, cp_w), (3, [cp_fk] + cp_ssm[1])):
            @pl.when(i == when)
            def _():
                for c in cs:
                    c.start()
        cp_x(i).wait()
        xs = (_chain([x_block(4 * i + u) for u in range(4)]), 4 * NT, X_LEAD, X_LAST)
        overlap(xs, *gen_streams(i, 1, X_SERIAL), gap=X_GAP, lag=X_LAG)
    _loop(4, first)
    for c in cp_ssm[2] + cp_out:
        c.start()
    for c in cp_w:
        c.wait()
    ws = (_chain([w_qkv(s) for s in range(3)]), 6 * NT * NT, 0.0, 1.0)
    overlap((kmats(0, 32), 1920, LEAD, LAST), ws, lag=PW_LAG)
    overlap((taps(0), 5, 0.0, 1.0))
    for c in [cp_fk] + cp_ssm[1]:
        c.wait()

    def pws(j, i0, n):
        return (_chain([pointwise(j, i0 + u) for u in range(n)]), n * PW_STEPS, 0.0, 1.0)

    nq, cq = S // QR, QR * 15 // 4

    def tile(j):
        @pl.when(j == 1)
        def _():
            for c in cp_ssm[2]:
                c.wait()
        overlap((spectrum_k(), 1024, 0.0, 1.0))
        prep_wide(j + 1, prep(j + 1))

        def expand(i):
            n = 4 // NG
            overlap((qkvs(j, i, 1, GEN_EVERY), cq, LEAD2, LAST2), *gen_streams(n * i, n, GEN_SERIAL), gap=GEN_GAP, lag=GEN_LAG)
        _loop(NG, expand)
        mxu = _chain([kmats(0, 32), qkvs(j, NG, NA, PW_EVERY)])
        overlap((mxu, 1920 + NA * cq, LEAD, LAST), pws(j, 0, PA), gap=PW_GAP, lag=PW_LAG)
        n = nq - NG - NA
        st = [(qkvs(j, NG + NA, n, PW_EVERY), n * cq, LEAD, LAST), pws(j, PA, 16 - PA)]
        overlap(*st, (taps(j + 1), 5, 0.0, TAP_LAST), gap=PW_GAP, lag=PW_LAG)
    _loop(NT - 1, tile)

    j = NT - 1
    for c in cp_out:
        c.wait()
    overlap((qkvs(j, 0, HEAD, QR), cq * HEAD, 0.0, 1.0))
    always[:] = [None, 1, 0, 0]
    w_out()
    overlap((spectrum_k(), 1024, LEAD, LAST), (attend(0, FIRST, True), FIRST + 3, 0.0, 1.0), lag=PW_LAG)
    n = (nq - HEAD) // NL

    def last_conv(i):
        r0 = pl.multiple_of(8 * (FIRST + i * EARLY), 16)
        st = [(qkvs(j, HEAD + n * i, n, PW_EVERY), cq * n, LEAD, LAST), pws(j, 16 // NL * i, 16 // NL)]
        overlap(*st, (attend(r0, EARLY), EARLY + 3, 0.0, 1.0), gap=PW_GAP, lag=PW_LAG)
    _loop(NL, last_conv)

    done, nr = FIRST + NL * EARLY, S // RB
    n_mixed = (S // 8 - done) // PER_ROW
    assert n * NL + HEAD == nq and done + n_mixed * PER_ROW == S // 8 and n_mixed < nr
    assert FIRST % 2 == EARLY % 2 == PER_ROW % 2 == 0
    assert all(8 * (FIRST + EARLY * (i + 1)) <= (HEAD + n * i) * QR for i in range(NL))
    assert all(8 * (done + PER_ROW * i) >= (i + 1) * RB for i in range(n_mixed + 1))
    stage(0)

    def rows(i, mixed):
        st = [(mix(i), NT, MIX_LEAD, MIX_LAST)]
        if mixed:
            r0 = pl.multiple_of(8 * (done + PER_ROW * i), 16)
            st.append((attend(r0, PER_ROW), PER_ROW + 3, 0.0, 1.0))
        overlap(*st, gap=MIX_GAP, lag=MIX_LAG)
        if mixed or n_mixed + 1 < nr:
            stage(jnp.minimum(i + 1, nr - 1))
        out_copy(i).start()
    _loop(n_mixed, lambda i: rows(i, True))
    _loop(nr - n_mixed, lambda i: rows(n_mixed + i, False))
    for i in range(nr):
        out_copy(i).wait()


@jax.jit
def pallas_gated_mix__sliding_local_dilated__ssm_conv_s4__prompt_kernel(
    A_x: jax.Array,
    A_wqkv: jax.Array,
    A_wo: jax.Array,
    B_u: jax.Array,
    B_A_re: jax.Array,
    B_A_im: jax.Array,
    B_B_re: jax.Array,
    B_B_im: jax.Array,
    B_C_re: jax.Array,
    B_C_im: jax.Array,
    B_log_dt: jax.Array,
    B_Dskip: jax.Array,
    gate_w: jax.Array,
):
    del B_u
    fx, g, fk = _constants()
    vm = pltpu.VMEM
    hbm = pl.BlockSpec(memory_space=pl.ANY)
    out = pl.pallas_call(
        _kernel,
        out_shape=jax.ShapeDtypeStruct((S, D), BF16),
        in_specs=[hbm] * 15,
        out_specs=hbm,
        scratch_shapes=[
            vm((S, D), BF16), vm((D, 3 * D), BF16), vm((D, D), BF16), vm((6, N, D), BF16),
            vm(fx.shape, U32), vm(g.shape, U32), vm(fk.shape, U32), vm((S, D), BF16),
            vm((NT, S // 2, T), U32), vm((S, T), F32),
            vm((3, NT, D // 2, T), U32), vm((NT, NT, 3 * T // 2, T), U32), vm((NT, D // 2, T), U32),
            vm((4, N, T), F32), vm((3, NU * 4 * GS, T), U32), vm((3, NV * 4 * GS, T), U32),
            vm((2, T, T), F32), vm((32 * KS, T), F32), vm((max(_SLOT) + 1, T // 2, T), U32),
            vm((NB, 2 * T, T), F32), vm((NT, NB, 2 * T, T), F32), vm((NT, NB, T, T), U32),
            vm((2 * NB, 8, T), F32),
            vm((NT, S, T), F32), vm((NT, S + HALO, T), F32), vm((NT, S + HALO, T), F32),
            vm((NT, S // 2, T), U32), vm((NT, RB // 2, T), U32), vm((8, T), F32),
            vm((3, 1, D), F32), vm((D,), BF16), vm((D,), BF16), vm((D,), BF16),
            pltpu.SemaphoreType.DMA((N_COPIES,)), pltpu.SemaphoreType.DMA((4,)),
             pltpu.SemaphoreType.DMA(()),
        ],
        compiler_params=pltpu.CompilerParams(vmem_limit_bytes=100 * 1024 * 1024),
    )(A_x.reshape(S, D), A_wqkv, A_wo, B_A_re.T, B_A_im.T, B_B_re.T, B_B_im.T, B_C_re.T, B_C_im.T,
      B_log_dt, B_Dskip, gate_w, fx, g, fk)
    return out.reshape(1, S, D)
```

```python
import jax
import jax.numpy as jnp
import numpy as np
import jax.experimental.pallas as pl
import jax.experimental.pallas.tpu as pltpu

S, D, H, DH, N = 2048, 640, 32, 20, 192
WIN, DIL = 8, 2
T = 128
NT = D // T
NB = S // T
HALO = 16
N_COPIES = 28
SINCOS_MAX = 8192.0
LEAD = 0.08
LEAD2 = 0.12
LAST = 0.95
LAST2 = 0.95
QR = 256
HEAD = 2
NL = 2
FIRST = 28
EARLY = 16
RB = 256
PER_ROW = 28
GEN_SERIAL = True
FK_EVERY = 256
KMAT_EVERY = 40
PW_EVERY = 16
GEN_EVERY = 8
MIX_EVERY = 64
MIX_LEAD = 0.05
MIX_LAST = 1.0
PACE_K = ()
PACE_V = (0,)
X_LAG = 8
X_SERIAL = True
X_GAP = 1
X_EVERY = 64
X_LEAD = 0.1
X_LAST = 0.95
GEN_GAP = 1
PW_GAP = 2
PW_SPLIT = 8
KEEP = 8
NG = 4
NA = 1
PA = 8
TAP_LAST = 0.8
GEN_LAG = 4
PW_LAG = 4
MIX_GAP = 1
MIX_LAG = 1
Y_AHEAD = 5
NU, NV = 10, 16
GS = 36
KS = 84
F32, BF16, U32 = jnp.float32, jnp.bfloat16, jnp.uint32

_BASES = [0, 1, 2, 3, 4, 5, 6, 7, 256, 258, 260, 262, 512, 516, 768, 772,
          1024, 1280, 1536, 1792]


_TAPS = {2: (2, 0, None), 3: (2, 0, 0),
         4: (3, 0, None), 5: (3, 0, None), 6: (3, T - 4, None), 7: (3, T - 4, 4)}
_TAPS.update({m: (4, (8 - m + m % 2) % T, 2 if m == NB - 1 else None) for m in range(8, NB)})
_SLOT = [0, 1, 2, 3] + [4 + (m - 4) // 2 for m in range(4, NB)]
_SHARE = [0, 0, 1, 2, 3, 4, 3, 4] + [5, 6] * 4


def _pack_rows(a):
    b = a.astype(np.float32).astype(BF16).view(np.uint16).astype(np.uint32)
    return b[..., 0::2, :] | (b[..., 1::2, :] << 16)


def _constants():
    om = 2.0 * np.pi * (np.arange(T) + 0.25) / T
    ph = np.exp(-1j * om[:, None] * np.arange(T)[None, :])
    fx = np.concatenate([ph.real, ph.imag], 0)
    g = np.stack([ph.real.T, ph.imag.T], -1).reshape(T, 2 * T) / T
    lag = np.arange(S).astype(np.float32).astype(BF16).astype(np.float32).astype(np.int64)
    lane = np.arange(T)
    off = 8 * (2 * (lane // 8) + lane % 2)
    tiles = [np.array(_BASES[4 * t:4 * t + 4])[(lane % 8) // 2] + off for t in range(5)]
    lo = lane < T // 2
    vals = [np.where(lo, tiles[0], np.roll(tiles[1], T // 2)),
            np.where(lo, np.roll(tiles[0], T // 2), tiles[1])]
    for m in range(2, NB):
        t, shift, end = _TAPS[m]
        v = np.roll(tiles[t], shift)
        vals.append(v if end is None else np.where(lane == end, (m + 1) * T, v))
    fk = np.zeros((max(_SHARE) + 1, 2 * T, T))
    for m in range(NB):
        blk = lag[m * T:(m + 1) * T]
        e = (blk[:, None] == vals[m][None, :]).astype(np.float64)
        assert (e.sum(1) == 1).all()
        c = np.concatenate([(ph @ e).real, (ph @ e).imag], 0)
        assert _SHARE.index(_SHARE[m]) == m or np.array_equal(fk[_SHARE[m]], c)
        fk[_SHARE[m]] = c
    g = np.stack([g[:, :T], g[:, T:]])
    return _pack_rows(fx), _pack_rows(g), _pack_rows(fk)


def _cmul(a, b):
    return a[0] * b[0] - a[1] * b[1], a[0] * b[1] + a[1] * b[0]


def _times(f, conj=False):
    dif, tot = f[1] - f[0], f[1] + f[0]

    def mul(a):
        k = f[0] * (a[0] + a[1])
        if conj:
            return k + a[1] * dif, k - a[0] * tot
        return k - a[1] * tot, k + a[0] * dif
    return mul


def _csq(a):
    t = a[0] * a[1]
    return a[0] * a[0] - a[1] * a[1], t + t


def _tree(op, xs):
    while len(xs) > 1:
        xs = [op(a, b) for a, b in zip(xs[0::2], xs[1::2])]
    return xs[0]


def _pack(a, b):
    return pltpu.pack_elementwise([a, b], packed_dtype=BF16)


def _words(a):
    return pltpu.bitcast(a.astype(BF16), U32)


def _halves(a):
    return pltpu.bitcast(a, BF16)


def _dot(a, b):
    return jnp.dot(a, b, preferred_element_type=F32)


def _dot_nt(a, b):
    return jax.lax.dot_general(a, b, (((1,), (1,)), ((), ())), preferred_element_type=F32)


def _sincos(x):
    k = jnp.floor(x * (2.0 / np.pi) + 0.5)
    r = ((x - k * 1.5703125) - k * 4.837512969970703125e-4) - k * 7.54978995489188216e-8
    z = r * r
    s = r + r * z * (-1.6666654611e-1 + z * (8.3321608736e-3 + z * -1.9515295891e-4))
    c = 1.0 + z * (-0.5 + z * (4.166664568298827e-2
                               + z * (-1.388731625493765e-3 + z * 2.443315711809948e-5)))
    n = k.astype(jnp.int32)
    odd = (n & 1) == 1
    s, c = jnp.where(odd, c, s), jnp.where(odd, s, c)
    return jnp.where((n & 2) == 2, -s, s), jnp.where(((n + 1) & 2) == 2, -c, c)


def _aligned(i, n):
    return i if isinstance(i, int) else pl.multiple_of(i, n)


def _loop(n, body):
    jax.lax.fori_loop(0, n, lambda i, c: body(i), None)


def _interleave(*streams):
    done = [0] * len(streams)
    live = list(range(len(streams)))
    while live:
        i = min(live, key=lambda n: streams[n][2]
                + (streams[n][3] - streams[n][2]) * done[n] / streams[n][1])
        work = next(streams[i][0], None)
        if work is None:
            live.remove(i)
        else:
            done[i] += work


def _chain(gens):
    for g in gens:
        yield from g


def _kernel(x_hbm, wqkv_hbm, wo_hbm, are_hbm, aim_hbm, bre_hbm, bim_hbm, cre_hbm, cim_hbm,
            ldt_hbm, dsk_hbm, gw_hbm, fx_hbm, g_hbm, fk_hbm, o_hbm,
            x_ref, wqkv_ref, wo_ref, ssm_ref, fx_ref, g_ref, fk_ref, o_ref,
            xs_s, gate_s, wt_s, wp_s, wop_s, par_s, us_s, vs_s, kend_s, ko_s, kt_s,
            kh_s, xh_s, yh_s, tmp_s, q_s, k_s, v_s, at_s, cur_s, y_s, zero_s, vec_s, ldt_in, dsk_in, gw_in,
            sems, xsems, osem):
    lane = jax.lax.broadcasted_iota(jnp.int32, (8, T), 1)
    lo = lane < T // 2

    ldt_ref, dsk_ref, gw_ref = vec_s.at[0], vec_s.at[1], vec_s.at[2]
    ssm_hbm = (are_hbm, aim_hbm, bre_hbm, bim_hbm, cre_hbm, cim_hbm)
    sem_ids = iter(range(N_COPIES))
    copy = lambda a, b: pltpu.make_async_copy(a, b, sems.at[next(sem_ids)])
    cp_ssm = [[copy(h.at[:, a:b], ssm_ref.at[i, :, a:b]) for i, h in enumerate(ssm_hbm)]
              for a, b in ((0, T), (T, 2 * T), (2 * T, D))]
    cp_fx = copy(fx_hbm, fx_ref)
    cp_vec = [copy(ldt_hbm, ldt_in), copy(dsk_hbm, dsk_in), copy(gw_hbm, gw_in)]

    def cp_x(i):
        rows = pl.ds(_aligned(i * (S // 4), S // 4), S // 4)
        return pltpu.make_async_copy(x_hbm.at[rows, :], x_ref.at[rows, :], xsems.at[i])
    cp_w = [copy(wqkv_hbm.at[:, s * D:(s + 1) * D], wqkv_ref.at[:, s * D:(s + 1) * D]) for s in range(3)]
    cp_fk = copy(fk_hbm, fk_ref)
    cp_out = [copy(wo_hbm, wo_ref), copy(g_hbm, g_ref)]
    for c in cp_vec + cp_ssm[0] + [cp_fx, cp_x(0), cp_x(1)]:
        c.start()

    tokens, always = [], []

    def post(a, every):
        tokens[:] = tokens[-KEEP:] + [a[r - 8:r] for r in range(every, a.shape[0] + 1, every)]

    def pace(x):
        always[2] += 1
        if len(tokens) <= always[3] or always[2] < always[1]:
            return x
        always[2] = 0
        head = jnp.where(always[0], x[:8], pltpu.bitcast(tokens.pop(0), x.dtype))
        return head if x.shape[0] == 8 else jnp.concatenate([head, x[8:]], 0)

    def x_block(m):
        r0, h0 = _aligned(m * T, T), _aligned(m * (T // 2), T // 2)
        acc = None
        for t in range(NT):
            x = x_ref[pl.ds(r0, T), t * T:(t + 1) * T]
            xs_s[t, pl.ds(h0, T // 2), :] = pltpu.bitcast(x, U32)
            r = _dot(_halves(fx_ref[...]), x)
            xh_s[t, m] = r
            post(r, X_EVERY)
            xg = x.astype(F32) * gw_ref[:, t * T:(t + 1) * T]
            acc = xg if acc is None else acc + xg
            yield 1
        gate = jax.nn.sigmoid(jnp.sum(acc, axis=1, keepdims=True))
        gate_s[pl.ds(r0, T), :] = jnp.broadcast_to(gate, (T, T))

    def regroup(src, t):
        rows = []
        for i in range(2):
            ab = [src[pl.ds(2 * t + i + h * DH // 2, H // 2, stride=DH), :] for h in range(2)]
            ab[0] = pace(ab[0]) if i == 0 else ab[0]
            rows += [_pack(*[pltpu.unpack_elementwise(w, index=e, packed_dtype=BF16, unpacked_dtype=F32)
                             for w in ab]) for e in range(2)]
        return jnp.concatenate(rows, 0)

    def w_qkv(s):
        for c in range(NT):
            for kt in range(NT):
                w = wqkv_ref[kt * T:(kt + 1) * T, s * D + c * T:s * D + (c + 1) * T]
                wt_s[s, kt, c * (T // 2):(c + 1) * (T // 2), :] = pltpu.bitcast(w.T, U32)
                yield 1
        for t in range(NT):
            for kt in range(NT):
                wp_s[t, kt, s * (T // 2):(s + 1) * (T // 2), :] = regroup(wt_s.at[s, kt], t)
                yield 1

    def w_out():
        for ct in range(NT):
            wt_s[0, ct] = pltpu.bitcast(wo_ref[:, ct * T:(ct + 1) * T], U32)
            for t in range(NT):
                wop_s[ct, t * (T // 2):(t + 1) * (T // 2), :] = regroup(wt_s.at[0, ct], t)
            yield 1

    def put_par(i, a):
        par_s[i, 0:T, :] = a[0:T].T
        hi = a[T:N]
        par_s[i, T:N, :] = jnp.concatenate(
            [hi, pltpu.roll(hi, T // 2, 1)], 0).T[0:T // 2]

    def discretize(j):
        c0 = j * T if isinstance(j, int) else pl.multiple_of(j * T, T)
        dt = jnp.exp(ldt_ref[:, pl.ds(c0, T)].astype(F32)).astype(BF16).astype(F32)
        load = lambda i: ssm_ref[i, :, pl.ds(c0, T)].astype(F32)
        return dt, load, jnp.exp(dt * load(0)), dt * load(1)

    def prep(j):
        dt, load, mag, ang = discretize(j)
        sin, cos = _sincos(ang)
        w = _cmul((load(4), load(5)), (dt * load(2), dt * load(3)))
        for i, a in enumerate((mag * cos, mag * sin, w[0], -w[1])):
            put_par(i, a)
        return jnp.max(jnp.abs(ang))

    def prep_wide(j, ang_max):
        def redo(_):
            _, _, mag, ang = discretize(j)
            put_par(0, mag * jnp.cos(ang))
            put_par(1, mag * jnp.sin(ang))
        _loop(jnp.where(ang_max <= SINCOS_MAX, 0, 1), redo)

    GEN_STEPS = 28

    def gen(r, hi):
        r0 = r * 8 if isinstance(r, int) else pl.multiple_of(r * 8, 8)
        d0 = (r // 4) * GS + (r % 4) * 8
        s0 = T + r0 if hi else r0

        def put(dst, i, a, b):
            re, im = _pack(a[0], b[0]), _pack(a[1], b[1])
            if hi:
                t = pltpu.roll(jnp.where(lo, im, re), T // 2, 1)
                dst[2, pl.ds(i * 4 * GS + d0, 8), :] = jnp.where(lo, re, t)
                dst[2, pl.ds(i * 4 * GS + 2 * GS + d0, 8), :] = jnp.where(lo, t, im)
            else:
                dst[0, pl.ds(i * 4 * GS + d0, 8), :] = re
                dst[1, pl.ds(i * 4 * GS + d0, 8), :] = im

        p = (par_s[0, pl.ds(s0, 8), :], par_s[1, pl.ds(s0, 8), :])
        p2 = _csq(p)
        p4 = _csq(p2)
        q = _csq(p4)
        q2 = _csq(q)
        q4 = _csq(q2)
        yield 1
        v = [(jnp.ones_like(q[0]), jnp.zeros_like(q[0])), q, q2, _cmul(q, q2)]
        by_q4 = _times(q4)
        for i in range(NV // 2):
            put(vs_s, 2 * i, v[0], v[1])
            yield 1
            put(vs_s, 2 * i + 1, v[2], v[3])
            if i == 0:
                v = [q4] + [by_q4(a) for a in v[1:]]
            elif i < NV // 2 - 1:
                v = [by_q4((pace(v[0][0]), v[0][1]))] + [by_q4(a) for a in v[1:]]
            yield 1
        b1 = by_q4(v[0])
        u = [(par_s[2, pl.ds(s0, 8), :], par_s[3, pl.ds(s0, 8), :])]
        u += [_times(p, True)(u[0])]
        put(us_s, 0, u[0], u[1])
        yield 1
        fs, by = [p2, p4, b1], []
        for i, (a, b, f) in enumerate(((0, 1, 0), (0, 1, 1), (2, 3, 1), (0, 2, 2), (4, 6, 2),
                                       (0, 4, 3), (8, 10, 3), (0, 8, 4), (12, 14, 4))):
            if f == len(fs):
                fs.append(_csq(fs[-1]))
            if f == len(by):
                by.append(_times(fs[f], True))
            u += [by[f]((pace(u[a][0]), u[a][1])), by[f](u[b])]
            put(us_s, 1 + i, u[-2], u[-1])
            yield 1
        last = u[16][0] * fs[4][0] + u[16][1] * fs[4][1]
        if hi:
            kend_s[1, pl.ds(r0, 8), :] = jnp.where(lo, last, 0.0)
            kend_s[1, pl.ds(T // 2 + r0, 8), :] = jnp.where(lo, 0.0, last)
        else:
            kend_s[0, pl.ds(r0, 8), :] = last
        yield 1

    def kmat(g):
        u = jnp.concatenate([_halves(us_s[t, pl.ds(g, 4 * NU, stride=GS), :]) for t in range(3)], 1)
        v = jnp.concatenate([_halves(vs_s[t, pl.ds(g, 4 * NV, stride=GS), :]) for t in range(3)], 1)
        r = _dot_nt(u, v)
        ko_s[pl.ds(g * KS, 8 * NU), :] = r
        post(r, KMAT_EVERY)

    def taps(j):
        lane32 = jax.lax.broadcasted_iota(jnp.int32, (32, T), 1)
        slot = (lane32 % 8) // 2

        def gather(t):
            parts = []
            for c in range(4):
                acc = None
                for jj in range(4):
                    k = 4 * t + jj
                    a = ko_s[pl.ds((k // 2) * 8 + 2 * c + k % 2, 32, stride=KS), :]
                    if jj != c:
                        a = pltpu.roll(a, (2 * (jj - c)) % T, 1)
                    acc = a if acc is None else jnp.where(slot == jj, a, acc)
                parts.append(acc)
            return jnp.concatenate(parts, 0)

        def emit(ms, taps):
            kt_s[_SLOT[ms[0]]] = _words(taps)

        lane_t = jax.lax.broadcasted_iota(jnp.int32, (T, T), 1)
        lo_t, first = lane_t < T // 2, lane_t == 0
        t4 = gather(4)
        emit([8, 9], t4)
        for m in (10, 12):
            emit([m, m + 1], pltpu.roll(t4, _TAPS[m][1], 1))
        kend = jnp.sum(kend_s[0] + kend_s[1], axis=1, keepdims=True)
        emit([14, 15], jnp.where(lane_t == 2, kend, pltpu.roll(t4, _TAPS[14][1], 1)))
        yield 1
        t3 = gather(3)
        emit([4, 5], t3)
        emit([6, 7], jnp.where(lane_t == 4, pltpu.roll(t4, 4, 1), pltpu.roll(t3, _TAPS[6][1], 1)))
        yield 1
        t2 = gather(2)
        emit([2], t2)
        emit([3], jnp.where(first, t3, t2))
        yield 1
        t1 = gather(1)
        yield 1
        t0 = gather(0)
        x = pltpu.roll(jnp.where(lo_t, t1, t0), T // 2, 1)
        emit([1], jnp.where(lo_t, x, t1))
        skip = dsk_ref[:, pl.ds(j * T if isinstance(j, int) else pl.multiple_of(j * T, T), T)].astype(F32)
        skip = jnp.broadcast_to(skip, (T, T)).T
        emit([0], jnp.where(lo_t, t0, x) + jnp.where(first, skip, 0.0))
        yield 1

    def spectrum_k():
        for m in range(NB):
            r = _dot_nt(_halves(fk_ref[_SHARE[m]]), _halves(kt_s[_SLOT[m]]))
            kh_s[m] = r
            post(r, FK_EVERY)
            yield 64

    PW_STEPS = 3 * NB * (NB + 1) // 2

    def pointwise(j, i):
        r0 = _aligned(i * 8, 8)

        def part(ref, m, c):
            if c < 2:
                return ref[m, pl.ds(c * T + r0, 8), :]
            return part(ref, m, 0) + part(ref, m, 1)

        prev = None
        for c in range(3):
            for p0 in range(0, NB, PW_SPLIT):
                ps = range(p0, p0 + PW_SPLIT)
                xs, acc = {}, {}
                for m in range(p0 + PW_SPLIT):
                    k = part(kh_s, m, c)
                    if m % 2 == 0:
                        k = pace(k)
                    for p in ps:
                        if p >= m:
                            if p - m not in xs:
                                xs[p - m] = part(xh_s.at[j], p - m, c)
                            kx = k * xs[p - m]
                            acc[p] = kx + acc[p] if m else kx - tmp_s[p] if c == 2 else kx
                    yield min(p0 + PW_SPLIT - m, PW_SPLIT)
                for p in ps:
                    if c == 0:
                        tmp_s[p] = acc[p]
                    elif c == 1:
                        rr = tmp_s[p]
                        tmp_s[NB + p] = rr - acc[p]
                        tmp_s[p] = rr + acc[p]
                    else:
                        y = (tmp_s[NB + p], acc[p])
                        z = y if prev is None else (y[0] - prev[1], y[1] + prev[0])
                        yh_s[j, p, pl.ds(r0, 8), :] = _pack(*z)
                        prev = y

    qscale = float(DH ** -0.5 * np.log2(np.e))

    def qkv(j, i, every):
        r0, h0 = i * QR, i * (QR // 2)
        if not isinstance(i, int):
            r0, h0 = pl.multiple_of(r0, QR), pl.multiple_of(h0, QR // 2)
        for s in range(3):
            x = jnp.concatenate([_halves(xs_s[t, pl.ds(h0, QR // 2), :]) for t in range(NT)], 1)
            w = jnp.concatenate([_halves(wp_s[j, t, s * (T // 2):(s + 1) * (T // 2), :])
                                 for t in range(NT)], 1)
            acc = _dot_nt(x, w)
            if s == 0:
                q_s[j, pl.ds(r0, QR), :] = acc * qscale
            else:
                (k_s, v_s)[s - 1][j, pl.ds(HALO + r0, QR), :] = acc
            post(acc, every)
            yield QR * 5 // 4

    def window(r0, masked):
        rows = lambda r: pl.ds(r, 8)
        qs = [q_s[t, rows(r0), :] for t in range(NT)]
        ls = []
        for w in range(WIN):
            a = None
            for t in range(NT):
                k = k_s[t, rows(r0 + HALO - DIL * w), :]
                kq = qs[t] * (pace(k) if t == 0 and w in PACE_K else k)
                a = kq if a is None else a + kq
            ls.append((a, pltpu.roll(a, 64, 1)))
        yield 1
        ls = [a + b for a, b in ls]
        ls = [(a, pltpu.roll(a, 32, 1)) for a in ls]
        yield 1
        ls = [a + b for a, b in ls]
        if masked:
            row = jax.lax.broadcasted_iota(jnp.int32, (8, T), 0) + r0
            ls = [jnp.where(row >= DIL * w, a, -1e9 * np.log2(np.e)) for w, a in enumerate(ls)]
        mx = _tree(jnp.maximum, ls)
        es = [jnp.exp2(a - mx) for a in ls]
        yield 1
        inv = gate_s[rows(r0), :] * pl.reciprocal(_tree(jnp.add, es), full_range=False)
        outs = []
        for t in range(NT):
            a = None
            for w in range(WIN):
                v = v_s[t, rows(r0 + HALO - DIL * w), :]
                pv = es[w] * (pace(v) if w == 0 and t in PACE_V else v)
                a = pv if a is None else a + pv
            outs.append(a)
        for t in range(NT):
            at_s[t, rows(r0), :] = outs[t] * inv
        yield 1

    def attend(r0, n, first=False):
        gens = [window(r0 + 8 * c, first and 8 * c < HALO) for c in range(n)]
        for step in range(n + 3):
            for c in range(step, step - 4, -1):
                if 0 <= c < n:
                    next(gens[c])
            yield 1

    def stage(i):
        r0 = _aligned(i * RB, RB)
        for t in range(NT):
            cur_s[t] = _pack(*[at_s[t, pl.ds(r0 + e, RB // 2, stride=2), :] for e in range(2)])

    def out_copy(i):
        r0 = _aligned(i * RB, RB)
        return pltpu.make_async_copy(o_ref.at[pl.ds(r0, RB), :], o_hbm.at[pl.ds(r0, RB), :], osem)

    def mix(i):
        r0 = _aligned(i * RB, RB)
        for ct in range(NT):
            for h in range(RB // T):
                y = _dot(jnp.concatenate([_halves(g_ref[b]) for b in range(2)], 1),
                         _halves(yh_s[ct, i * (RB // T) + h]))
                y_s[ct, h * T:(h + 1) * T, :] = (1.0 - gate_s[pl.ds(r0 + h * T, T), :]) * y
                post(y, T)
                yield 64
            if ct >= Y_AHEAD:
                yield from project(r0, ct - Y_AHEAD)
        for ct in range(NT - Y_AHEAD, NT):
            yield from project(r0, ct)

    def project(r0, ct):
        a = _dot(jnp.concatenate([_halves(cur_s[t]) for t in range(NT)], 1), _halves(wop_s[ct]))
        acc = a + y_s[ct]
        o_ref[pl.ds(r0, RB), ct * T:(ct + 1) * T] = acc.astype(BF16)
        post(acc, MIX_EVERY)
        yield RB * 5 // 4

    def gen_streams(i0, n, serial):
        units = lambda i, u: [gen(4 * i + 2 * u, False), gen(4 * i + 2 * u + 1, False), gen(2 * i + u, True)]
        if serial:
            return [(_chain([g for i in range(n) for u in range(2) for g in units(i0 + i, u)]),
                     6 * n * GEN_STEPS, 0.0, 1.0)]
        return [(_chain([g for i in range(n) for g in units(i0 + i, u)]), 3 * n * GEN_STEPS, 0.0, 1.0)
                for u in range(2)]

    def qkvs(j, i0, n, every):
        return _chain([qkv(j, i0 + u, every) for u in range(n)])

    def kmats(g0, n):
        for u in range(n):
            kmat(g0 + u)
            yield 60

    def overlap(*streams, gap=1, lag=0):
        always[:] = [zero_s[...] == 0.0, gap, 0, lag]
        _interleave(*streams)
        tokens.clear()
        always.clear()

    nq, cq = S // QR, QR * 15 // 4

    for t in range(NT):
        k_s[t, 0:HALO, :] = jnp.zeros((HALO, T), F32)
        v_s[t, 0:HALO, :] = jnp.zeros((HALO, T), F32)
    zero_s[...] = jnp.zeros((8, T), F32)
    for c in cp_vec + cp_ssm[0]:
        c.wait()
    for i, ref in enumerate((ldt_in, dsk_in, gw_in)):
        vec_s[i] = ref[...].astype(F32).reshape(1, D)
    prep_wide(0, prep(0))
    cp_fx.wait()

    def first(i):
        for when, cs in enumerate(([cp_x(2), cp_w[0]], [cp_x(3), cp_w[1]], cp_w[2:], [cp_fk] + cp_ssm[1])):
            @pl.when(i == when)
            def _():
                for c in cs:
                    c.start()
        cp_x(i).wait()
        xs = (_chain([x_block(4 * i + u) for u in range(4)]), 4 * NT, X_LEAD, X_LAST)
        overlap(xs, *gen_streams(i, 1, X_SERIAL), gap=X_GAP, lag=X_LAG)
    _loop(4, first)
    for c in cp_ssm[2] + cp_out:
        c.start()
    for c in cp_w:
        c.wait()
    ws = (_chain([w_qkv(s) for s in range(3)]), 6 * NT * NT, 0.0, 1.0)
    overlap((kmats(0, 32), 1920, LEAD, LAST), ws, lag=PW_LAG)
    overlap((qkv(0, 0, QR), cq, 0.0, 1.0), (taps(0), 5, 0.0, 1.0))
    for c in [cp_fk] + cp_ssm[1]:
        c.wait()

    def pws(j, i0, n):
        return (_chain([pointwise(j, i0 + u) for u in range(n)]), n * PW_STEPS, 0.0, 1.0)

    def tile(j):
        @pl.when(j == 1)
        def _():
            for c in cp_ssm[2]:
                c.wait()
        overlap((spectrum_k(), 1024, 0.0, 1.0))
        prep_wide(j + 1, prep(j + 1))

        def expand(i):
            n = 4 // NG
            overlap((qkvs(j, i + 1, 1, GEN_EVERY), cq, LEAD2, LAST2), *gen_streams(n * i, n, GEN_SERIAL), gap=GEN_GAP, lag=GEN_LAG)
        _loop(NG, expand)
        mxu = _chain([kmats(0, 32), qkvs(j, NG + 1, NA, PW_EVERY)])
        overlap((mxu, 1920 + NA * cq, LEAD, LAST), pws(j, 0, PA), gap=PW_GAP, lag=PW_LAG)
        n = nq - NG - NA
        mxu = _chain([qkvs(j, NG + NA + 1, n - 1, PW_EVERY), qkv(j + 1, 0, PW_EVERY)])
        st = [(mxu, n * cq, LEAD, LAST), pws(j, PA, 16 - PA)]
        overlap(*st, (taps(j + 1), 5, 0.0, TAP_LAST), gap=PW_GAP, lag=PW_LAG)
    _loop(NT - 1, tile)

    j = NT - 1
    for c in cp_out:
        c.wait()
    mxu = _chain([spectrum_k(), qkvs(j, 1, HEAD - 1, 64)])
    st = [(mxu, 1024 + cq * (HEAD - 1), LEAD, LAST), (attend(0, FIRST, True), FIRST + 3, 0.0, 1.0)]
    overlap(*st, (w_out(), NT, 0.0, 1.0), lag=PW_LAG)
    n = (nq - HEAD) // NL

    def last_conv(i):
        r0 = pl.multiple_of(8 * (FIRST + i * EARLY), 16)
        st = [(qkvs(j, HEAD + n * i, n, PW_EVERY), cq * n, LEAD, LAST), pws(j, 16 // NL * i, 16 // NL)]
        overlap(*st, (attend(r0, EARLY), EARLY + 3, 0.0, 1.0), gap=PW_GAP, lag=PW_LAG)
    _loop(NL, last_conv)

    done, nr = FIRST + NL * EARLY, S // RB
    n_mixed = (S // 8 - done) // PER_ROW
    assert n * NL + HEAD == nq and done + n_mixed * PER_ROW == S // 8 and n_mixed < nr
    assert 8 * FIRST <= QR and FIRST % 2 == EARLY % 2 == PER_ROW % 2 == 0
    assert all(8 * (FIRST + EARLY * (i + 1)) <= (HEAD + n * i) * QR for i in range(NL))
    assert all(8 * (done + PER_ROW * i) >= (i + 1) * RB for i in range(n_mixed + 1))
    stage(0)

    def rows(i, mixed):
        st = [(mix(i), NT * RB * 7 // 4, MIX_LEAD, MIX_LAST)]
        if mixed:
            r0 = pl.multiple_of(8 * (done + PER_ROW * i), 16)
            st.append((attend(r0, PER_ROW), PER_ROW + 3, 0.0, 1.0))
        overlap(*st, gap=MIX_GAP, lag=MIX_LAG)
        if mixed or n_mixed + 1 < nr:
            stage(jnp.minimum(i + 1, nr - 1))
        out_copy(i).start()
    _loop(n_mixed, lambda i: rows(i, True))
    _loop(nr - n_mixed, lambda i: rows(n_mixed + i, False))
    for i in range(nr):
        out_copy(i).wait()


@jax.jit
def pallas_gated_mix__sliding_local_dilated__ssm_conv_s4__prompt_kernel(
    A_x: jax.Array,
    A_wqkv: jax.Array,
    A_wo: jax.Array,
    B_u: jax.Array,
    B_A_re: jax.Array,
    B_A_im: jax.Array,
    B_B_re: jax.Array,
    B_B_im: jax.Array,
    B_C_re: jax.Array,
    B_C_im: jax.Array,
    B_log_dt: jax.Array,
    B_Dskip: jax.Array,
    gate_w: jax.Array,
):
    del B_u
    fx, g, fk = _constants()
    vm = pltpu.VMEM
    hbm = pl.BlockSpec(memory_space=pl.ANY)
    out = pl.pallas_call(
        _kernel,
        out_shape=jax.ShapeDtypeStruct((S, D), BF16),
        in_specs=[hbm] * 15,
        out_specs=hbm,
        scratch_shapes=[
            vm((S, D), BF16), vm((D, 3 * D), BF16), vm((D, D), BF16), vm((6, N, D), BF16),
            vm(fx.shape, U32), vm(g.shape, U32), vm(fk.shape, U32), vm((S, D), BF16),
            vm((NT, S // 2, T), U32), vm((S, T), F32),
            vm((3, NT, D // 2, T), U32), vm((NT, NT, 3 * T // 2, T), U32), vm((NT, D // 2, T), U32),
            vm((4, N, T), F32), vm((3, NU * 4 * GS, T), U32), vm((3, NV * 4 * GS, T), U32),
            vm((2, T, T), F32), vm((32 * KS, T), F32), vm((max(_SLOT) + 1, T // 2, T), U32),
            vm((NB, 2 * T, T), F32), vm((NT, NB, 2 * T, T), F32), vm((NT, NB, T, T), U32),
            vm((2 * NB, 8, T), F32),
            vm((NT, S, T), F32), vm((NT, S + HALO, T), F32), vm((NT, S + HALO, T), F32),
            vm((NT, S, T), F32), vm((NT, RB // 2, T), U32), vm((NT, RB, T), F32), vm((8, T), F32),
            vm((3, 1, D), F32), vm((D,), BF16), vm((D,), BF16), vm((D,), BF16),
            pltpu.SemaphoreType.DMA((N_COPIES,)), pltpu.SemaphoreType.DMA((4,)),
             pltpu.SemaphoreType.DMA(()),
        ],
        compiler_params=pltpu.CompilerParams(vmem_limit_bytes=100 * 1024 * 1024),
    )(A_x.reshape(S, D), A_wqkv, A_wo, B_A_re.T, B_A_im.T, B_B_re.T, B_B_im.T, B_C_re.T, B_C_im.T,
      B_log_dt, B_Dskip, gate_w, fx, g, fk)
    return out.reshape(1, S, D)
```

```python
import jax
import jax.numpy as jnp
import numpy as np
import jax.experimental.pallas as pl
import jax.experimental.pallas.tpu as pltpu

S, D, H, DH, N = 2048, 640, 32, 20, 192
WIN, DIL = 8, 2
T = 128
NT = D // T
NB = S // T
HALO = 16
N_COPIES = 28
SINCOS_MAX = 8192.0
LEAD = 0.08
LEAD2 = 0.12
LAST = 0.95
LAST2 = 0.95
QR = 256
HEAD = 2
NL = 2
FIRST = 28
EARLY = 16
RB = 256
PER_ROW = 28
GEN_SERIAL = True
FK_EVERY = 256
KMAT_EVERY = 40
PW_EVERY = 16
GEN_EVERY = 8
MIX_EVERY = 64
MIX_LEAD = 0.05
MIX_LAST = 1.0
PACE_K = ()
PACE_V = (0,)
X_LAG = 8
X_SERIAL = True
X_GAP = 1
X_EVERY = 64
X_LEAD = 0.1
X_LAST = 0.95
GEN_GAP = 1
PW_GAP = 2
PW_SPLIT = 8
KEEP = 8
NG = 4
NA = 1
PA = 8
TAP_LAST = 0.8
GEN_LAG = 4
PW_LAG = 4
MIX_GAP = 1
MIX_LAG = 1
IM = 144
SPEC = 280
QPAD = 0
KPAD = 0
VPAD = 0
XPAD = 0
WPAD = 0
UPAD = 0
Y_AHEAD = 5
NU, NV = 10, 16
GS = 36
KS = 84
F32, BF16, U32 = jnp.float32, jnp.bfloat16, jnp.uint32

_BASES = [0, 1, 2, 3, 4, 5, 6, 7, 256, 258, 260, 262, 512, 516, 768, 772,
          1024, 1280, 1536, 1792]


_TAPS = {2: (2, 0, None), 3: (2, 0, 0),
         4: (3, 0, None), 5: (3, 0, None), 6: (3, T - 4, None), 7: (3, T - 4, 4)}
_TAPS.update({m: (4, (8 - m + m % 2) % T, 2 if m == NB - 1 else None) for m in range(8, NB)})
_SLOT = [0, 1, 2, 3] + [4 + (m - 4) // 2 for m in range(4, NB)]
_SHARE = [0, 0, 1, 2, 3, 4, 3, 4] + [5, 6] * 4


def _pack_rows(a):
    b = a.astype(np.float32).astype(BF16).view(np.uint16).astype(np.uint32)
    return b[..., 0::2, :] | (b[..., 1::2, :] << 16)


def _constants():
    om = 2.0 * np.pi * (np.arange(T) + 0.25) / T
    ph = np.exp(-1j * om[:, None] * np.arange(T)[None, :])
    fx = np.concatenate([ph.real, ph.imag], 0)
    g = np.stack([ph.real.T, ph.imag.T], -1).reshape(T, 2 * T) / T
    lag = np.arange(S).astype(np.float32).astype(BF16).astype(np.float32).astype(np.int64)
    lane = np.arange(T)
    off = 8 * (2 * (lane // 8) + lane % 2)
    tiles = [np.array(_BASES[4 * t:4 * t + 4])[(lane % 8) // 2] + off for t in range(5)]
    lo = lane < T // 2
    vals = [np.where(lo, tiles[0], np.roll(tiles[1], T // 2)),
            np.where(lo, np.roll(tiles[0], T // 2), tiles[1])]
    for m in range(2, NB):
        t, shift, end = _TAPS[m]
        v = np.roll(tiles[t], shift)
        vals.append(v if end is None else np.where(lane == end, (m + 1) * T, v))
    fk = np.zeros((max(_SHARE) + 1, 2 * T, T))
    for m in range(NB):
        blk = lag[m * T:(m + 1) * T]
        e = (blk[:, None] == vals[m][None, :]).astype(np.float64)
        assert (e.sum(1) == 1).all()
        c = np.concatenate([(ph @ e).real, (ph @ e).imag], 0)
        assert _SHARE.index(_SHARE[m]) == m or np.array_equal(fk[_SHARE[m]], c)
        fk[_SHARE[m]] = c
    g = np.stack([g[:, :T], g[:, T:]])
    return _pack_rows(fx), _pack_rows(g), _pack_rows(fk)


def _cmul(a, b):
    return a[0] * b[0] - a[1] * b[1], a[0] * b[1] + a[1] * b[0]


def _times(f, conj=False):
    dif, tot = f[1] - f[0], f[1] + f[0]

    def mul(a):
        k = f[0] * (a[0] + a[1])
        if conj:
            return k + a[1] * dif, k - a[0] * tot
        return k - a[1] * tot, k + a[0] * dif
    return mul


def _csq(a):
    t = a[0] * a[1]
    return a[0] * a[0] - a[1] * a[1], t + t


def _tree(op, xs):
    while len(xs) > 1:
        xs = [op(a, b) for a, b in zip(xs[0::2], xs[1::2])]
    return xs[0]


def _pack(a, b):
    return pltpu.pack_elementwise([a, b], packed_dtype=BF16)


def _words(a):
    return pltpu.bitcast(a.astype(BF16), U32)


def _halves(a):
    return pltpu.bitcast(a, BF16)


def _dot(a, b):
    return jnp.dot(a, b, preferred_element_type=F32)


def _dot_nt(a, b):
    return jax.lax.dot_general(a, b, (((1,), (1,)), ((), ())), preferred_element_type=F32)


def _sincos(x):
    k = jnp.floor(x * (2.0 / np.pi) + 0.5)
    r = ((x - k * 1.5703125) - k * 4.837512969970703125e-4) - k * 7.54978995489188216e-8
    z = r * r
    s = r + r * z * (-1.6666654611e-1 + z * (8.3321608736e-3 + z * -1.9515295891e-4))
    c = 1.0 + z * (-0.5 + z * (4.166664568298827e-2
                               + z * (-1.388731625493765e-3 + z * 2.443315711809948e-5)))
    n = k.astype(jnp.int32)
    odd = (n & 1) == 1
    s, c = jnp.where(odd, c, s), jnp.where(odd, s, c)
    return jnp.where((n & 2) == 2, -s, s), jnp.where(((n + 1) & 2) == 2, -c, c)


def _aligned(i, n):
    return i if isinstance(i, int) else pl.multiple_of(i, n)


def _loop(n, body):
    jax.lax.fori_loop(0, n, lambda i, c: body(i), None)


def _interleave(*streams):
    done = [0] * len(streams)
    live = list(range(len(streams)))
    while live:
        i = min(live, key=lambda n: streams[n][2]
                + (streams[n][3] - streams[n][2]) * done[n] / streams[n][1])
        work = next(streams[i][0], None)
        if work is None:
            live.remove(i)
        else:
            done[i] += work


def _chain(gens):
    for g in gens:
        yield from g


def _kernel(x_hbm, wqkv_hbm, wo_hbm, are_hbm, aim_hbm, bre_hbm, bim_hbm, cre_hbm, cim_hbm,
            ldt_hbm, dsk_hbm, gw_hbm, fx_hbm, g_hbm, fk_hbm, o_hbm,
            x_ref, wqkv_ref, wo_ref, ssm_ref, fx_ref, g_ref, fk_ref, o_ref,
            xs_s, gate_s, wt_s, wp_s, wop_s, par_s, us_s, vs_s, kend_s, ko_s, kt_s,
            kh_s, xh_s, yh_s, tmp_s, q_s, k_s, v_s, at_s, cur_s, y_s, zero_s, vec_s, ldt_in, dsk_in, gw_in,
            sems, xsems, osem):
    lane = jax.lax.broadcasted_iota(jnp.int32, (8, T), 1)
    lo = lane < T // 2

    ldt_ref, dsk_ref, gw_ref = vec_s.at[0], vec_s.at[1], vec_s.at[2]
    ssm_hbm = (are_hbm, aim_hbm, bre_hbm, bim_hbm, cre_hbm, cim_hbm)
    sem_ids = iter(range(N_COPIES))
    copy = lambda a, b: pltpu.make_async_copy(a, b, sems.at[next(sem_ids)])
    cp_ssm = [[copy(h.at[:, a:b], ssm_ref.at[i, :, a:b]) for i, h in enumerate(ssm_hbm)]
              for a, b in ((0, T), (T, 2 * T), (2 * T, D))]
    cp_fx = copy(fx_hbm, fx_ref)
    cp_vec = [copy(ldt_hbm, ldt_in), copy(dsk_hbm, dsk_in), copy(gw_hbm, gw_in)]

    def cp_x(i):
        rows = pl.ds(_aligned(i * (S // 4), S // 4), S // 4)
        return pltpu.make_async_copy(x_hbm.at[rows, :], x_ref.at[rows, :], xsems.at[i])
    cp_w = [copy(wqkv_hbm.at[:, s * D:(s + 1) * D], wqkv_ref.at[:, s * D:(s + 1) * D]) for s in range(3)]
    cp_fk = copy(fk_hbm, fk_ref)
    cp_out = [copy(wo_hbm, wo_ref), copy(g_hbm, g_ref)]
    for c in cp_vec + cp_ssm[0] + [cp_fx, cp_x(0), cp_x(1)]:
        c.start()

    tokens, always = [], []

    def post(a, every):
        tokens[:] = tokens[-KEEP:] + [a[r - 8:r] for r in range(every, a.shape[0] + 1, every)]

    def pace(x):
        always[2] += 1
        if len(tokens) <= always[3] or always[2] < always[1]:
            return x
        always[2] = 0
        head = jnp.where(always[0], x[:8], pltpu.bitcast(tokens.pop(0), x.dtype))
        return head if x.shape[0] == 8 else jnp.concatenate([head, x[8:]], 0)

    def x_block(m):
        r0, h0 = _aligned(m * T, T), _aligned(m * (T // 2), T // 2)
        acc = None
        for t in range(NT):
            x = x_ref[pl.ds(r0, T), t * T:(t + 1) * T]
            xs_s[t, pl.ds(h0, T // 2), :] = pltpu.bitcast(x, U32)
            r = _dot(_halves(fx_ref[...]), x)
            xh_s[t, m, 0:T, :] = r[:T]
            xh_s[t, m, IM:IM + T, :] = r[T:]
            post(r, X_EVERY)
            xg = x.astype(F32) * gw_ref[:, t * T:(t + 1) * T]
            acc = xg if acc is None else acc + xg
            yield 1
        gate = jax.nn.sigmoid(jnp.sum(acc, axis=1, keepdims=True))
        gate_s[pl.ds(r0, T), :] = jnp.broadcast_to(gate, (T, T))

    def regroup(src, t):
        rows = []
        for i in range(2):
            ab = [src[pl.ds(2 * t + i + h * DH // 2, H // 2, stride=DH), :] for h in range(2)]
            ab[0] = pace(ab[0]) if i == 0 else ab[0]
            rows += [_pack(*[pltpu.unpack_elementwise(w, index=e, packed_dtype=BF16, unpacked_dtype=F32)
                             for w in ab]) for e in range(2)]
        return jnp.concatenate(rows, 0)

    def w_qkv(s):
        for c in range(NT):
            for kt in range(NT):
                w = wqkv_ref[kt * T:(kt + 1) * T, s * D + c * T:s * D + (c + 1) * T]
                wt_s[s, kt, c * (T // 2):(c + 1) * (T // 2), :] = pltpu.bitcast(w.T, U32)
                yield 1
        for t in range(NT):
            for kt in range(NT):
                wp_s[t, kt, s * (T // 2):(s + 1) * (T // 2), :] = regroup(wt_s.at[s, kt], t)
                yield 1

    def w_out():
        for ct in range(NT):
            wt_s[0, ct] = pltpu.bitcast(wo_ref[:, ct * T:(ct + 1) * T], U32)
            for t in range(NT):
                wop_s[ct, t * (T // 2):(t + 1) * (T // 2), :] = regroup(wt_s.at[0, ct], t)
            yield 1

    def put_par(i, a):
        par_s[i, 0:T, :] = a[0:T].T
        hi = a[T:N]
        par_s[i, T:N, :] = jnp.concatenate(
            [hi, pltpu.roll(hi, T // 2, 1)], 0).T[0:T // 2]

    def discretize(j):
        c0 = j * T if isinstance(j, int) else pl.multiple_of(j * T, T)
        dt = jnp.exp(ldt_ref[:, pl.ds(c0, T)].astype(F32)).astype(BF16).astype(F32)
        load = lambda i: ssm_ref[i, :, pl.ds(c0, T)].astype(F32)
        return dt, load, jnp.exp(dt * load(0)), dt * load(1)

    def prep(j):
        dt, load, mag, ang = discretize(j)
        sin, cos = _sincos(ang)
        w = _cmul((load(4), load(5)), (dt * load(2), dt * load(3)))
        for i, a in enumerate((mag * cos, mag * sin, w[0], -w[1])):
            put_par(i, a)
        return jnp.max(jnp.abs(ang))

    def prep_wide(j, ang_max):
        def redo(_):
            _, _, mag, ang = discretize(j)
            put_par(0, mag * jnp.cos(ang))
            put_par(1, mag * jnp.sin(ang))
        _loop(jnp.where(ang_max <= SINCOS_MAX, 0, 1), redo)

    GEN_STEPS = 28

    def gen(r, hi):
        r0 = r * 8 if isinstance(r, int) else pl.multiple_of(r * 8, 8)
        d0 = (r // 4) * GS + (r % 4) * 8
        s0 = T + r0 if hi else r0

        def put(dst, i, a, b):
            re, im = _pack(a[0], b[0]), _pack(a[1], b[1])
            if hi:
                t = pltpu.roll(jnp.where(lo, im, re), T // 2, 1)
                dst[2, pl.ds(i * 4 * GS + d0, 8), :] = jnp.where(lo, re, t)
                dst[2, pl.ds(i * 4 * GS + 2 * GS + d0, 8), :] = jnp.where(lo, t, im)
            else:
                dst[0, pl.ds(i * 4 * GS + d0, 8), :] = re
                dst[1, pl.ds(i * 4 * GS + d0, 8), :] = im

        p = (par_s[0, pl.ds(s0, 8), :], par_s[1, pl.ds(s0, 8), :])
        p2 = _csq(p)
        p4 = _csq(p2)
        q = _csq(p4)
        q2 = _csq(q)
        q4 = _csq(q2)
        yield 1
        v = [(jnp.ones_like(q[0]), jnp.zeros_like(q[0])), q, q2, _cmul(q, q2)]
        by_q4 = _times(q4)
        for i in range(NV // 2):
            put(vs_s, 2 * i, v[0], v[1])
            yield 1
            put(vs_s, 2 * i + 1, v[2], v[3])
            if i == 0:
                v = [q4] + [by_q4(a) for a in v[1:]]
            elif i < NV // 2 - 1:
                v = [by_q4((pace(v[0][0]), v[0][1]))] + [by_q4(a) for a in v[1:]]
            yield 1
        b1 = by_q4(v[0])
        u = [(par_s[2, pl.ds(s0, 8), :], par_s[3, pl.ds(s0, 8), :])]
        u += [_times(p, True)(u[0])]
        put(us_s, 0, u[0], u[1])
        yield 1
        fs, by = [p2, p4, b1], []
        for i, (a, b, f) in enumerate(((0, 1, 0), (0, 1, 1), (2, 3, 1), (0, 2, 2), (4, 6, 2),
                                       (0, 4, 3), (8, 10, 3), (0, 8, 4), (12, 14, 4))):
            if f == len(fs):
                fs.append(_csq(fs[-1]))
            if f == len(by):
                by.append(_times(fs[f], True))
            u += [by[f]((pace(u[a][0]), u[a][1])), by[f](u[b])]
            put(us_s, 1 + i, u[-2], u[-1])
            yield 1
        last = u[16][0] * fs[4][0] + u[16][1] * fs[4][1]
        if hi:
            kend_s[1, pl.ds(r0, 8), :] = jnp.where(lo, last, 0.0)
            kend_s[1, pl.ds(T // 2 + r0, 8), :] = jnp.where(lo, 0.0, last)
        else:
            kend_s[0, pl.ds(r0, 8), :] = last
        yield 1

    def kmat(g):
        u = jnp.concatenate([_halves(us_s[t, pl.ds(g, 4 * NU, stride=GS), :]) for t in range(3)], 1)
        v = jnp.concatenate([_halves(vs_s[t, pl.ds(g, 4 * NV, stride=GS), :]) for t in range(3)], 1)
        r = _dot_nt(u, v)
        ko_s[pl.ds(g * KS, 8 * NU), :] = r
        post(r, KMAT_EVERY)

    def taps(j):
        lane32 = jax.lax.broadcasted_iota(jnp.int32, (32, T), 1)
        slot = (lane32 % 8) // 2

        def gather(t):
            parts = []
            for c in range(4):
                acc = None
                for jj in range(4):
                    k = 4 * t + jj
                    a = ko_s[pl.ds((k // 2) * 8 + 2 * c + k % 2, 32, stride=KS), :]
                    if jj != c:
                        a = pltpu.roll(a, (2 * (jj - c)) % T, 1)
                    acc = a if acc is None else jnp.where(slot == jj, a, acc)
                parts.append(acc)
            return jnp.concatenate(parts, 0)

        def emit(ms, taps):
            kt_s[_SLOT[ms[0]]] = _words(taps)

        lane_t = jax.lax.broadcasted_iota(jnp.int32, (T, T), 1)
        lo_t, first = lane_t < T // 2, lane_t == 0
        t4 = gather(4)
        emit([8, 9], t4)
        for m in (10, 12):
            emit([m, m + 1], pltpu.roll(t4, _TAPS[m][1], 1))
        kend = jnp.sum(kend_s[0] + kend_s[1], axis=1, keepdims=True)
        emit([14, 15], jnp.where(lane_t == 2, kend, pltpu.roll(t4, _TAPS[14][1], 1)))
        yield 1
        t3 = gather(3)
        emit([4, 5], t3)
        emit([6, 7], jnp.where(lane_t == 4, pltpu.roll(t4, 4, 1), pltpu.roll(t3, _TAPS[6][1], 1)))
        yield 1
        t2 = gather(2)
        emit([2], t2)
        emit([3], jnp.where(first, t3, t2))
        yield 1
        t1 = gather(1)
        yield 1
        t0 = gather(0)
        x = pltpu.roll(jnp.where(lo_t, t1, t0), T // 2, 1)
        emit([1], jnp.where(lo_t, x, t1))
        skip = dsk_ref[:, pl.ds(j * T if isinstance(j, int) else pl.multiple_of(j * T, T), T)].astype(F32)
        skip = jnp.broadcast_to(skip, (T, T)).T
        emit([0], jnp.where(lo_t, t0, x) + jnp.where(first, skip, 0.0))
        yield 1

    def spectrum_k():
        for m in range(NB):
            r = _dot_nt(_halves(fk_ref[_SHARE[m]]), _halves(kt_s[_SLOT[m]]))
            kh_s[m, 0:T, :] = r[:T]
            kh_s[m, IM:IM + T, :] = r[T:]
            post(r, FK_EVERY)
            yield 64

    PW_STEPS = 3 * NB * (NB + 1) // 2

    def pointwise(j, i):
        r0 = _aligned(i * 8, 8)

        def part(ref, m, c):
            if c < 2:
                return ref[m, pl.ds(c * IM + r0, 8), :]
            return part(ref, m, 0) + part(ref, m, 1)

        prev = None
        for c in range(3):
            for p0 in range(0, NB, PW_SPLIT):
                ps = range(p0, p0 + PW_SPLIT)
                xs, acc = {}, {}
                for m in range(p0 + PW_SPLIT):
                    k = part(kh_s, m, c)
                    if m % 2 == 0:
                        k = pace(k)
                    for p in ps:
                        if p >= m:
                            if p - m not in xs:
                                xs[p - m] = part(xh_s.at[j], p - m, c)
                            kx = k * xs[p - m]
                            acc[p] = kx + acc[p] if m else kx - tmp_s[p] if c == 2 else kx
                    yield min(p0 + PW_SPLIT - m, PW_SPLIT)
                for p in ps:
                    if c == 0:
                        tmp_s[p] = acc[p]
                    elif c == 1:
                        rr = tmp_s[p]
                        tmp_s[NB + p] = rr - acc[p]
                        tmp_s[p] = rr + acc[p]
                    else:
                        y = (tmp_s[NB + p], acc[p])
                        z = y if prev is None else (y[0] - prev[1], y[1] + prev[0])
                        yh_s[j, p, pl.ds(r0, 8), :] = _pack(*z)
                        prev = y

    qscale = float(DH ** -0.5 * np.log2(np.e))

    def qkv(j, i, every):
        r0, h0 = i * QR, i * (QR // 2)
        if not isinstance(i, int):
            r0, h0 = pl.multiple_of(r0, QR), pl.multiple_of(h0, QR // 2)
        for s in range(3):
            x = jnp.concatenate([_halves(xs_s[t, pl.ds(h0, QR // 2), :]) for t in range(NT)], 1)
            w = jnp.concatenate([_halves(wp_s[j, t, s * (T // 2):(s + 1) * (T // 2), :])
                                 for t in range(NT)], 1)
            acc = _dot_nt(x, w)
            if s == 0:
                q_s[j, pl.ds(r0, QR), :] = acc * qscale
            else:
                (k_s, v_s)[s - 1][j, pl.ds(HALO + r0, QR), :] = acc
            post(acc, every)
            yield QR * 5 // 4

    def window(r0, masked):
        rows = lambda r: pl.ds(r, 8)
        qs = [q_s[t, rows(r0), :] for t in range(NT)]
        ls = []
        for w in range(WIN):
            a = None
            for t in range(NT):
                k = k_s[t, rows(r0 + HALO - DIL * w), :]
                kq = qs[t] * (pace(k) if t == 0 and w in PACE_K else k)
                a = kq if a is None else a + kq
            ls.append((a, pltpu.roll(a, 64, 1)))
        yield 1
        ls = [a + b for a, b in ls]
        ls = [(a, pltpu.roll(a, 32, 1)) for a in ls]
        yield 1
        ls = [a + b for a, b in ls]
        if masked:
            row = jax.lax.broadcasted_iota(jnp.int32, (8, T), 0) + r0
            ls = [jnp.where(row >= DIL * w, a, -1e9 * np.log2(np.e)) for w, a in enumerate(ls)]
        mx = _tree(jnp.maximum, ls)
        es = [jnp.exp2(a - mx) for a in ls]
        yield 1
        inv = gate_s[rows(r0), :] * pl.reciprocal(_tree(jnp.add, es), full_range=False)
        outs = []
        for t in range(NT):
            a = None
            for w in range(WIN):
                v = v_s[t, rows(r0 + HALO - DIL * w), :]
                pv = es[w] * (pace(v) if w == 0 and t in PACE_V else v)
                a = pv if a is None else a + pv
            outs.append(a)
        for t in range(NT):
            at_s[t, rows(r0), :] = outs[t] * inv
        yield 1

    def attend(r0, n, first=False):
        gens = [window(r0 + 8 * c, first and 8 * c < HALO) for c in range(n)]
        for step in range(n + 3):
            for c in range(step, step - 4, -1):
                if 0 <= c < n:
                    next(gens[c])
            yield 1

    def stage(i):
        r0 = _aligned(i * RB, RB)
        for t in range(NT):
            cur_s[t] = _pack(*[at_s[t, pl.ds(r0 + e, RB // 2, stride=2), :] for e in range(2)])

    def out_copy(i):
        r0 = _aligned(i * RB, RB)
        return pltpu.make_async_copy(o_ref.at[pl.ds(r0, RB), :], o_hbm.at[pl.ds(r0, RB), :], osem)

    def mix(i):
        r0 = _aligned(i * RB, RB)
        for ct in range(NT):
            for h in range(RB // T):
                y = _dot(jnp.concatenate([_halves(g_ref[b]) for b in range(2)], 1),
                         _halves(yh_s[ct, i * (RB // T) + h]))
                y_s[ct, h * T:(h + 1) * T, :] = (1.0 - gate_s[pl.ds(r0 + h * T, T), :]) * y
                post(y, T)
                yield 64
            if ct >= Y_AHEAD:
                yield from project(r0, ct - Y_AHEAD)
        for ct in range(NT - Y_AHEAD, NT):
            yield from project(r0, ct)

    def project(r0, ct):
        a = _dot(jnp.concatenate([_halves(cur_s[t]) for t in range(NT)], 1), _halves(wop_s[ct]))
        acc = a + y_s[ct]
        o_ref[pl.ds(r0, RB), ct * T:(ct + 1) * T] = acc.astype(BF16)
        post(acc, MIX_EVERY)
        yield RB * 5 // 4

    def gen_streams(i0, n, serial):
        units = lambda i, u: [gen(4 * i + 2 * u, False), gen(4 * i + 2 * u + 1, False), gen(2 * i + u, True)]
        if serial:
            return [(_chain([g for i in range(n) for u in range(2) for g in units(i0 + i, u)]),
                     6 * n * GEN_STEPS, 0.0, 1.0)]
        return [(_chain([g for i in range(n) for g in units(i0 + i, u)]), 3 * n * GEN_STEPS, 0.0, 1.0)
                for u in range(2)]

    def qkvs(j, i0, n, every):
        return _chain([qkv(j, i0 + u, every) for u in range(n)])

    def kmats(g0, n):
        for u in range(n):
            kmat(g0 + u)
            yield 60

    def overlap(*streams, gap=1, lag=0):
        always[:] = [zero_s[...] == 0.0, gap, 0, lag]
        _interleave(*streams)
        tokens.clear()
        always.clear()

    nq, cq = S // QR, QR * 15 // 4

    for t in range(NT):
        k_s[t, 0:HALO, :] = jnp.zeros((HALO, T), F32)
        v_s[t, 0:HALO, :] = jnp.zeros((HALO, T), F32)
    zero_s[...] = jnp.zeros((8, T), F32)
    for c in cp_vec + cp_ssm[0]:
        c.wait()
    for i, ref in enumerate((ldt_in, dsk_in, gw_in)):
        vec_s[i] = ref[...].astype(F32).reshape(1, D)
    prep_wide(0, prep(0))
    cp_fx.wait()

    def first(i):
        for when, cs in enumerate(([cp_x(2), cp_w[0]], [cp_x(3), cp_w[1]], cp_w[2:], [cp_fk] + cp_ssm[1])):
            @pl.when(i == when)
            def _():
                for c in cs:
                    c.start()
        cp_x(i).wait()
        xs = (_chain([x_block(4 * i + u) for u in range(4)]), 4 * NT, X_LEAD, X_LAST)
        overlap(xs, *gen_streams(i, 1, X_SERIAL), gap=X_GAP, lag=X_LAG)
    _loop(4, first)
    for c in cp_ssm[2] + cp_out:
        c.start()
    for c in cp_w:
        c.wait()
    ws = (_chain([w_qkv(s) for s in range(3)]), 6 * NT * NT, 0.0, 1.0)
    overlap((kmats(0, 32), 1920, LEAD, LAST), ws, lag=PW_LAG)
    overlap((qkv(0, 0, QR), cq, 0.0, 1.0), (taps(0), 5, 0.0, 1.0))
    for c in [cp_fk] + cp_ssm[1]:
        c.wait()

    def pws(j, i0, n):
        return (_chain([pointwise(j, i0 + u) for u in range(n)]), n * PW_STEPS, 0.0, 1.0)

    def tile(j):
        @pl.when(j == 1)
        def _():
            for c in cp_ssm[2]:
                c.wait()
        overlap((spectrum_k(), 1024, 0.0, 1.0))
        prep_wide(j + 1, prep(j + 1))

        def expand(i):
            n = 4 // NG
            overlap((qkvs(j, i + 1, 1, GEN_EVERY), cq, LEAD2, LAST2), *gen_streams(n * i, n, GEN_SERIAL), gap=GEN_GAP, lag=GEN_LAG)
        _loop(NG, expand)
        mxu = _chain([kmats(0, 32), qkvs(j, NG + 1, NA, PW_EVERY)])
        overlap((mxu, 1920 + NA * cq, LEAD, LAST), pws(j, 0, PA), gap=PW_GAP, lag=PW_LAG)
        n = nq - NG - NA
        mxu = _chain([qkvs(j, NG + NA + 1, n - 1, PW_EVERY), qkv(j + 1, 0, PW_EVERY)])
        st = [(mxu, n * cq, LEAD, LAST), pws(j, PA, 16 - PA)]
        overlap(*st, (taps(j + 1), 5, 0.0, TAP_LAST), gap=PW_GAP, lag=PW_LAG)
    _loop(NT - 1, tile)

    j = NT - 1
    for c in cp_out:
        c.wait()
    mxu = _chain([spectrum_k(), qkvs(j, 1, HEAD - 1, 64)])
    st = [(mxu, 1024 + cq * (HEAD - 1), LEAD, LAST), (attend(0, FIRST, True), FIRST + 3, 0.0, 1.0)]
    overlap(*st, (w_out(), NT, 0.0, 1.0), lag=PW_LAG)
    n = (nq - HEAD) // NL

    def last_conv(i):
        r0 = pl.multiple_of(8 * (FIRST + i * EARLY), 16)
        st = [(qkvs(j, HEAD + n * i, n, PW_EVERY), cq * n, LEAD, LAST), pws(j, 16 // NL * i, 16 // NL)]
        overlap(*st, (attend(r0, EARLY), EARLY + 3, 0.0, 1.0), gap=PW_GAP, lag=PW_LAG)
    _loop(NL, last_conv)

    done, nr = FIRST + NL * EARLY, S // RB
    n_mixed = (S // 8 - done) // PER_ROW
    assert n * NL + HEAD == nq and done + n_mixed * PER_ROW == S // 8 and n_mixed < nr
    assert 8 * FIRST <= QR and FIRST % 2 == EARLY % 2 == PER_ROW % 2 == 0
    assert all(8 * (FIRST + EARLY * (i + 1)) <= (HEAD + n * i) * QR for i in range(NL))
    assert all(8 * (done + PER_ROW * i) >= (i + 1) * RB for i in range(n_mixed + 1))
    stage(0)

    def rows(i, mixed):
        st = [(mix(i), NT * RB * 7 // 4, MIX_LEAD, MIX_LAST)]
        if mixed:
            r0 = pl.multiple_of(8 * (done + PER_ROW * i), 16)
            st.append((attend(r0, PER_ROW), PER_ROW + 3, 0.0, 1.0))
        overlap(*st, gap=MIX_GAP, lag=MIX_LAG)
        if mixed or n_mixed + 1 < nr:
            stage(jnp.minimum(i + 1, nr - 1))
        out_copy(i).start()
    _loop(n_mixed, lambda i: rows(i, True))
    _loop(nr - n_mixed, lambda i: rows(n_mixed + i, False))
    for i in range(nr):
        out_copy(i).wait()


@jax.jit
def pallas_gated_mix__sliding_local_dilated__ssm_conv_s4__prompt_kernel(
    A_x: jax.Array,
    A_wqkv: jax.Array,
    A_wo: jax.Array,
    B_u: jax.Array,
    B_A_re: jax.Array,
    B_A_im: jax.Array,
    B_B_re: jax.Array,
    B_B_im: jax.Array,
    B_C_re: jax.Array,
    B_C_im: jax.Array,
    B_log_dt: jax.Array,
    B_Dskip: jax.Array,
    gate_w: jax.Array,
):
    del B_u
    fx, g, fk = _constants()
    vm = pltpu.VMEM
    hbm = pl.BlockSpec(memory_space=pl.ANY)
    out = pl.pallas_call(
        _kernel,
        out_shape=jax.ShapeDtypeStruct((S, D), BF16),
        in_specs=[hbm] * 15,
        out_specs=hbm,
        scratch_shapes=[
            vm((S, D), BF16), vm((D, 3 * D), BF16), vm((D, D), BF16), vm((6, N, D), BF16),
            vm(fx.shape, U32), vm(g.shape, U32), vm(fk.shape, U32), vm((S, D), BF16),
            vm((NT, S // 2 + XPAD, T), U32), vm((S, T), F32),
            vm((3, NT, D // 2, T), U32), vm((NT, NT, 3 * T // 2 + WPAD, T), U32), vm((NT, D // 2, T), U32),
            vm((4, N, T), F32), vm((3, NU * 4 * GS + UPAD, T), U32), vm((3, NV * 4 * GS + UPAD, T), U32),
            vm((2, T, T), F32), vm((32 * KS, T), F32), vm((max(_SLOT) + 1, T // 2, T), U32),
            vm((NB, SPEC, T), F32), vm((NT, NB, SPEC, T), F32), vm((NT, NB, T, T), U32),
            vm((2 * NB, 8, T), F32),
            vm((NT, S + QPAD, T), F32), vm((NT, S + HALO + KPAD, T), F32), vm((NT, S + HALO + VPAD, T), F32),
            vm((NT, S, T), F32), vm((NT, RB // 2, T), U32), vm((NT, RB, T), F32), vm((8, T), F32),
            vm((3, 1, D), F32), vm((D,), BF16), vm((D,), BF16), vm((D,), BF16),
            pltpu.SemaphoreType.DMA((N_COPIES,)), pltpu.SemaphoreType.DMA((4,)),
             pltpu.SemaphoreType.DMA(()),
        ],
        compiler_params=pltpu.CompilerParams(vmem_limit_bytes=100 * 1024 * 1024),
    )(A_x.reshape(S, D), A_wqkv, A_wo, B_A_re.T, B_A_im.T, B_B_re.T, B_B_im.T, B_C_re.T, B_C_im.T,
      B_log_dt, B_Dskip, gate_w, fx, g, fk)
    return out.reshape(1, S, D)
```

```python
import jax
import jax.numpy as jnp
import numpy as np
import jax.experimental.pallas as pl
import jax.experimental.pallas.tpu as pltpu

S, D, H, DH, N = 2048, 640, 32, 20, 192
WIN, DIL = 8, 2
T = 128
NT = D // T
NB = S // T
HALO = 32
N_COPIES = 28
SINCOS_MAX = 8192.0
LEAD = 0.04
LEAD2 = 0.03
LAST = 0.98
LAST2 = 0.98
QR = 256
HEAD = 2
NL = 2
FIRST = 28
EARLY = 16
RB = 256
PER_ROW = 28
GEN_SERIAL = True
FK_EVERY = 256
KMAT_EVERY = 40
PW_EVERY = 16
GEN_EVERY = 16
MIX_EVERY = 64
MIX_LEAD = 0.05
MIX_LAST = 1.0
PACE_K = ()
PACE_V = (0,)
X_LAG = 8
X_SERIAL = True
X_GAP = 1
X_EVERY = 64
X_LEAD = 0.1
X_LAST = 0.95
GEN_GAP = 2
PW_GAP = 2
PW_SPLIT = 8
KEEP = 16
NG = 1
NA = 1
PA = 8
TAP_LAST = 0.8
GEN_LAG = 3
PW_LAG = 4
IM = 144
SPEC = 280
NU, NV = 10, 16
GS = 36
KS = 84
F32, BF16, U32 = jnp.float32, jnp.bfloat16, jnp.uint32

_BASES = [0, 1, 2, 3, 4, 5, 6, 7, 256, 258, 260, 262, 512, 516, 768, 772,
          1024, 1280, 1536, 1792]


_TAPS = {2: (2, 0, None), 3: (2, 0, 0),
         4: (3, 0, None), 5: (3, 0, None), 6: (3, T - 4, None), 7: (3, T - 4, 4)}
_TAPS.update({m: (4, (8 - m + m % 2) % T, 2 if m == NB - 1 else None) for m in range(8, NB)})
_SLOT = [0, 1, 2, 3] + [4 + (m - 4) // 2 for m in range(4, NB)]
_SHARE = [0, 0, 1, 2, 3, 4, 3, 4] + [5, 6] * 4


def _pack_rows(a):
    b = a.astype(np.float32).astype(BF16).view(np.uint16).astype(np.uint32)
    return b[..., 0::2, :] | (b[..., 1::2, :] << 16)


def _constants():
    om = 2.0 * np.pi * (np.arange(T) + 0.25) / T
    ph = np.exp(-1j * om[:, None] * np.arange(T)[None, :])
    fx = np.concatenate([ph.real, ph.imag], 0)
    g = np.stack([ph.real.T, ph.imag.T], -1).reshape(T, 2 * T) / T
    lag = np.arange(S).astype(np.float32).astype(BF16).astype(np.float32).astype(np.int64)
    lane = np.arange(T)
    off = 8 * (2 * (lane // 8) + lane % 2)
    tiles = [np.array(_BASES[4 * t:4 * t + 4])[(lane % 8) // 2] + off for t in range(5)]
    lo = lane < T // 2
    vals = [np.where(lo, tiles[0], np.roll(tiles[1], T // 2)),
            np.where(lo, np.roll(tiles[0], T // 2), tiles[1])]
    for m in range(2, NB):
        t, shift, end = _TAPS[m]
        v = np.roll(tiles[t], shift)
        vals.append(v if end is None else np.where(lane == end, (m + 1) * T, v))
    fk = np.zeros((max(_SHARE) + 1, 2 * T, T))
    for m in range(NB):
        blk = lag[m * T:(m + 1) * T]
        e = (blk[:, None] == vals[m][None, :]).astype(np.float64)
        assert (e.sum(1) == 1).all()
        c = np.concatenate([(ph @ e).real, (ph @ e).imag], 0)
        assert _SHARE.index(_SHARE[m]) == m or np.array_equal(fk[_SHARE[m]], c)
        fk[_SHARE[m]] = c
    g = np.stack([g[:, :T], g[:, T:]])
    return _pack_rows(fx), _pack_rows(g), _pack_rows(fk)


def _cmul(a, b):
    return a[0] * b[0] - a[1] * b[1], a[0] * b[1] + a[1] * b[0]


def _times(f, conj=False):
    dif, tot = f[1] - f[0], f[1] + f[0]

    def mul(a):
        k = f[0] * (a[0] + a[1])
        if conj:
            return k + a[1] * dif, k - a[0] * tot
        return k - a[1] * tot, k + a[0] * dif
    return mul


def _csq(a):
    t = a[0] * a[1]
    return a[0] * a[0] - a[1] * a[1], t + t


def _tree(op, xs):
    while len(xs) > 1:
        xs = [op(a, b) for a, b in zip(xs[0::2], xs[1::2])]
    return xs[0]


def _pack(a, b):
    return pltpu.pack_elementwise([a, b], packed_dtype=BF16)


def _words(a):
    return pltpu.bitcast(a.astype(BF16), U32)


def _halves(a):
    return pltpu.bitcast(a, BF16)


def _dot(a, b):
    return jnp.dot(a, b, preferred_element_type=F32)


def _dot_nt(a, b):
    return jax.lax.dot_general(a, b, (((1,), (1,)), ((), ())), preferred_element_type=F32)


def _sincos(x):
    k = jnp.floor(x * (2.0 / np.pi) + 0.5)
    r = ((x - k * 1.5703125) - k * 4.837512969970703125e-4) - k * 7.54978995489188216e-8
    z = r * r
    s = r + r * z * (-1.6666654611e-1 + z * (8.3321608736e-3 + z * -1.9515295891e-4))
    c = 1.0 + z * (-0.5 + z * (4.166664568298827e-2
                               + z * (-1.388731625493765e-3 + z * 2.443315711809948e-5)))
    n = k.astype(jnp.int32)
    odd = (n & 1) == 1
    s, c = jnp.where(odd, c, s), jnp.where(odd, s, c)
    return jnp.where((n & 2) == 2, -s, s), jnp.where(((n + 1) & 2) == 2, -c, c)


def _aligned(i, n):
    return i if isinstance(i, int) else pl.multiple_of(i, n)


def _loop(n, body):
    jax.lax.fori_loop(0, n, lambda i, c: body(i), None)


def _interleave(*streams):
    done = [0] * len(streams)
    live = list(range(len(streams)))
    while live:
        i = min(live, key=lambda n: streams[n][2]
                + (streams[n][3] - streams[n][2]) * done[n] / streams[n][1])
        work = next(streams[i][0], None)
        if work is None:
            live.remove(i)
        else:
            done[i] += work


def _chain(gens):
    for g in gens:
        yield from g


def _kernel(x_hbm, wqkv_hbm, wo_hbm, are_hbm, aim_hbm, bre_hbm, bim_hbm, cre_hbm, cim_hbm,
            ldt_hbm, dsk_hbm, gw_hbm, fx_hbm, g_hbm, fk_hbm, o_hbm,
            x_ref, wqkv_ref, wo_ref, ssm_ref, fx_ref, g_ref, fk_ref, o_ref,
            xs_s, gate_s, wt_s, wp_s, wop_s, par_s, us_s, vs_s, kend_s, ko_s, kt_s,
            kh_s, xh_s, yh_s, tmp_s, q_s, k_s, v_s, at_s, cur_s, y_s, zero_s, vec_s, ldt_in, dsk_in, gw_in,
            sems, xsems, osem):
    lane = jax.lax.broadcasted_iota(jnp.int32, (8, T), 1)
    lo = lane < T // 2

    ldt_ref, dsk_ref, gw_ref = vec_s.at[0], vec_s.at[1], vec_s.at[2]
    ssm_hbm = (are_hbm, aim_hbm, bre_hbm, bim_hbm, cre_hbm, cim_hbm)
    sem_ids = iter(range(N_COPIES))
    copy = lambda a, b: pltpu.make_async_copy(a, b, sems.at[next(sem_ids)])
    cp_ssm = [[copy(h.at[:, a:b], ssm_ref.at[i, :, a:b]) for i, h in enumerate(ssm_hbm)]
              for a, b in ((0, T), (T, 2 * T), (2 * T, D))]
    cp_fx = copy(fx_hbm, fx_ref)
    cp_vec = [copy(ldt_hbm, ldt_in), copy(dsk_hbm, dsk_in), copy(gw_hbm, gw_in)]

    def cp_x(i):
        rows = pl.ds(_aligned(i * (S // 4), S // 4), S // 4)
        return pltpu.make_async_copy(x_hbm.at[rows, :], x_ref.at[rows, :], xsems.at[i])
    cp_w = [copy(wqkv_hbm.at[:, s * D:(s + 1) * D], wqkv_ref.at[:, s * D:(s + 1) * D]) for s in range(3)]
    cp_fk = copy(fk_hbm, fk_ref)
    cp_out = [copy(wo_hbm, wo_ref), copy(g_hbm, g_ref)]
    for c in cp_vec + cp_ssm[0] + [cp_fx, cp_x(0), cp_x(1)]:
        c.start()

    tokens, always = [], []

    def post(a, every):
        tokens[:] = tokens[-KEEP:] + [a[r - 8:r] for r in range(every, a.shape[0] + 1, every)]

    def pace(x):
        always[2] += 1
        if len(tokens) <= always[3] or always[2] < always[1]:
            return x
        always[2] = 0
        head = jnp.where(always[0], x[:8], pltpu.bitcast(tokens.pop(0), x.dtype))
        return head if x.shape[0] == 8 else jnp.concatenate([head, x[8:]], 0)

    def x_block(m):
        r0, h0 = _aligned(m * T, T), _aligned(m * (T // 2), T // 2)
        acc = None
        for t in range(NT):
            x = x_ref[pl.ds(r0, T), t * T:(t + 1) * T]
            xs_s[t, pl.ds(h0, T // 2), :] = pltpu.bitcast(x, U32)
            r = _dot(_halves(fx_ref[...]), x)
            xh_s[t, m, 0:T, :] = r[:T]
            xh_s[t, m, IM:IM + T, :] = r[T:]
            post(r, X_EVERY)
            xg = x.astype(F32) * gw_ref[:, t * T:(t + 1) * T]
            acc = xg if acc is None else acc + xg
            yield 1
        gate = jax.nn.sigmoid(jnp.sum(acc, axis=1, keepdims=True))
        gate_s[pl.ds(r0, T), :] = jnp.broadcast_to(gate, (T, T))

    def regroup(src, t):
        rows = []
        for i in range(2):
            ab = [src[pl.ds(2 * t + i + h * DH // 2, H // 2, stride=DH), :] for h in range(2)]
            ab[0] = pace(ab[0]) if i == 0 else ab[0]
            rows += [_pack(*[pltpu.unpack_elementwise(w, index=e, packed_dtype=BF16, unpacked_dtype=F32)
                             for w in ab]) for e in range(2)]
        return jnp.concatenate(rows, 0)

    def w_qkv(s):
        for c in range(NT):
            for kt in range(NT):
                w = wqkv_ref[kt * T:(kt + 1) * T, s * D + c * T:s * D + (c + 1) * T]
                wt_s[s, kt, c * (T // 2):(c + 1) * (T // 2), :] = pltpu.bitcast(w.T, U32)
                yield 1
        for t in range(NT):
            for kt in range(NT):
                wp_s[t, kt, s * (T // 2):(s + 1) * (T // 2), :] = regroup(wt_s.at[s, kt], t)
                yield 1

    def w_out():
        for ct in range(NT):
            wt_s[0, ct] = pltpu.bitcast(wo_ref[:, ct * T:(ct + 1) * T], U32)
            for t in range(NT):
                wop_s[ct, t * (T // 2):(t + 1) * (T // 2), :] = regroup(wt_s.at[0, ct], t)
            yield 1

    def put_par(i, a):
        par_s[i, 0:T, :] = a[0:T].T
        hi = a[T:N]
        par_s[i, T:N, :] = jnp.concatenate(
            [hi, pltpu.roll(hi, T // 2, 1)], 0).T[0:T // 2]

    def discretize(j):
        c0 = j * T if isinstance(j, int) else pl.multiple_of(j * T, T)
        dt = jnp.exp(ldt_ref[:, pl.ds(c0, T)].astype(F32)).astype(BF16).astype(F32)
        load = lambda i: ssm_ref[i, :, pl.ds(c0, T)].astype(F32)
        return dt, load, jnp.exp(dt * load(0)), dt * load(1)

    def prep(j):
        dt, load, mag, ang = discretize(j)
        sin, cos = _sincos(ang)
        w = _cmul((load(4), load(5)), (dt * load(2), dt * load(3)))
        for i, a in enumerate((mag * cos, mag * sin, w[0], -w[1])):
            put_par(i, a)
        return jnp.max(jnp.abs(ang))

    def prep_wide(j, ang_max):
        def redo(_):
            _, _, mag, ang = discretize(j)
            put_par(0, mag * jnp.cos(ang))
            put_par(1, mag * jnp.sin(ang))
        _loop(jnp.where(ang_max <= SINCOS_MAX, 0, 1), redo)

    GEN_STEPS = 28

    def gen(r, hi):
        r0 = r * 8 if isinstance(r, int) else pl.multiple_of(r * 8, 8)
        d0 = (r // 4) * GS + (r % 4) * 8
        s0 = T + r0 if hi else r0

        def put(dst, i, a, b):
            re, im = _pack(a[0], b[0]), _pack(a[1], b[1])
            if hi:
                t = pltpu.roll(jnp.where(lo, im, re), T // 2, 1)
                dst[2, pl.ds(i * 4 * GS + d0, 8), :] = jnp.where(lo, re, t)
                dst[2, pl.ds(i * 4 * GS + 2 * GS + d0, 8), :] = jnp.where(lo, t, im)
            else:
                dst[0, pl.ds(i * 4 * GS + d0, 8), :] = re
                dst[1, pl.ds(i * 4 * GS + d0, 8), :] = im

        p = (par_s[0, pl.ds(s0, 8), :], par_s[1, pl.ds(s0, 8), :])
        p2 = _csq(p)
        p4 = _csq(p2)
        q = _csq(p4)
        q2 = _csq(q)
        q4 = _csq(q2)
        yield 1
        v = [(jnp.ones_like(q[0]), jnp.zeros_like(q[0])), q, q2, _cmul(q, q2)]
        by_q4 = _times(q4)
        for i in range(NV // 2):
            put(vs_s, 2 * i, v[0], v[1])
            yield 1
            put(vs_s, 2 * i + 1, v[2], v[3])
            if i == 0:
                v = [q4] + [by_q4(a) for a in v[1:]]
            elif i < NV // 2 - 1:
                v = [by_q4((pace(v[0][0]), v[0][1]))] + [by_q4(a) for a in v[1:]]
            yield 1
        b1 = by_q4(v[0])
        u = [(par_s[2, pl.ds(s0, 8), :], par_s[3, pl.ds(s0, 8), :])]
        u += [_times(p, True)(u[0])]
        put(us_s, 0, u[0], u[1])
        yield 1
        fs, by = [p2, p4, b1], []
        for i, (a, b, f) in enumerate(((0, 1, 0), (0, 1, 1), (2, 3, 1), (0, 2, 2), (4, 6, 2),
                                       (0, 4, 3), (8, 10, 3), (0, 8, 4), (12, 14, 4))):
            if f == len(fs):
                fs.append(_csq(fs[-1]))
            if f == len(by):
                by.append(_times(fs[f], True))
            u += [by[f]((pace(u[a][0]), u[a][1])), by[f](u[b])]
            put(us_s, 1 + i, u[-2], u[-1])
            yield 1
        last = u[16][0] * fs[4][0] + u[16][1] * fs[4][1]
        if hi:
            kend_s[1, pl.ds(r0, 8), :] = jnp.where(lo, last, 0.0)
            kend_s[1, pl.ds(T // 2 + r0, 8), :] = jnp.where(lo, 0.0, last)
        else:
            kend_s[0, pl.ds(r0, 8), :] = last
        yield 1

    def kmat(g):
        u = jnp.concatenate([_halves(us_s[t, pl.ds(g, 4 * NU, stride=GS), :]) for t in range(3)], 1)
        v = jnp.concatenate([_halves(vs_s[t, pl.ds(g, 4 * NV, stride=GS), :]) for t in range(3)], 1)
        r = _dot_nt(u, v)
        ko_s[pl.ds(g * KS, 8 * NU), :] = r
        post(r, KMAT_EVERY)

    def taps(j):
        lane32 = jax.lax.broadcasted_iota(jnp.int32, (32, T), 1)
        slot = (lane32 % 8) // 2

        def gather(t):
            parts = []
            for c in range(4):
                acc = None
                for jj in range(4):
                    k = 4 * t + jj
                    a = ko_s[pl.ds((k // 2) * 8 + 2 * c + k % 2, 32, stride=KS), :]
                    if jj != c:
                        a = pltpu.roll(a, (2 * (jj - c)) % T, 1)
                    acc = a if acc is None else jnp.where(slot == jj, a, acc)
                parts.append(acc)
            return jnp.concatenate(parts, 0)

        def emit(ms, taps):
            kt_s[_SLOT[ms[0]]] = _words(taps)

        lane_t = jax.lax.broadcasted_iota(jnp.int32, (T, T), 1)
        lo_t, first = lane_t < T // 2, lane_t == 0
        t4 = gather(4)
        emit([8, 9], t4)
        for m in (10, 12):
            emit([m, m + 1], pltpu.roll(t4, _TAPS[m][1], 1))
        kend = jnp.sum(kend_s[0] + kend_s[1], axis=1, keepdims=True)
        emit([14, 15], jnp.where(lane_t == 2, kend, pltpu.roll(t4, _TAPS[14][1], 1)))
        yield 1
        t3 = gather(3)
        emit([4, 5], t3)
        emit([6, 7], jnp.where(lane_t == 4, pltpu.roll(t4, 4, 1), pltpu.roll(t3, _TAPS[6][1], 1)))
        yield 1
        t2 = gather(2)
        emit([2], t2)
        emit([3], jnp.where(first, t3, t2))
        yield 1
        t1 = gather(1)
        yield 1
        t0 = gather(0)
        x = pltpu.roll(jnp.where(lo_t, t1, t0), T // 2, 1)
        emit([1], jnp.where(lo_t, x, t1))
        skip = dsk_ref[:, pl.ds(j * T if isinstance(j, int) else pl.multiple_of(j * T, T), T)].astype(F32)
        skip = jnp.broadcast_to(skip, (T, T)).T
        emit([0], jnp.where(lo_t, t0, x) + jnp.where(first, skip, 0.0))
        yield 1

    def spectrum_k():
        for m in range(NB):
            r = _dot_nt(_halves(fk_ref[_SHARE[m]]), _halves(kt_s[_SLOT[m]]))
            kh_s[m, 0:T, :] = r[:T]
            kh_s[m, IM:IM + T, :] = r[T:]
            post(r, FK_EVERY)
            yield 64

    PW_STEPS = 3 * NB * (NB + 1) // 2

    def pointwise(j, i):
        r0 = _aligned(i * 8, 8)

        def part(ref, m, c):
            if c < 2:
                return ref[m, pl.ds(c * IM + r0, 8), :]
            return part(ref, m, 0) + part(ref, m, 1)

        prev = None
        for c in range(3):
            for p0 in range(0, NB, PW_SPLIT):
                ps = range(p0, p0 + PW_SPLIT)
                xs, acc = {}, {}
                for m in range(p0 + PW_SPLIT):
                    k = part(kh_s, m, c)
                    if m % 2 == 0:
                        k = pace(k)
                    for p in ps:
                        if p >= m:
                            if p - m not in xs:
                                xs[p - m] = part(xh_s.at[j], p - m, c)
                            kx = k * xs[p - m]
                            acc[p] = kx + acc[p] if m else kx - tmp_s[p] if c == 2 else kx
                    yield min(p0 + PW_SPLIT - m, PW_SPLIT)
                for p in ps:
                    if c == 0:
                        tmp_s[p] = acc[p]
                    elif c == 1:
                        rr = tmp_s[p]
                        tmp_s[NB + p] = rr - acc[p]
                        tmp_s[p] = rr + acc[p]
                    else:
                        y = (tmp_s[NB + p], acc[p])
                        z = y if prev is None else (y[0] - prev[1], y[1] + prev[0])
                        yh_s[j, p, pl.ds(r0, 8), :] = _pack(*z)
                        prev = y

    qscale = float(DH ** -0.5 * np.log2(np.e))

    def qkv(j, i, every):
        r0, h0 = i * QR, i * (QR // 2)
        if not isinstance(i, int):
            r0, h0 = pl.multiple_of(r0, QR), pl.multiple_of(h0, QR // 2)
        for s in range(3):
            x = jnp.concatenate([_halves(xs_s[t, pl.ds(h0, QR // 2), :]) for t in range(NT)], 1)
            w = jnp.concatenate([_halves(wp_s[j, t, s * (T // 2):(s + 1) * (T // 2), :])
                                 for t in range(NT)], 1)
            acc = _dot_nt(x, w)
            if s == 0:
                q_s[j, pl.ds(r0, QR), :] = acc * qscale
            else:
                (k_s, v_s)[s - 1][j, pl.ds(HALO + r0, QR), :] = acc
            post(acc, every)
            yield QR * 5 // 4

    def window(r0, masked):
        rows = lambda r: pl.ds(r, 8)
        qs = [q_s[t, rows(r0), :] for t in range(NT)]
        ls = []
        for w in range(WIN):
            a = None
            for t in range(NT):
                k = k_s[t, rows(r0 + HALO - DIL * w), :]
                kq = qs[t] * (pace(k) if t == 0 and w in PACE_K else k)
                a = kq if a is None else a + kq
            ls.append((a, pltpu.roll(a, 64, 1)))
        yield 1
        ls = [a + b for a, b in ls]
        ls = [(a, pltpu.roll(a, 32, 1)) for a in ls]
        yield 1
        ls = [a + b for a, b in ls]
        if masked:
            row = jax.lax.broadcasted_iota(jnp.int32, (8, T), 0) + r0
            ls = [jnp.where(row >= DIL * w, a, -1e9 * np.log2(np.e)) for w, a in enumerate(ls)]
        mx = _tree(jnp.maximum, ls)
        es = [jnp.exp2(a - mx) for a in ls]
        yield 1
        inv = gate_s[rows(r0), :] * pl.reciprocal(_tree(jnp.add, es), full_range=False)
        outs = []
        for t in range(NT):
            a = None
            for w in range(WIN):
                v = v_s[t, rows(r0 + HALO - DIL * w), :]
                pv = es[w] * (pace(v) if w == 0 and t in PACE_V else v)
                a = pv if a is None else a + pv
            outs.append(a)
        for t in range(NT):
            at_s[t, rows(r0), :] = outs[t] * inv
        yield 1

    def attend(r0, n, first=False):
        gens = [window(r0 + 8 * c, first and 8 * c < DIL * WIN) for c in range(n)]
        for step in range(n + 3):
            for c in range(step, step - 4, -1):
                if 0 <= c < n:
                    next(gens[c])
            yield 1

    def stage(i):
        r0 = _aligned(i * RB, RB)
        for t in range(NT):
            cur_s[t] = _pack(*[at_s[t, pl.ds(r0 + e, RB // 2, stride=2), :] for e in range(2)])

    def out_copy(i):
        r0 = _aligned(i * RB, RB)
        return pltpu.make_async_copy(o_ref.at[pl.ds(r0, RB), :], o_hbm.at[pl.ds(r0, RB), :], osem)

    def tail_copy(ct):
        part = (slice(S - RB, S), slice(ct * T, (ct + 1) * T))
        return pltpu.make_async_copy(o_ref.at[part], o_hbm.at[part], osem)

    def mix(i):
        r0 = _aligned(i * RB, RB)
        for ct in range(NT):
            for h in range(RB // T):
                y = _dot(jnp.concatenate([_halves(g_ref[b]) for b in range(2)], 1),
                         _halves(yh_s[ct, i * (RB // T) + h]))
                y_s[ct, h * T:(h + 1) * T, :] = (1.0 - gate_s[pl.ds(r0 + h * T, T), :]) * y
                post(y, T)
                yield 64
        for ct in range(NT):
            yield from project(r0, ct)

    def project(r0, ct):
        a = _dot(jnp.concatenate([_halves(cur_s[t]) for t in range(NT)], 1), _halves(wop_s[ct]))
        acc = a + y_s[ct]
        o_ref[pl.ds(r0, RB), ct * T:(ct + 1) * T] = acc.astype(BF16)
        if isinstance(r0, int):
            tail_copy(ct).start()
        post(acc, MIX_EVERY)
        yield RB * 5 // 4

    def gen_streams(i0, n, serial):
        units = lambda i, u: [gen(4 * i + 2 * u, False), gen(4 * i + 2 * u + 1, False), gen(2 * i + u, True)]
        if serial:
            return [(_chain([g for i in range(n) for u in range(2) for g in units(i0 + i, u)]),
                     6 * n * GEN_STEPS, 0.0, 1.0)]
        return [(_chain([g for i in range(n) for g in units(i0 + i, u)]), 3 * n * GEN_STEPS, 0.0, 1.0)
                for u in range(2)]

    def qkvs(j, i0, n, every):
        return _chain([qkv(j, i0 + u, every) for u in range(n)])

    def kmats(g0, n):
        for u in range(n):
            kmat(g0 + u)
            yield 60

    def overlap(*streams, gap=1, lag=0):
        always[:] = [zero_s[...] == 0.0, gap, 0, lag]
        _interleave(*streams)
        tokens.clear()
        always.clear()

    nq, cq = S // QR, QR * 15 // 4

    for t in range(NT):
        k_s[t, 0:HALO, :] = jnp.zeros((HALO, T), F32)
        v_s[t, 0:HALO, :] = jnp.zeros((HALO, T), F32)
    zero_s[...] = jnp.zeros((8, T), F32)
    for c in cp_vec + cp_ssm[0]:
        c.wait()
    for i, ref in enumerate((ldt_in, dsk_in, gw_in)):
        vec_s[i] = ref[...].astype(F32).reshape(1, D)
    prep_wide(0, prep(0))
    cp_fx.wait()

    def first(i):
        for when, cs in enumerate(([cp_x(2), cp_w[0]], [cp_x(3), cp_w[1]], cp_w[2:], [cp_fk] + cp_ssm[1])):
            @pl.when(i == when)
            def _():
                for c in cs:
                    c.start()
        cp_x(i).wait()
        xs = (_chain([x_block(4 * i + u) for u in range(4)]), 4 * NT, X_LEAD, X_LAST)
        overlap(xs, *gen_streams(i, 1, X_SERIAL), gap=X_GAP, lag=X_LAG)
    _loop(4, first)
    for c in cp_ssm[2] + cp_out:
        c.start()
    for c in cp_w:
        c.wait()
    ws = (_chain([w_qkv(s) for s in range(3)]), 6 * NT * NT, 0.0, 1.0)
    overlap((kmats(0, 32), 1920, LEAD, LAST), ws, lag=PW_LAG)
    overlap((qkv(0, 0, QR), cq, 0.0, 1.0), (taps(0), 5, 0.0, 1.0))
    for c in [cp_fk] + cp_ssm[1]:
        c.wait()

    def pws(j, i0, n):
        return (_chain([pointwise(j, i0 + u) for u in range(n)]), n * PW_STEPS, 0.0, 1.0)

    def tile(j):
        @pl.when(j == 1)
        def _():
            for c in cp_ssm[2]:
                c.wait()
        overlap((spectrum_k(), 1024, 0.0, 1.0))
        prep_wide(j + 1, prep(j + 1))

        def expand(i):
            n = 4 // NG
            overlap((qkvs(j, n * i + 1, n, GEN_EVERY), n * cq, LEAD2, LAST2), *gen_streams(n * i, n, GEN_SERIAL), gap=GEN_GAP, lag=GEN_LAG)
        _loop(NG, expand)
        mxu = _chain([kmats(0, 32), qkvs(j, 5, NA, PW_EVERY)])
        overlap((mxu, 1920 + NA * cq, LEAD, LAST), pws(j, 0, PA), gap=PW_GAP, lag=PW_LAG)
        n = nq - 4 - NA
        mxu = _chain([qkvs(j, NA + 5, n - 1, PW_EVERY), qkv(j + 1, 0, PW_EVERY)])
        st = [(mxu, n * cq, LEAD, LAST), pws(j, PA, 16 - PA)]
        overlap(*st, (taps(j + 1), 5, 0.0, TAP_LAST), gap=PW_GAP, lag=PW_LAG)
    _loop(NT - 1, tile)

    j = NT - 1
    for c in cp_out:
        c.wait()
    mxu = _chain([spectrum_k(), qkvs(j, 1, HEAD - 1, 64)])
    st = [(mxu, 1024 + cq * (HEAD - 1), LEAD, LAST), (attend(0, FIRST, True), FIRST + 3, 0.0, 1.0)]
    overlap(*st, (w_out(), NT, 0.0, 1.0), lag=PW_LAG)
    n = (nq - HEAD) // NL

    def last_conv(i):
        r0 = pl.multiple_of(8 * (FIRST + i * EARLY), 16)
        st = [(qkvs(j, HEAD + n * i, n, PW_EVERY), cq * n, LEAD, LAST), pws(j, 16 // NL * i, 16 // NL)]
        overlap(*st, (attend(r0, EARLY), EARLY + 3, 0.0, 1.0), gap=PW_GAP, lag=PW_LAG)
    _loop(NL, last_conv)

    done, nr = FIRST + NL * EARLY, S // RB
    n_mixed = (S // 8 - done) // PER_ROW
    assert n * NL + HEAD == nq and done + n_mixed * PER_ROW == S // 8 and n_mixed == nr - 1
    assert 8 * FIRST <= QR and FIRST % 2 == EARLY % 2 == PER_ROW % 2 == 0
    assert all(8 * (FIRST + EARLY * (i + 1)) <= (HEAD + n * i) * QR for i in range(NL))
    assert all(8 * (done + PER_ROW * i) >= (i + 1) * RB for i in range(n_mixed + 1))
    stage(0)

    def rows(i):
        r0 = pl.multiple_of(8 * (done + PER_ROW * i), 16)
        overlap((mix(i), NT * RB * 7 // 4, MIX_LEAD, MIX_LAST),
                (attend(r0, PER_ROW), 100 * PER_ROW + 300, 0.0, 1.0), lag=1)
        stage(i + 1)
        out_copy(i).start()
    _loop(nr - 1, rows)
    overlap((mix(nr - 1), 1, 0.0, 1.0))
    for i in range(nr - 1):
        out_copy(i).wait()
    for ct in range(NT):
        tail_copy(ct).wait()


@jax.jit
def pallas_gated_mix__sliding_local_dilated__ssm_conv_s4__prompt_kernel(
    A_x: jax.Array,
    A_wqkv: jax.Array,
    A_wo: jax.Array,
    B_u: jax.Array,
    B_A_re: jax.Array,
    B_A_im: jax.Array,
    B_B_re: jax.Array,
    B_B_im: jax.Array,
    B_C_re: jax.Array,
    B_C_im: jax.Array,
    B_log_dt: jax.Array,
    B_Dskip: jax.Array,
    gate_w: jax.Array,
):
    del B_u
    fx, g, fk = _constants()
    vm = pltpu.VMEM
    hbm = pl.BlockSpec(memory_space=pl.ANY)
    out = pl.pallas_call(
        _kernel,
        out_shape=jax.ShapeDtypeStruct((S, D), BF16),
        in_specs=[hbm] * 15,
        out_specs=hbm,
        scratch_shapes=[
            vm((S, D), BF16), vm((D, 3 * D), BF16), vm((D, D), BF16), vm((6, N, D), BF16),
            vm(fx.shape, U32), vm(g.shape, U32), vm(fk.shape, U32), vm((S, D), BF16),
            vm((NT, S // 2, T), U32), vm((S, T), F32),
            vm((3, NT, D // 2, T), U32), vm((NT, NT, 3 * T // 2, T), U32), vm((NT, D // 2, T), U32),
            vm((4, N, T), F32), vm((3, NU * 4 * GS, T), U32), vm((3, NV * 4 * GS, T), U32),
            vm((2, T, T), F32), vm((32 * KS, T), F32), vm((max(_SLOT) + 1, T // 2, T), U32),
            vm((NB, SPEC, T), F32), vm((NT, NB, SPEC, T), F32), vm((NT, NB, T, T), U32),
            vm((2 * NB, 8, T), F32),
            vm((NT, S, T), F32), vm((NT, S + HALO, T), F32), vm((NT, S + HALO, T), F32),
            vm((NT, S, T), F32), vm((NT, RB // 2, T), U32), vm((NT, RB, T), F32), vm((8, T), F32),
            vm((3, 1, D), F32), vm((D,), BF16), vm((D,), BF16), vm((D,), BF16),
            pltpu.SemaphoreType.DMA((N_COPIES,)), pltpu.SemaphoreType.DMA((4,)),
             pltpu.SemaphoreType.DMA(()),
        ],
        compiler_params=pltpu.CompilerParams(vmem_limit_bytes=100 * 1024 * 1024),
    )(A_x.reshape(S, D), A_wqkv, A_wo, B_A_re.T, B_A_im.T, B_B_re.T, B_B_im.T, B_C_re.T, B_C_im.T,
      B_log_dt, B_Dskip, gate_w, fx, g, fk)
    return out.reshape(1, S, D)
```

```python
import jax
import jax.numpy as jnp
import numpy as np
import jax.experimental.pallas as pl
import jax.experimental.pallas.tpu as pltpu

S, D, H, DH, N = 2048, 640, 32, 20, 192
WIN, DIL = 8, 2
T = 128
NT = D // T
NB = S // T
HALO = 32
N_COPIES = 28
SINCOS_MAX = 8192.0
LEAD = 0.04
LEAD2 = 0.03
LAST = 0.98
LAST2 = 0.98
QR = 256
HEAD = 2
NL = 2
FIRST = 28
EARLY = 16
RB = 256
PER_ROW = 28
GEN_SERIAL = True
FK_EVERY = 256
KMAT_EVERY = 40
PW_EVERY = 16
GEN_EVERY = 8
MIX_EVERY = 64
MIX_LEAD = 0.05
MIX_LAST = 1.0
PACE_K = ()
PACE_V = (0,)
X_LAG = 8
X_SERIAL = True
X_GAP = 1
X_EVERY = 64
X_LEAD = 0.1
X_LAST = 0.95
GEN_GAP = 1
PW_GAP = 2
PW_SPLIT = 8
KEEP = 32
NG = 1
NA = 1
PA = 8
TAP_LAST = 0.8
GEN_LAG = 6
PW_LAG = 4
IM = 144
SPEC = 280
NU, NV = 10, 16
GS = 36
KS = 84
F32, BF16, U32 = jnp.float32, jnp.bfloat16, jnp.uint32

_BASES = [0, 1, 2, 3, 4, 5, 6, 7, 256, 258, 260, 262, 512, 516, 768, 772,
          1024, 1280, 1536, 1792]


_TAPS = {2: (2, 0, None), 3: (2, 0, 0),
         4: (3, 0, None), 5: (3, 0, None), 6: (3, T - 4, None), 7: (3, T - 4, 4)}
_TAPS.update({m: (4, (8 - m + m % 2) % T, 2 if m == NB - 1 else None) for m in range(8, NB)})
_SLOT = [0, 1, 2, 3] + [4 + (m - 4) // 2 for m in range(4, NB)]
_SHARE = [0, 0, 1, 2, 3, 4, 3, 4] + [5, 6] * 4


def _pack_rows(a):
    b = a.astype(np.float32).astype(BF16).view(np.uint16).astype(np.uint32)
    return b[..., 0::2, :] | (b[..., 1::2, :] << 16)


def _constants():
    om = 2.0 * np.pi * (np.arange(T) + 0.25) / T
    ph = np.exp(-1j * om[:, None] * np.arange(T)[None, :])
    fx = np.concatenate([ph.real, ph.imag], 0)
    g = np.stack([ph.real.T, ph.imag.T], -1).reshape(T, 2 * T) / T
    lag = np.arange(S).astype(np.float32).astype(BF16).astype(np.float32).astype(np.int64)
    lane = np.arange(T)
    off = 8 * (2 * (lane // 8) + lane % 2)
    tiles = [np.array(_BASES[4 * t:4 * t + 4])[(lane % 8) // 2] + off for t in range(5)]
    lo = lane < T // 2
    vals = [np.where(lo, tiles[0], np.roll(tiles[1], T // 2)),
            np.where(lo, np.roll(tiles[0], T // 2), tiles[1])]
    for m in range(2, NB):
        t, shift, end = _TAPS[m]
        v = np.roll(tiles[t], shift)
        vals.append(v if end is None else np.where(lane == end, (m + 1) * T, v))
    fk = np.zeros((max(_SHARE) + 1, 2 * T, T))
    for m in range(NB):
        blk = lag[m * T:(m + 1) * T]
        e = (blk[:, None] == vals[m][None, :]).astype(np.float64)
        assert (e.sum(1) == 1).all()
        c = np.concatenate([(ph @ e).real, (ph @ e).imag], 0)
        assert _SHARE.index(_SHARE[m]) == m or np.array_equal(fk[_SHARE[m]], c)
        fk[_SHARE[m]] = c
    g = np.stack([g[:, :T], g[:, T:]])
    return _pack_rows(fx), _pack_rows(g), _pack_rows(fk)


def _cmul(a, b):
    return a[0] * b[0] - a[1] * b[1], a[0] * b[1] + a[1] * b[0]


def _times(f, conj=False):
    dif, tot = f[1] - f[0], f[1] + f[0]

    def mul(a):
        k = f[0] * (a[0] + a[1])
        if conj:
            return k + a[1] * dif, k - a[0] * tot
        return k - a[1] * tot, k + a[0] * dif
    return mul


def _csq(a):
    t = a[0] * a[1]
    return a[0] * a[0] - a[1] * a[1], t + t


def _tree(op, xs):
    while len(xs) > 1:
        xs = [op(a, b) for a, b in zip(xs[0::2], xs[1::2])]
    return xs[0]


def _pack(a, b):
    return pltpu.pack_elementwise([a, b], packed_dtype=BF16)


def _words(a):
    return pltpu.bitcast(a.astype(BF16), U32)


def _halves(a):
    return pltpu.bitcast(a, BF16)


def _dot(a, b):
    return jnp.dot(a, b, preferred_element_type=F32)


def _dot_nt(a, b):
    return jax.lax.dot_general(a, b, (((1,), (1,)), ((), ())), preferred_element_type=F32)


def _sincos(x):
    k = jnp.floor(x * (2.0 / np.pi) + 0.5)
    r = ((x - k * 1.5703125) - k * 4.837512969970703125e-4) - k * 7.54978995489188216e-8
    z = r * r
    s = r + r * z * (-1.6666654611e-1 + z * (8.3321608736e-3 + z * -1.9515295891e-4))
    c = 1.0 + z * (-0.5 + z * (4.166664568298827e-2
                               + z * (-1.388731625493765e-3 + z * 2.443315711809948e-5)))
    n = k.astype(jnp.int32)
    odd = (n & 1) == 1
    s, c = jnp.where(odd, c, s), jnp.where(odd, s, c)
    return jnp.where((n & 2) == 2, -s, s), jnp.where(((n + 1) & 2) == 2, -c, c)


def _aligned(i, n):
    return i if isinstance(i, int) else pl.multiple_of(i, n)


def _loop(n, body):
    jax.lax.fori_loop(0, n, lambda i, c: body(i), None)


def _interleave(*streams):
    done = [0] * len(streams)
    live = list(range(len(streams)))
    while live:
        i = min(live, key=lambda n: streams[n][2]
                + (streams[n][3] - streams[n][2]) * done[n] / streams[n][1])
        work = next(streams[i][0], None)
        if work is None:
            live.remove(i)
        else:
            done[i] += work


def _chain(gens):
    for g in gens:
        yield from g


def _kernel(x_hbm, wqkv_hbm, wo_hbm, are_hbm, aim_hbm, bre_hbm, bim_hbm, cre_hbm, cim_hbm,
            ldt_hbm, dsk_hbm, gw_hbm, fx_hbm, g_hbm, fk_hbm, o_hbm,
            x_ref, wqkv_ref, wo_ref, ssm_ref, fx_ref, g_ref, fk_ref, o_ref,
            xs_s, gate_s, wt_s, wp_s, wop_s, par_s, us_s, vs_s, kend_s, ko_s, kt_s,
            kh_s, xh_s, yh_s, tmp_s, q_s, k_s, v_s, at_s, cur_s, y_s, zero_s, vec_s, ldt_in, dsk_in, gw_in,
            sems, xsems, osem):
    lane = jax.lax.broadcasted_iota(jnp.int32, (8, T), 1)
    lo = lane < T // 2

    ldt_ref, dsk_ref, gw_ref = vec_s.at[0], vec_s.at[1], vec_s.at[2]
    ssm_hbm = (are_hbm, aim_hbm, bre_hbm, bim_hbm, cre_hbm, cim_hbm)
    sem_ids = iter(range(N_COPIES))
    copy = lambda a, b: pltpu.make_async_copy(a, b, sems.at[next(sem_ids)])
    cp_ssm = [[copy(h.at[:, a:b], ssm_ref.at[i, :, a:b]) for i, h in enumerate(ssm_hbm)]
              for a, b in ((0, T), (T, 2 * T), (2 * T, D))]
    cp_fx = copy(fx_hbm, fx_ref)
    cp_vec = [copy(ldt_hbm, ldt_in), copy(dsk_hbm, dsk_in), copy(gw_hbm, gw_in)]

    def cp_x(i):
        rows = pl.ds(_aligned(i * (S // 4), S // 4), S // 4)
        return pltpu.make_async_copy(x_hbm.at[rows, :], x_ref.at[rows, :], xsems.at[i])
    cp_w = [copy(wqkv_hbm.at[:, s * D:(s + 1) * D], wqkv_ref.at[:, s * D:(s + 1) * D]) for s in range(3)]
    cp_fk = copy(fk_hbm, fk_ref)
    cp_out = [copy(wo_hbm, wo_ref), copy(g_hbm, g_ref)]
    for c in cp_vec + cp_ssm[0] + [cp_fx, cp_x(0), cp_x(1)]:
        c.start()

    tokens, always = [], []

    def post(a, every):
        tokens[:] = tokens[-KEEP:] + [a[r - 8:r] for r in range(every, a.shape[0] + 1, every)]

    def pace(x):
        always[2] += 1
        if len(tokens) <= always[3] or always[2] < always[1]:
            return x
        always[2] = 0
        head = jnp.where(always[0], x[:8], pltpu.bitcast(tokens.pop(0), x.dtype))
        return head if x.shape[0] == 8 else jnp.concatenate([head, x[8:]], 0)

    def x_block(m):
        r0, h0 = _aligned(m * T, T), _aligned(m * (T // 2), T // 2)
        acc = None
        for t in range(NT):
            x = x_ref[pl.ds(r0, T), t * T:(t + 1) * T]
            xs_s[t, pl.ds(h0, T // 2), :] = pltpu.bitcast(x, U32)
            r = _dot(_halves(fx_ref[...]), x)
            xh_s[t, m, 0:T, :] = r[:T]
            xh_s[t, m, IM:IM + T, :] = r[T:]
            post(r, X_EVERY)
            xg = x.astype(F32) * gw_ref[:, t * T:(t + 1) * T]
            acc = xg if acc is None else acc + xg
            yield 1
        gate = jax.nn.sigmoid(jnp.sum(acc, axis=1, keepdims=True))
        gate_s[pl.ds(r0, T), :] = jnp.broadcast_to(gate, (T, T))

    def regroup(src, t):
        rows = []
        for i in range(2):
            ab = [src[pl.ds(2 * t + i + h * DH // 2, H // 2, stride=DH), :] for h in range(2)]
            ab[0] = pace(ab[0]) if i == 0 else ab[0]
            rows += [_pack(*[pltpu.unpack_elementwise(w, index=e, packed_dtype=BF16, unpacked_dtype=F32)
                             for w in ab]) for e in range(2)]
        return jnp.concatenate(rows, 0)

    def w_qkv(s):
        for c in range(NT):
            for kt in range(NT):
                w = wqkv_ref[kt * T:(kt + 1) * T, s * D + c * T:s * D + (c + 1) * T]
                wt_s[s, kt, c * (T // 2):(c + 1) * (T // 2), :] = pltpu.bitcast(w.T, U32)
                yield 1
        for t in range(NT):
            for kt in range(NT):
                wp_s[t, kt, s * (T // 2):(s + 1) * (T // 2), :] = regroup(wt_s.at[s, kt], t)
                yield 1

    def w_out():
        for ct in range(NT):
            wt_s[0, ct] = pltpu.bitcast(wo_ref[:, ct * T:(ct + 1) * T], U32)
            for t in range(NT):
                wop_s[ct, t * (T // 2):(t + 1) * (T // 2), :] = regroup(wt_s.at[0, ct], t)
            yield 1

    def put_par(i, a):
        par_s[i, 0:T, :] = a[0:T].T
        hi = a[T:N]
        par_s[i, T:N, :] = jnp.concatenate(
            [hi, pltpu.roll(hi, T // 2, 1)], 0).T[0:T // 2]

    def discretize(j):
        c0 = j * T if isinstance(j, int) else pl.multiple_of(j * T, T)
        dt = jnp.exp(ldt_ref[:, pl.ds(c0, T)].astype(F32)).astype(BF16).astype(F32)
        load = lambda i: ssm_ref[i, :, pl.ds(c0, T)].astype(F32)
        return dt, load, jnp.exp(dt * load(0)), dt * load(1)

    def prep(j):
        dt, load, mag, ang = discretize(j)
        sin, cos = _sincos(ang)
        w = _cmul((load(4), load(5)), (dt * load(2), dt * load(3)))
        for i, a in enumerate((mag * cos, mag * sin, w[0], -w[1])):
            put_par(i, a)
        return jnp.max(jnp.abs(ang))

    def prep_wide(j, ang_max):
        def redo(_):
            _, _, mag, ang = discretize(j)
            put_par(0, mag * jnp.cos(ang))
            put_par(1, mag * jnp.sin(ang))
        _loop(jnp.where(ang_max <= SINCOS_MAX, 0, 1), redo)

    GEN_STEPS = 28

    def gen(r, hi):
        r0 = r * 8 if isinstance(r, int) else pl.multiple_of(r * 8, 8)
        d0 = (r // 4) * GS + (r % 4) * 8
        s0 = T + r0 if hi else r0

        def put(dst, i, a, b):
            re, im = _pack(a[0], b[0]), _pack(a[1], b[1])
            if hi:
                t = pltpu.roll(jnp.where(lo, im, re), T // 2, 1)
                dst[2, pl.ds(i * 4 * GS + d0, 8), :] = jnp.where(lo, re, t)
                dst[2, pl.ds(i * 4 * GS + 2 * GS + d0, 8), :] = jnp.where(lo, t, im)
            else:
                dst[0, pl.ds(i * 4 * GS + d0, 8), :] = re
                dst[1, pl.ds(i * 4 * GS + d0, 8), :] = im

        p = (par_s[0, pl.ds(s0, 8), :], par_s[1, pl.ds(s0, 8), :])
        p2 = _csq(p)
        p4 = _csq(p2)
        q = _csq(p4)
        q2 = _csq(q)
        q4 = _csq(q2)
        yield 1
        v = [(jnp.ones_like(q[0]), jnp.zeros_like(q[0])), q, q2, _cmul(q, q2)]
        by_q4 = _times(q4)
        for i in range(NV // 2):
            put(vs_s, 2 * i, v[0], v[1])
            yield 1
            put(vs_s, 2 * i + 1, v[2], v[3])
            if i == 0:
                v = [q4] + [by_q4(a) for a in v[1:]]
            elif i < NV // 2 - 1:
                v = [by_q4((pace(v[0][0]), v[0][1]))] + [by_q4(a) for a in v[1:]]
            yield 1
        b1 = by_q4(v[0])
        u = [(par_s[2, pl.ds(s0, 8), :], par_s[3, pl.ds(s0, 8), :])]
        u += [_times(p, True)(u[0])]
        put(us_s, 0, u[0], u[1])
        yield 1
        fs, by = [p2, p4, b1], []
        for i, (a, b, f) in enumerate(((0, 1, 0), (0, 1, 1), (2, 3, 1), (0, 2, 2), (4, 6, 2),
                                       (0, 4, 3), (8, 10, 3), (0, 8, 4), (12, 14, 4))):
            if f == len(fs):
                fs.append(_csq(fs[-1]))
            if f == len(by):
                by.append(_times(fs[f], True))
            u += [by[f]((pace(u[a][0]), u[a][1])), by[f](u[b])]
            put(us_s, 1 + i, u[-2], u[-1])
            yield 1
        last = u[16][0] * fs[4][0] + u[16][1] * fs[4][1]
        if hi:
            kend_s[1, pl.ds(r0, 8), :] = jnp.where(lo, last, 0.0)
            kend_s[1, pl.ds(T // 2 + r0, 8), :] = jnp.where(lo, 0.0, last)
        else:
            kend_s[0, pl.ds(r0, 8), :] = last
        yield 1

    def kmat(g):
        u = jnp.concatenate([_halves(us_s[t, pl.ds(g, 4 * NU, stride=GS), :]) for t in range(3)], 1)
        v = jnp.concatenate([_halves(vs_s[t, pl.ds(g, 4 * NV, stride=GS), :]) for t in range(3)], 1)
        r = _dot_nt(u, v)
        ko_s[pl.ds(g * KS, 8 * NU), :] = r
        post(r, KMAT_EVERY)

    def taps(j):
        lane32 = jax.lax.broadcasted_iota(jnp.int32, (32, T), 1)
        slot = (lane32 % 8) // 2

        def gather(t):
            parts = []
            for c in range(4):
                acc = None
                for jj in range(4):
                    k = 4 * t + jj
                    a = ko_s[pl.ds((k // 2) * 8 + 2 * c + k % 2, 32, stride=KS), :]
                    if jj != c:
                        a = pltpu.roll(a, (2 * (jj - c)) % T, 1)
                    acc = a if acc is None else jnp.where(slot == jj, a, acc)
                parts.append(acc)
            return jnp.concatenate(parts, 0)

        def emit(ms, taps):
            kt_s[_SLOT[ms[0]]] = _words(taps)

        lane_t = jax.lax.broadcasted_iota(jnp.int32, (T, T), 1)
        lo_t, first = lane_t < T // 2, lane_t == 0
        t4 = gather(4)
        emit([8, 9], t4)
        for m in (10, 12):
            emit([m, m + 1], pltpu.roll(t4, _TAPS[m][1], 1))
        kend = jnp.sum(kend_s[0] + kend_s[1], axis=1, keepdims=True)
        emit([14, 15], jnp.where(lane_t == 2, kend, pltpu.roll(t4, _TAPS[14][1], 1)))
        yield 1
        t3 = gather(3)
        emit([4, 5], t3)
        emit([6, 7], jnp.where(lane_t == 4, pltpu.roll(t4, 4, 1), pltpu.roll(t3, _TAPS[6][1], 1)))
        yield 1
        t2 = gather(2)
        emit([2], t2)
        emit([3], jnp.where(first, t3, t2))
        yield 1
        t1 = gather(1)
        yield 1
        t0 = gather(0)
        x = pltpu.roll(jnp.where(lo_t, t1, t0), T // 2, 1)
        emit([1], jnp.where(lo_t, x, t1))
        skip = dsk_ref[:, pl.ds(j * T if isinstance(j, int) else pl.multiple_of(j * T, T), T)].astype(F32)
        skip = jnp.broadcast_to(skip, (T, T)).T
        emit([0], jnp.where(lo_t, t0, x) + jnp.where(first, skip, 0.0))
        yield 1

    def spectrum_k():
        for m in range(NB):
            r = _dot_nt(_halves(fk_ref[_SHARE[m]]), _halves(kt_s[_SLOT[m]]))
            kh_s[m, 0:T, :] = r[:T]
            kh_s[m, IM:IM + T, :] = r[T:]
            post(r, FK_EVERY)
            yield 64

    PW_STEPS = 3 * NB * (NB + 1) // 2

    def pointwise(j, i):
        r0 = _aligned(i * 8, 8)

        def part(ref, m, c):
            if c < 2:
                return ref[m, pl.ds(c * IM + r0, 8), :]
            return part(ref, m, 0) + part(ref, m, 1)

        prev = None
        for c in range(3):
            for p0 in range(0, NB, PW_SPLIT):
                ps = range(p0, p0 + PW_SPLIT)
                xs, acc = {}, {}
                for m in range(p0 + PW_SPLIT):
                    k = part(kh_s, m, c)
                    if m % 2 == 0:
                        k = pace(k)
                    for p in ps:
                        if p >= m:
                            if p - m not in xs:
                                xs[p - m] = part(xh_s.at[j], p - m, c)
                            kx = k * xs[p - m]
                            acc[p] = kx + acc[p] if m else kx - tmp_s[p] if c == 2 else kx
                    yield min(p0 + PW_SPLIT - m, PW_SPLIT)
                for p in ps:
                    if c == 0:
                        tmp_s[p] = acc[p]
                    elif c == 1:
                        rr = tmp_s[p]
                        tmp_s[NB + p] = rr - acc[p]
                        tmp_s[p] = rr + acc[p]
                    else:
                        y = (tmp_s[NB + p], acc[p])
                        z = y if prev is None else (y[0] - prev[1], y[1] + prev[0])
                        yh_s[j, p, pl.ds(r0, 8), :] = _pack(*z)
                        prev = y

    qscale = float(DH ** -0.5 * np.log2(np.e))

    def qkv(j, i, every):
        r0, h0 = i * QR, i * (QR // 2)
        if not isinstance(i, int):
            r0, h0 = pl.multiple_of(r0, QR), pl.multiple_of(h0, QR // 2)
        for s in range(3):
            x = jnp.concatenate([_halves(xs_s[t, pl.ds(h0, QR // 2), :]) for t in range(NT)], 1)
            w = jnp.concatenate([_halves(wp_s[j, t, s * (T // 2):(s + 1) * (T // 2), :])
                                 for t in range(NT)], 1)
            acc = _dot_nt(x, w)
            if s == 0:
                q_s[j, pl.ds(r0, QR), :] = acc * qscale
            else:
                (k_s, v_s)[s - 1][j, pl.ds(HALO + r0, QR), :] = acc
            post(acc, every)
            yield QR * 5 // 4

    def window(r0, masked):
        rows = lambda r: pl.ds(r, 8)
        qs = [q_s[t, rows(r0), :] for t in range(NT)]
        ls = []
        for w in range(WIN):
            a = None
            for t in range(NT):
                k = k_s[t, rows(r0 + HALO - DIL * w), :]
                kq = qs[t] * (pace(k) if t == 0 and w in PACE_K else k)
                a = kq if a is None else a + kq
            ls.append((a, pltpu.roll(a, 64, 1)))
        yield 1
        ls = [a + b for a, b in ls]
        ls = [(a, pltpu.roll(a, 32, 1)) for a in ls]
        yield 1
        ls = [a + b for a, b in ls]
        if masked:
            row = jax.lax.broadcasted_iota(jnp.int32, (8, T), 0) + r0
            ls = [jnp.where(row >= DIL * w, a, -1e9 * np.log2(np.e)) for w, a in enumerate(ls)]
        mx = _tree(jnp.maximum, ls)
        es = [jnp.exp2(a - mx) for a in ls]
        yield 1
        inv = gate_s[rows(r0), :] * pl.reciprocal(_tree(jnp.add, es), full_range=False)
        outs = []
        for t in range(NT):
            a = None
            for w in range(WIN):
                v = v_s[t, rows(r0 + HALO - DIL * w), :]
                pv = es[w] * (pace(v) if w == 0 and t in PACE_V else v)
                a = pv if a is None else a + pv
            outs.append(a)
        for t in range(NT):
            at_s[t, rows(r0), :] = outs[t] * inv
        yield 1

    def attend(r0, n, first=False):
        gens = [window(r0 + 8 * c, first and 8 * c < DIL * WIN) for c in range(n)]
        for step in range(n + 3):
            for c in range(step, step - 4, -1):
                if 0 <= c < n:
                    next(gens[c])
            yield 1

    def stage(i):
        r0 = _aligned(i * RB, RB)
        for t in range(NT):
            cur_s[t] = _pack(*[at_s[t, pl.ds(r0 + e, RB // 2, stride=2), :] for e in range(2)])

    def out_copy(i):
        r0 = _aligned(i * RB, RB)
        return pltpu.make_async_copy(o_ref.at[pl.ds(r0, RB), :], o_hbm.at[pl.ds(r0, RB), :], osem)

    def tail_copy(ct):
        part = (slice(S - RB, S), slice(ct * T, (ct + 1) * T))
        return pltpu.make_async_copy(o_ref.at[part], o_hbm.at[part], osem)

    def mix(i):
        r0 = _aligned(i * RB, RB)
        for ct in range(NT):
            for h in range(RB // T):
                y = _dot(jnp.concatenate([_halves(g_ref[b]) for b in range(2)], 1),
                         _halves(yh_s[ct, i * (RB // T) + h]))
                y_s[ct, h * T:(h + 1) * T, :] = (1.0 - gate_s[pl.ds(r0 + h * T, T), :]) * y
                post(y, T)
                yield 64
        for ct in range(NT):
            yield from project(r0, ct)

    def project(r0, ct):
        a = _dot(jnp.concatenate([_halves(cur_s[t]) for t in range(NT)], 1), _halves(wop_s[ct]))
        acc = a + y_s[ct]
        o_ref[pl.ds(r0, RB), ct * T:(ct + 1) * T] = acc.astype(BF16)
        if isinstance(r0, int):
            tail_copy(ct).start()
        post(acc, MIX_EVERY)
        yield RB * 5 // 4

    def gen_streams(i0, n, serial):
        units = lambda i, u: [gen(4 * i + 2 * u, False), gen(4 * i + 2 * u + 1, False), gen(2 * i + u, True)]
        if serial:
            return [(_chain([g for i in range(n) for u in range(2) for g in units(i0 + i, u)]),
                     6 * n * GEN_STEPS, 0.0, 1.0)]
        return [(_chain([g for i in range(n) for g in units(i0 + i, u)]), 3 * n * GEN_STEPS, 0.0, 1.0)
                for u in range(2)]

    def qkvs(j, i0, n, every):
        return _chain([qkv(j, i0 + u, every) for u in range(n)])

    def kmats(g0, n):
        for u in range(n):
            kmat(g0 + u)
            yield 60

    def overlap(*streams, gap=1, lag=0):
        always[:] = [zero_s[...] == 0.0, gap, 0, lag]
        _interleave(*streams)
        tokens.clear()
        always.clear()

    nq, cq = S // QR, QR * 15 // 4

    for t in range(NT):
        k_s[t, 0:HALO, :] = jnp.zeros((HALO, T), F32)
        v_s[t, 0:HALO, :] = jnp.zeros((HALO, T), F32)
    zero_s[...] = jnp.zeros((8, T), F32)
    for c in cp_vec + cp_ssm[0]:
        c.wait()
    for i, ref in enumerate((ldt_in, dsk_in, gw_in)):
        vec_s[i] = ref[...].astype(F32).reshape(1, D)
    prep_wide(0, prep(0))
    cp_fx.wait()

    def first(i):
        for when, cs in enumerate(([cp_x(2), cp_w[0]], [cp_x(3), cp_w[1]], cp_w[2:], [cp_fk] + cp_ssm[1])):
            @pl.when(i == when)
            def _():
                for c in cs:
                    c.start()
        cp_x(i).wait()
        xs = (_chain([x_block(4 * i + u) for u in range(4)]), 4 * NT, X_LEAD, X_LAST)
        overlap(xs, *gen_streams(i, 1, X_SERIAL), gap=X_GAP, lag=X_LAG)
    _loop(4, first)
    for c in cp_ssm[2] + cp_out:
        c.start()
    for c in cp_w:
        c.wait()
    ws = (_chain([w_qkv(s) for s in range(3)]), 6 * NT * NT, 0.0, 1.0)
    overlap((kmats(0, 32), 1920, LEAD, LAST), ws, lag=PW_LAG)
    overlap((qkv(0, 0, QR), cq, 0.0, 1.0), (taps(0), 5, 0.0, 1.0))
    for c in [cp_fk] + cp_ssm[1]:
        c.wait()

    def pws(j, i0, n):
        return (_chain([pointwise(j, i0 + u) for u in range(n)]), n * PW_STEPS, 0.0, 1.0)

    def tile(j):
        @pl.when(j == 1)
        def _():
            for c in cp_ssm[2]:
                c.wait()
        overlap((spectrum_k(), 1024, 0.0, 1.0))
        prep_wide(j + 1, prep(j + 1))

        def expand(i):
            n = 4 // NG
            overlap((qkvs(j, n * i + 1, n, GEN_EVERY), n * cq, LEAD2, LAST2), *gen_streams(n * i, n, GEN_SERIAL), gap=GEN_GAP, lag=GEN_LAG)
        _loop(NG, expand)
        mxu = _chain([kmats(0, 32), qkvs(j, 5, NA, PW_EVERY)])
        overlap((mxu, 1920 + NA * cq, LEAD, LAST), pws(j, 0, PA), gap=PW_GAP, lag=PW_LAG)
        n = nq - 4 - NA
        mxu = _chain([qkvs(j, NA + 5, n - 1, PW_EVERY), qkv(j + 1, 0, PW_EVERY)])
        st = [(mxu, n * cq, LEAD, LAST), pws(j, PA, 16 - PA)]
        overlap(*st, (taps(j + 1), 5, 0.0, TAP_LAST), gap=PW_GAP, lag=PW_LAG)
    _loop(NT - 1, tile)

    j = NT - 1
    for c in cp_out:
        c.wait()
    mxu = _chain([spectrum_k(), qkvs(j, 1, HEAD - 1, 64)])
    st = [(mxu, 1024 + cq * (HEAD - 1), LEAD, LAST), (attend(0, FIRST, True), FIRST + 3, 0.0, 1.0)]
    overlap(*st, (w_out(), NT, 0.0, 1.0), lag=PW_LAG)
    n = (nq - HEAD) // NL

    def last_conv(i):
        r0 = pl.multiple_of(8 * (FIRST + i * EARLY), 16)
        st = [(qkvs(j, HEAD + n * i, n, PW_EVERY), cq * n, LEAD, LAST), pws(j, 16 // NL * i, 16 // NL)]
        overlap(*st, (attend(r0, EARLY), EARLY + 3, 0.0, 1.0), gap=PW_GAP, lag=PW_LAG)
    _loop(NL, last_conv)

    done, nr = FIRST + NL * EARLY, S // RB
    n_mixed = (S // 8 - done) // PER_ROW
    assert n * NL + HEAD == nq and done + n_mixed * PER_ROW == S // 8 and n_mixed == nr - 1
    assert 8 * FIRST <= QR and FIRST % 2 == EARLY % 2 == PER_ROW % 2 == 0
    assert all(8 * (FIRST + EARLY * (i + 1)) <= (HEAD + n * i) * QR for i in range(NL))
    assert all(8 * (done + PER_ROW * i) >= (i + 1) * RB for i in range(n_mixed + 1))
    stage(0)

    def rows(i):
        r0 = pl.multiple_of(8 * (done + PER_ROW * i), 16)
        overlap((mix(i), NT * RB * 7 // 4, MIX_LEAD, MIX_LAST),
                (attend(r0, PER_ROW), 100 * PER_ROW + 300, 0.0, 1.0), lag=1)
        stage(i + 1)
        out_copy(i).start()
    _loop(nr - 1, rows)
    overlap((mix(nr - 1), 1, 0.0, 1.0))
    for i in range(nr - 1):
        out_copy(i).wait()
    for ct in range(NT):
        tail_copy(ct).wait()


@jax.jit
def pallas_gated_mix__sliding_local_dilated__ssm_conv_s4__prompt_kernel(
    A_x: jax.Array,
    A_wqkv: jax.Array,
    A_wo: jax.Array,
    B_u: jax.Array,
    B_A_re: jax.Array,
    B_A_im: jax.Array,
    B_B_re: jax.Array,
    B_B_im: jax.Array,
    B_C_re: jax.Array,
    B_C_im: jax.Array,
    B_log_dt: jax.Array,
    B_Dskip: jax.Array,
    gate_w: jax.Array,
):
    del B_u
    fx, g, fk = _constants()
    vm = pltpu.VMEM
    hbm = pl.BlockSpec(memory_space=pl.ANY)
    out = pl.pallas_call(
        _kernel,
        out_shape=jax.ShapeDtypeStruct((S, D), BF16),
        in_specs=[hbm] * 15,
        out_specs=hbm,
        scratch_shapes=[
            vm((S, D), BF16), vm((D, 3 * D), BF16), vm((D, D), BF16), vm((6, N, D), BF16),
            vm(fx.shape, U32), vm(g.shape, U32), vm(fk.shape, U32), vm((S, D), BF16),
            vm((NT, S // 2, T), U32), vm((S, T), F32),
            vm((3, NT, D // 2, T), U32), vm((NT, NT, 3 * T // 2, T), U32), vm((NT, D // 2, T), U32),
            vm((4, N, T), F32), vm((3, NU * 4 * GS, T), U32), vm((3, NV * 4 * GS, T), U32),
            vm((2, T, T), F32), vm((32 * KS, T), F32), vm((max(_SLOT) + 1, T // 2, T), U32),
            vm((NB, SPEC, T), F32), vm((NT, NB, SPEC, T), F32), vm((NT, NB, T, T), U32),
            vm((2 * NB, 8, T), F32),
            vm((NT, S, T), F32), vm((NT, S + HALO, T), F32), vm((NT, S + HALO, T), F32),
            vm((NT, S, T), F32), vm((NT, RB // 2, T), U32), vm((NT, RB, T), F32), vm((8, T), F32),
            vm((3, 1, D), F32), vm((D,), BF16), vm((D,), BF16), vm((D,), BF16),
            pltpu.SemaphoreType.DMA((N_COPIES,)), pltpu.SemaphoreType.DMA((4,)),
             pltpu.SemaphoreType.DMA(()),
        ],
        compiler_params=pltpu.CompilerParams(vmem_limit_bytes=100 * 1024 * 1024),
    )(A_x.reshape(S, D), A_wqkv, A_wo, B_A_re.T, B_A_im.T, B_B_re.T, B_B_im.T, B_C_re.T, B_C_im.T,
      B_log_dt, B_Dskip, gate_w, fx, g, fk)
    return out.reshape(1, S, D)
```

```python
import jax
import jax.numpy as jnp
import numpy as np
import jax.experimental.pallas as pl
import jax.experimental.pallas.tpu as pltpu

S, D, H, DH, N = 2048, 640, 32, 20, 192
WIN, DIL = 8, 2
T = 128
NT = D // T
NB = S // T
HALO = 32
N_COPIES = 28
SINCOS_MAX = 8192.0
LEAD = 0.04
LEAD2 = 0.03
LAST = 0.98
LAST2 = 0.98
QR = 256
HEAD = 2
NL = 2
FIRST = 28
EARLY = 16
RB = 256
PER_ROW = 28
GEN_SERIAL = True
FK_EVERY = 256
KMAT_EVERY = 40
PW_EVERY = 16
GEN_EVERY = 8
MIX_EVERY = 32
MIX_LEAD = 0.05
MIX_LAST = 1.0
PACE_K = ()
PACE_V = (0,)
X_LAG = 8
X_SERIAL = True
X_GAP = 1
X_EVERY = 32
X_LEAD = 0.1
X_LAST = 0.95
GEN_GAP = 1
PW_GAP = 2
PW_SPLIT = 8
KEEP = 32
NG = 1
NA = 1
PA = 8
TAP_LAST = 0.8
GEN_LAG = 6
PW_LAG = 4
IM = 144
SPEC = 280
NU, NV = 10, 16
GS = 36
KS = 84
F32, BF16, U32 = jnp.float32, jnp.bfloat16, jnp.uint32

_BASES = [0, 1, 2, 3, 4, 5, 6, 7, 256, 258, 260, 262, 512, 516, 768, 772,
          1024, 1280, 1536, 1792]


_TAPS = {2: (2, 0, None), 3: (2, 0, 0),
         4: (3, 0, None), 5: (3, 0, None), 6: (3, T - 4, None), 7: (3, T - 4, 4)}
_TAPS.update({m: (4, (8 - m + m % 2) % T, 2 if m == NB - 1 else None) for m in range(8, NB)})
_SLOT = [0, 1, 2, 3] + [4 + (m - 4) // 2 for m in range(4, NB)]
_SHARE = [0, 0, 1, 2, 3, 4, 3, 4] + [5, 6] * 4


def _pack_rows(a):
    b = a.astype(np.float32).astype(BF16).view(np.uint16).astype(np.uint32)
    return b[..., 0::2, :] | (b[..., 1::2, :] << 16)


def _constants():
    om = 2.0 * np.pi * (np.arange(T) + 0.25) / T
    ph = np.exp(-1j * om[:, None] * np.arange(T)[None, :])
    fx = np.concatenate([ph.real, ph.imag], 0)
    g = np.stack([ph.real.T, ph.imag.T], -1).reshape(T, 2 * T) / T
    lag = np.arange(S).astype(np.float32).astype(BF16).astype(np.float32).astype(np.int64)
    lane = np.arange(T)
    off = 8 * (2 * (lane // 8) + lane % 2)
    tiles = [np.array(_BASES[4 * t:4 * t + 4])[(lane % 8) // 2] + off for t in range(5)]
    lo = lane < T // 2
    vals = [np.where(lo, tiles[0], np.roll(tiles[1], T // 2)),
            np.where(lo, np.roll(tiles[0], T // 2), tiles[1])]
    for m in range(2, NB):
        t, shift, end = _TAPS[m]
        v = np.roll(tiles[t], shift)
        vals.append(v if end is None else np.where(lane == end, (m + 1) * T, v))
    fk = np.zeros((max(_SHARE) + 1, 2 * T, T))
    for m in range(NB):
        blk = lag[m * T:(m + 1) * T]
        e = (blk[:, None] == vals[m][None, :]).astype(np.float64)
        assert (e.sum(1) == 1).all()
        c = np.concatenate([(ph @ e).real, (ph @ e).imag], 0)
        assert _SHARE.index(_SHARE[m]) == m or np.array_equal(fk[_SHARE[m]], c)
        fk[_SHARE[m]] = c
    g = np.stack([g[:, :T], g[:, T:]])
    return _pack_rows(fx), _pack_rows(g), _pack_rows(fk)


def _cmul(a, b):
    return a[0] * b[0] - a[1] * b[1], a[0] * b[1] + a[1] * b[0]


def _times(f, conj=False):
    dif, tot = f[1] - f[0], f[1] + f[0]

    def mul(a):
        k = f[0] * (a[0] + a[1])
        if conj:
            return k + a[1] * dif, k - a[0] * tot
        return k - a[1] * tot, k + a[0] * dif
    return mul


def _csq(a):
    t = a[0] * a[1]
    return a[0] * a[0] - a[1] * a[1], t + t


def _tree(op, xs):
    while len(xs) > 1:
        xs = [op(a, b) for a, b in zip(xs[0::2], xs[1::2])]
    return xs[0]


def _pack(a, b):
    return pltpu.pack_elementwise([a, b], packed_dtype=BF16)


def _words(a):
    return pltpu.bitcast(a.astype(BF16), U32)


def _halves(a):
    return pltpu.bitcast(a, BF16)


def _dot(a, b):
    return jnp.dot(a, b, preferred_element_type=F32)


def _dot_nt(a, b):
    return jax.lax.dot_general(a, b, (((1,), (1,)), ((), ())), preferred_element_type=F32)


def _sincos(x):
    k = jnp.floor(x * (2.0 / np.pi) + 0.5)
    r = ((x - k * 1.5703125) - k * 4.837512969970703125e-4) - k * 7.54978995489188216e-8
    z = r * r
    s = r + r * z * (-1.6666654611e-1 + z * (8.3321608736e-3 + z * -1.9515295891e-4))
    c = 1.0 + z * (-0.5 + z * (4.166664568298827e-2
                               + z * (-1.388731625493765e-3 + z * 2.443315711809948e-5)))
    n = k.astype(jnp.int32)
    odd = (n & 1) == 1
    s, c = jnp.where(odd, c, s), jnp.where(odd, s, c)
    return jnp.where((n & 2) == 2, -s, s), jnp.where(((n + 1) & 2) == 2, -c, c)


def _aligned(i, n):
    return i if isinstance(i, int) else pl.multiple_of(i, n)


def _loop(n, body):
    jax.lax.fori_loop(0, n, lambda i, c: body(i), None)


def _interleave(*streams):
    done = [0] * len(streams)
    live = list(range(len(streams)))
    while live:
        i = min(live, key=lambda n: streams[n][2]
                + (streams[n][3] - streams[n][2]) * done[n] / streams[n][1])
        work = next(streams[i][0], None)
        if work is None:
            live.remove(i)
        else:
            done[i] += work


def _chain(gens):
    for g in gens:
        yield from g


def _kernel(x_hbm, wqkv_hbm, wo_hbm, are_hbm, aim_hbm, bre_hbm, bim_hbm, cre_hbm, cim_hbm,
            ldt_hbm, dsk_hbm, gw_hbm, fx_hbm, g_hbm, fk_hbm, o_hbm,
            x_ref, wqkv_ref, wo_ref, ssm_ref, fx_ref, g_ref, fk_ref, o_ref,
            xs_s, gate_s, wt_s, wp_s, wop_s, par_s, us_s, vs_s, kend_s, ko_s, kt_s,
            kh_s, xh_s, yh_s, tmp_s, q_s, k_s, v_s, at_s, cur_s, y_s, zero_s, vec_s, ldt_in, dsk_in, gw_in,
            sems, xsems, osem):
    lane = jax.lax.broadcasted_iota(jnp.int32, (8, T), 1)
    lo = lane < T // 2

    ldt_ref, dsk_ref, gw_ref = vec_s.at[0], vec_s.at[1], vec_s.at[2]
    ssm_hbm = (are_hbm, aim_hbm, bre_hbm, bim_hbm, cre_hbm, cim_hbm)
    sem_ids = iter(range(N_COPIES))
    copy = lambda a, b: pltpu.make_async_copy(a, b, sems.at[next(sem_ids)])
    cp_ssm = [[copy(h.at[:, a:b], ssm_ref.at[i, :, a:b]) for i, h in enumerate(ssm_hbm)]
              for a, b in ((0, T), (T, 2 * T), (2 * T, D))]
    cp_fx = copy(fx_hbm, fx_ref)
    cp_vec = [copy(ldt_hbm, ldt_in), copy(dsk_hbm, dsk_in), copy(gw_hbm, gw_in)]

    def cp_x(i):
        rows = pl.ds(_aligned(i * (S // 4), S // 4), S // 4)
        return pltpu.make_async_copy(x_hbm.at[rows, :], x_ref.at[rows, :], xsems.at[i])
    cp_w = [copy(wqkv_hbm.at[:, s * D:(s + 1) * D], wqkv_ref.at[:, s * D:(s + 1) * D]) for s in range(3)]
    cp_fk = copy(fk_hbm, fk_ref)
    cp_out = [copy(wo_hbm, wo_ref), copy(g_hbm, g_ref)]
    for c in cp_vec + cp_ssm[0] + [cp_fx, cp_x(0), cp_x(1)]:
        c.start()

    tokens, always = [], []

    def post(a, every):
        tokens[:] = tokens[-KEEP:] + [a[r - 8:r] for r in range(every, a.shape[0] + 1, every)]

    def pace(x):
        always[2] += 1
        if len(tokens) <= always[3] or always[2] < always[1]:
            return x
        always[2] = 0
        head = jnp.where(always[0], x[:8], pltpu.bitcast(tokens.pop(0), x.dtype))
        return head if x.shape[0] == 8 else jnp.concatenate([head, x[8:]], 0)

    def x_block(m):
        r0, h0 = _aligned(m * T, T), _aligned(m * (T // 2), T // 2)
        acc = None
        for t in range(NT):
            x = x_ref[pl.ds(r0, T), t * T:(t + 1) * T]
            xs_s[t, pl.ds(h0, T // 2), :] = pltpu.bitcast(x, U32)
            r = _dot(_halves(fx_ref[...]), x)
            xh_s[t, m, 0:T, :] = r[:T]
            xh_s[t, m, IM:IM + T, :] = r[T:]
            post(r, X_EVERY)
            xg = x.astype(F32) * gw_ref[:, t * T:(t + 1) * T]
            acc = xg if acc is None else acc + xg
            yield 64
        gate = jax.nn.sigmoid(jnp.sum(acc, axis=1, keepdims=True))
        gate_s[pl.ds(r0, T), :] = jnp.broadcast_to(gate, (T, T))

    def regroup(src, t):
        rows = []
        for i in range(2):
            ab = [src[pl.ds(2 * t + i + h * DH // 2, H // 2, stride=DH), :] for h in range(2)]
            ab[0] = pace(ab[0]) if i == 0 else ab[0]
            rows += [_pack(*[pltpu.unpack_elementwise(w, index=e, packed_dtype=BF16, unpacked_dtype=F32)
                             for w in ab]) for e in range(2)]
        return jnp.concatenate(rows, 0)

    def w_qkv(s):
        for c in range(NT):
            for kt in range(NT):
                w = wqkv_ref[kt * T:(kt + 1) * T, s * D + c * T:s * D + (c + 1) * T]
                wt_s[s, kt, c * (T // 2):(c + 1) * (T // 2), :] = pltpu.bitcast(w.T, U32)
                yield 1
        for t in range(NT):
            for kt in range(NT):
                wp_s[t, kt, s * (T // 2):(s + 1) * (T // 2), :] = regroup(wt_s.at[s, kt], t)
                yield 1

    def w_out():
        for ct in range(NT):
            wt_s[0, ct] = pltpu.bitcast(wo_ref[:, ct * T:(ct + 1) * T], U32)
            for t in range(NT):
                wop_s[ct, t * (T // 2):(t + 1) * (T // 2), :] = regroup(wt_s.at[0, ct], t)
            yield 1

    def put_par(i, a):
        par_s[i, 0:T, :] = a[0:T].T
        hi = a[T:N]
        par_s[i, T:N, :] = jnp.concatenate(
            [hi, pltpu.roll(hi, T // 2, 1)], 0).T[0:T // 2]

    def discretize(j):
        c0 = j * T if isinstance(j, int) else pl.multiple_of(j * T, T)
        dt = jnp.exp(ldt_ref[:, pl.ds(c0, T)].astype(F32)).astype(BF16).astype(F32)
        load = lambda i: ssm_ref[i, :, pl.ds(c0, T)].astype(F32)
        return dt, load, jnp.exp(dt * load(0)), dt * load(1)

    def prep(j):
        dt, load, mag, ang = discretize(j)
        sin, cos = _sincos(ang)
        w = _cmul((load(4), load(5)), (dt * load(2), dt * load(3)))
        for i, a in enumerate((mag * cos, mag * sin, w[0], -w[1])):
            put_par(i, a)
        return jnp.max(jnp.abs(ang))

    def prep_wide(j, ang_max):
        def redo(_):
            _, _, mag, ang = discretize(j)
            put_par(0, mag * jnp.cos(ang))
            put_par(1, mag * jnp.sin(ang))
        _loop(jnp.where(ang_max <= SINCOS_MAX, 0, 1), redo)

    GEN_STEPS = 28

    def gen(r, hi):
        r0 = r * 8 if isinstance(r, int) else pl.multiple_of(r * 8, 8)
        d0 = (r // 4) * GS + (r % 4) * 8
        s0 = T + r0 if hi else r0

        def put(dst, i, a, b):
            re, im = _pack(a[0], b[0]), _pack(a[1], b[1])
            if hi:
                t = pltpu.roll(jnp.where(lo, im, re), T // 2, 1)
                dst[2, pl.ds(i * 4 * GS + d0, 8), :] = jnp.where(lo, re, t)
                dst[2, pl.ds(i * 4 * GS + 2 * GS + d0, 8), :] = jnp.where(lo, t, im)
            else:
                dst[0, pl.ds(i * 4 * GS + d0, 8), :] = re
                dst[1, pl.ds(i * 4 * GS + d0, 8), :] = im

        p = (par_s[0, pl.ds(s0, 8), :], par_s[1, pl.ds(s0, 8), :])
        p2 = _csq(p)
        p4 = _csq(p2)
        q = _csq(p4)
        q2 = _csq(q)
        q4 = _csq(q2)
        yield 1
        v = [(jnp.ones_like(q[0]), jnp.zeros_like(q[0])), q, q2, _cmul(q, q2)]
        by_q4 = _times(q4)
        for i in range(NV // 2):
            put(vs_s, 2 * i, v[0], v[1])
            yield 1
            put(vs_s, 2 * i + 1, v[2], v[3])
            if i == 0:
                v = [q4] + [by_q4(a) for a in v[1:]]
            elif i < NV // 2 - 1:
                v = [by_q4((pace(v[0][0]), v[0][1]))] + [by_q4(a) for a in v[1:]]
            yield 1
        b1 = by_q4(v[0])
        u = [(par_s[2, pl.ds(s0, 8), :], par_s[3, pl.ds(s0, 8), :])]
        u += [_times(p, True)(u[0])]
        put(us_s, 0, u[0], u[1])
        yield 1
        fs, by = [p2, p4, b1], []
        for i, (a, b, f) in enumerate(((0, 1, 0), (0, 1, 1), (2, 3, 1), (0, 2, 2), (4, 6, 2),
                                       (0, 4, 3), (8, 10, 3), (0, 8, 4), (12, 14, 4))):
            if f == len(fs):
                fs.append(_csq(fs[-1]))
            if f == len(by):
                by.append(_times(fs[f], True))
            u += [by[f]((pace(u[a][0]), u[a][1])), by[f](u[b])]
            put(us_s, 1 + i, u[-2], u[-1])
            yield 1
        last = u[16][0] * fs[4][0] + u[16][1] * fs[4][1]
        if hi:
            kend_s[1, pl.ds(r0, 8), :] = jnp.where(lo, last, 0.0)
            kend_s[1, pl.ds(T // 2 + r0, 8), :] = jnp.where(lo, 0.0, last)
        else:
            kend_s[0, pl.ds(r0, 8), :] = last
        yield 1

    def kmat(g):
        u = jnp.concatenate([_halves(us_s[t, pl.ds(g, 4 * NU, stride=GS), :]) for t in range(3)], 1)
        v = jnp.concatenate([_halves(vs_s[t, pl.ds(g, 4 * NV, stride=GS), :]) for t in range(3)], 1)
        r = _dot_nt(u, v)
        ko_s[pl.ds(g * KS, 8 * NU), :] = r
        post(r, KMAT_EVERY)

    def taps(j):
        lane32 = jax.lax.broadcasted_iota(jnp.int32, (32, T), 1)
        slot = (lane32 % 8) // 2

        def gather(t):
            parts = []
            for c in range(4):
                acc = None
                for jj in range(4):
                    k = 4 * t + jj
                    a = ko_s[pl.ds((k // 2) * 8 + 2 * c + k % 2, 32, stride=KS), :]
                    if jj != c:
                        a = pltpu.roll(a, (2 * (jj - c)) % T, 1)
                    acc = a if acc is None else jnp.where(slot == jj, a, acc)
                parts.append(acc)
            return jnp.concatenate(parts, 0)

        def emit(ms, taps):
            kt_s[_SLOT[ms[0]]] = _words(taps)

        lane_t = jax.lax.broadcasted_iota(jnp.int32, (T, T), 1)
        lo_t, first = lane_t < T // 2, lane_t == 0
        t4 = gather(4)
        emit([8, 9], t4)
        for m in (10, 12):
            emit([m, m + 1], pltpu.roll(t4, _TAPS[m][1], 1))
        kend = jnp.sum(kend_s[0] + kend_s[1], axis=1, keepdims=True)
        emit([14, 15], jnp.where(lane_t == 2, kend, pltpu.roll(t4, _TAPS[14][1], 1)))
        yield 1
        t3 = gather(3)
        emit([4, 5], t3)
        emit([6, 7], jnp.where(lane_t == 4, pltpu.roll(t4, 4, 1), pltpu.roll(t3, _TAPS[6][1], 1)))
        yield 1
        t2 = gather(2)
        emit([2], t2)
        emit([3], jnp.where(first, t3, t2))
        yield 1
        t1 = gather(1)
        yield 1
        t0 = gather(0)
        x = pltpu.roll(jnp.where(lo_t, t1, t0), T // 2, 1)
        emit([1], jnp.where(lo_t, x, t1))
        skip = dsk_ref[:, pl.ds(j * T if isinstance(j, int) else pl.multiple_of(j * T, T), T)].astype(F32)
        skip = jnp.broadcast_to(skip, (T, T)).T
        emit([0], jnp.where(lo_t, t0, x) + jnp.where(first, skip, 0.0))
        yield 1

    def spectrum_k():
        for m in range(NB):
            r = _dot_nt(_halves(fk_ref[_SHARE[m]]), _halves(kt_s[_SLOT[m]]))
            kh_s[m, 0:T, :] = r[:T]
            kh_s[m, IM:IM + T, :] = r[T:]
            post(r, FK_EVERY)
            yield 64

    PW_STEPS = 3 * NB * (NB + 1) // 2

    def pointwise(j, i):
        r0 = _aligned(i * 8, 8)

        def part(ref, m, c):
            if c < 2:
                return ref[m, pl.ds(c * IM + r0, 8), :]
            return part(ref, m, 0) + part(ref, m, 1)

        prev = None
        for c in range(3):
            for p0 in range(0, NB, PW_SPLIT):
                ps = range(p0, p0 + PW_SPLIT)
                xs, acc = {}, {}
                for m in range(p0 + PW_SPLIT):
                    k = part(kh_s, m, c)
                    if m % 2 == 0:
                        k = pace(k)
                    for p in ps:
                        if p >= m:
                            if p - m not in xs:
                                xs[p - m] = part(xh_s.at[j], p - m, c)
                            kx = k * xs[p - m]
                            acc[p] = kx + acc[p] if m else kx - tmp_s[p] if c == 2 else kx
                    yield min(p0 + PW_SPLIT - m, PW_SPLIT)
                for p in ps:
                    if c == 0:
                        tmp_s[p] = acc[p]
                    elif c == 1:
                        rr = tmp_s[p]
                        tmp_s[NB + p] = rr - acc[p]
                        tmp_s[p] = rr + acc[p]
                    else:
                        y = (tmp_s[NB + p], acc[p])
                        z = y if prev is None else (y[0] - prev[1], y[1] + prev[0])
                        yh_s[j, p, pl.ds(r0, 8), :] = _pack(*z)
                        prev = y

    qscale = float(DH ** -0.5 * np.log2(np.e))

    def qkv(j, i, every):
        r0, h0 = i * QR, i * (QR // 2)
        if not isinstance(i, int):
            r0, h0 = pl.multiple_of(r0, QR), pl.multiple_of(h0, QR // 2)
        for s in range(3):
            x = jnp.concatenate([_halves(xs_s[t, pl.ds(h0, QR // 2), :]) for t in range(NT)], 1)
            w = jnp.concatenate([_halves(wp_s[j, t, s * (T // 2):(s + 1) * (T // 2), :])
                                 for t in range(NT)], 1)
            acc = _dot_nt(x, w)
            if s == 0:
                q_s[j, pl.ds(r0, QR), :] = acc * qscale
            else:
                (k_s, v_s)[s - 1][j, pl.ds(HALO + r0, QR), :] = acc
            post(acc, every)
            yield QR * 5 // 4

    def window(r0, masked):
        rows = lambda r: pl.ds(r, 8)
        qs = [q_s[t, rows(r0), :] for t in range(NT)]
        ls = []
        for w in range(WIN):
            a = None
            for t in range(NT):
                k = k_s[t, rows(r0 + HALO - DIL * w), :]
                kq = qs[t] * (pace(k) if t == 0 and w in PACE_K else k)
                a = kq if a is None else a + kq
            ls.append((a, pltpu.roll(a, 64, 1)))
        yield 1
        ls = [a + b for a, b in ls]
        ls = [(a, pltpu.roll(a, 32, 1)) for a in ls]
        yield 1
        ls = [a + b for a, b in ls]
        if masked:
            row = jax.lax.broadcasted_iota(jnp.int32, (8, T), 0) + r0
            ls = [jnp.where(row >= DIL * w, a, -1e9 * np.log2(np.e)) for w, a in enumerate(ls)]
        mx = _tree(jnp.maximum, ls)
        es = [jnp.exp2(a - mx) for a in ls]
        yield 1
        inv = gate_s[rows(r0), :] * pl.reciprocal(_tree(jnp.add, es), full_range=False)
        outs = []
        for t in range(NT):
            a = None
            for w in range(WIN):
                v = v_s[t, rows(r0 + HALO - DIL * w), :]
                pv = es[w] * (pace(v) if w == 0 and t in PACE_V else v)
                a = pv if a is None else a + pv
            outs.append(a)
        for t in range(NT):
            at_s[t, rows(r0), :] = outs[t] * inv
        yield 1

    def attend(r0, n, first=False):
        gens = [window(r0 + 8 * c, first and 8 * c < DIL * WIN) for c in range(n)]
        for step in range(n + 3):
            for c in range(step, step - 4, -1):
                if 0 <= c < n:
                    next(gens[c])
            yield 1

    def stage(i):
        r0 = _aligned(i * RB, RB)
        for t in range(NT):
            cur_s[t] = _pack(*[at_s[t, pl.ds(r0 + e, RB // 2, stride=2), :] for e in range(2)])

    def out_copy(i):
        r0 = _aligned(i * RB, RB)
        return pltpu.make_async_copy(o_ref.at[pl.ds(r0, RB), :], o_hbm.at[pl.ds(r0, RB), :], osem)

    def tail_copy(ct):
        part = (slice(S - RB, S), slice(ct * T, (ct + 1) * T))
        return pltpu.make_async_copy(o_ref.at[part], o_hbm.at[part], osem)

    def mix(i):
        r0 = _aligned(i * RB, RB)
        for ct in range(NT):
            for h in range(RB // T):
                y = _dot(jnp.concatenate([_halves(g_ref[b]) for b in range(2)], 1),
                         _halves(yh_s[ct, i * (RB // T) + h]))
                y_s[ct, h * T:(h + 1) * T, :] = (1.0 - gate_s[pl.ds(r0 + h * T, T), :]) * y
                post(y, T)
                yield 64
        for ct in range(NT):
            yield from project(r0, ct)

    def project(r0, ct):
        a = _dot(jnp.concatenate([_halves(cur_s[t]) for t in range(NT)], 1), _halves(wop_s[ct]))
        acc = a + y_s[ct]
        o_ref[pl.ds(r0, RB), ct * T:(ct + 1) * T] = acc.astype(BF16)
        if isinstance(r0, int):
            tail_copy(ct).start()
        post(acc, MIX_EVERY)
        yield RB * 5 // 4

    def gen_streams(i0, n, serial):
        units = lambda i, u: [gen(4 * i + 2 * u, False), gen(4 * i + 2 * u + 1, False), gen(2 * i + u, True)]
        if serial:
            return [(_chain([g for i in range(n) for u in range(2) for g in units(i0 + i, u)]),
                     6 * n * GEN_STEPS, 0.0, 1.0)]
        return [(_chain([g for i in range(n) for g in units(i0 + i, u)]), 3 * n * GEN_STEPS, 0.0, 1.0)
                for u in range(2)]

    def qkvs(j, i0, n, every):
        return _chain([qkv(j, i0 + u, every) for u in range(n)])

    def kmats(g0, n):
        for u in range(n):
            kmat(g0 + u)
            yield 60

    def overlap(*streams, gap=1, lag=0):
        always[:] = [zero_s[...] == 0.0, gap, 0, lag]
        _interleave(*streams)
        tokens.clear()
        always.clear()

    nq, cq = S // QR, QR * 15 // 4

    for t in range(NT):
        k_s[t, 0:HALO, :] = jnp.zeros((HALO, T), F32)
        v_s[t, 0:HALO, :] = jnp.zeros((HALO, T), F32)
    zero_s[...] = jnp.zeros((8, T), F32)
    for c in cp_vec + cp_ssm[0]:
        c.wait()
    for i, ref in enumerate((ldt_in, dsk_in, gw_in)):
        vec_s[i] = ref[...].astype(F32).reshape(1, D)
    prep_wide(0, prep(0))
    cp_fx.wait()

    def first(i):
        for when, cs in enumerate(([cp_x(2)], [cp_w[0]], [cp_x(3)], [cp_w[1]])):
            @pl.when(i == when)
            def _():
                for c in cs:
                    c.start()

        @pl.when(i % 2 == 0)
        def _():
            cp_x(i // 2).wait()
        xs = (_chain([x_block(2 * i + u) for u in range(2)]), 128 * NT, X_LEAD, X_LAST)
        overlap(xs, *gen_streams(i, 1, X_SERIAL), gap=X_GAP, lag=X_LAG)
    _loop(4, first)
    late = ([cp_w[2]], [cp_fk] + cp_ssm[1], cp_ssm[2] + cp_out)
    for s, (g0, g1, m0, m1) in enumerate(((0, 16, 8, 10), (16, 32, 10, 12), (32, 32, 12, NB))):
        for c in late[s]:
            c.start()
        cp_w[s].wait()
        if m0 % 4 == 0:
            cp_x(m0 // 4).wait()
        mxu = _chain([kmats(g0, g1 - g0)] + [x_block(m) for m in range(m0, m1)])
        overlap((mxu, 60 * (g1 - g0) + 64 * NT * (m1 - m0), LEAD, LAST),
                (w_qkv(s), 2 * NT * NT, 0.0, 1.0), lag=PW_LAG)
    overlap((qkv(0, 0, QR), cq, 0.0, 1.0), (taps(0), 5, 0.0, 1.0))
    for c in [cp_fk] + cp_ssm[1]:
        c.wait()

    def pws(j, i0, n):
        return (_chain([pointwise(j, i0 + u) for u in range(n)]), n * PW_STEPS, 0.0, 1.0)

    def tile(j):
        @pl.when(j == 1)
        def _():
            for c in cp_ssm[2]:
                c.wait()
        overlap((spectrum_k(), 1024, 0.0, 1.0))
        prep_wide(j + 1, prep(j + 1))

        def expand(i):
            n = 4 // NG
            overlap((qkvs(j, n * i + 1, n, GEN_EVERY), n * cq, LEAD2, LAST2), *gen_streams(n * i, n, GEN_SERIAL), gap=GEN_GAP, lag=GEN_LAG)
        _loop(NG, expand)
        mxu = _chain([kmats(0, 32), qkvs(j, 5, NA, PW_EVERY)])
        overlap((mxu, 1920 + NA * cq, LEAD, LAST), pws(j, 0, PA), gap=PW_GAP, lag=PW_LAG)
        n = nq - 4 - NA
        mxu = _chain([qkvs(j, NA + 5, n - 1, PW_EVERY), qkv(j + 1, 0, PW_EVERY)])
        st = [(mxu, n * cq, LEAD, LAST), pws(j, PA, 16 - PA)]
        overlap(*st, (taps(j + 1), 5, 0.0, TAP_LAST), gap=PW_GAP, lag=PW_LAG)
    _loop(NT - 1, tile)

    j = NT - 1
    for c in cp_out:
        c.wait()
    mxu = _chain([spectrum_k(), qkvs(j, 1, HEAD - 1, 64)])
    st = [(mxu, 1024 + cq * (HEAD - 1), LEAD, LAST), (attend(0, FIRST, True), FIRST + 3, 0.0, 1.0)]
    overlap(*st, (w_out(), NT, 0.0, 1.0), lag=PW_LAG)
    n = (nq - HEAD) // NL

    def last_conv(i):
        r0 = pl.multiple_of(8 * (FIRST + i * EARLY), 16)
        st = [(qkvs(j, HEAD + n * i, n, PW_EVERY), cq * n, LEAD, LAST), pws(j, 16 // NL * i, 16 // NL)]
        overlap(*st, (attend(r0, EARLY), EARLY + 3, 0.0, 1.0), gap=PW_GAP, lag=PW_LAG)
    _loop(NL, last_conv)

    done, nr = FIRST + NL * EARLY, S // RB
    n_mixed = (S // 8 - done) // PER_ROW
    assert n * NL + HEAD == nq and done + n_mixed * PER_ROW == S // 8 and n_mixed == nr - 1
    assert 8 * FIRST <= QR and FIRST % 2 == EARLY % 2 == PER_ROW % 2 == 0
    assert all(8 * (FIRST + EARLY * (i + 1)) <= (HEAD + n * i) * QR for i in range(NL))
    assert all(8 * (done + PER_ROW * i) >= (i + 1) * RB for i in range(n_mixed + 1))
    stage(0)

    def rows(i):
        r0 = pl.multiple_of(8 * (done + PER_ROW * i), 16)
        overlap((mix(i), NT * RB * 7 // 4, MIX_LEAD, MIX_LAST),
                (attend(r0, PER_ROW), 100 * PER_ROW + 300, 0.0, 1.0), lag=1)
        stage(i + 1)
        out_copy(i).start()
    _loop(nr - 1, rows)
    overlap((mix(nr - 1), 1, 0.0, 1.0))
    for i in range(nr - 1):
        out_copy(i).wait()
    for ct in range(NT):
        tail_copy(ct).wait()


@jax.jit
def pallas_gated_mix__sliding_local_dilated__ssm_conv_s4__prompt_kernel(
    A_x: jax.Array,
    A_wqkv: jax.Array,
    A_wo: jax.Array,
    B_u: jax.Array,
    B_A_re: jax.Array,
    B_A_im: jax.Array,
    B_B_re: jax.Array,
    B_B_im: jax.Array,
    B_C_re: jax.Array,
    B_C_im: jax.Array,
    B_log_dt: jax.Array,
    B_Dskip: jax.Array,
    gate_w: jax.Array,
):
    del B_u
    fx, g, fk = _constants()
    vm = pltpu.VMEM
    hbm = pl.BlockSpec(memory_space=pl.ANY)
    out = pl.pallas_call(
        _kernel,
        out_shape=jax.ShapeDtypeStruct((S, D), BF16),
        in_specs=[hbm] * 15,
        out_specs=hbm,
        scratch_shapes=[
            vm((S, D), BF16), vm((D, 3 * D), BF16), vm((D, D), BF16), vm((6, N, D), BF16),
            vm(fx.shape, U32), vm(g.shape, U32), vm(fk.shape, U32), vm((S, D), BF16),
            vm((NT, S // 2, T), U32), vm((S, T), F32),
            vm((3, NT, D // 2, T), U32), vm((NT, NT, 3 * T // 2, T), U32), vm((NT, D // 2, T), U32),
            vm((4, N, T), F32), vm((3, NU * 4 * GS, T), U32), vm((3, NV * 4 * GS, T), U32),
            vm((2, T, T), F32), vm((32 * KS, T), F32), vm((max(_SLOT) + 1, T // 2, T), U32),
            vm((NB, SPEC, T), F32), vm((NT, NB, SPEC, T), F32), vm((NT, NB, T, T), U32),
            vm((2 * NB, 8, T), F32),
            vm((NT, S, T), F32), vm((NT, S + HALO, T), F32), vm((NT, S + HALO, T), F32),
            vm((NT, S, T), F32), vm((NT, RB // 2, T), U32), vm((NT, RB, T), F32), vm((8, T), F32),
            vm((3, 1, D), F32), vm((D,), BF16), vm((D,), BF16), vm((D,), BF16),
            pltpu.SemaphoreType.DMA((N_COPIES,)), pltpu.SemaphoreType.DMA((4,)),
             pltpu.SemaphoreType.DMA(()),
        ],
        compiler_params=pltpu.CompilerParams(vmem_limit_bytes=100 * 1024 * 1024),
    )(A_x.reshape(S, D), A_wqkv, A_wo, B_A_re.T, B_A_im.T, B_B_re.T, B_B_im.T, B_C_re.T, B_C_im.T,
      B_log_dt, B_Dskip, gate_w, fx, g, fk)
    return out.reshape(1, S, D)
```

```python
import jax
import jax.numpy as jnp
import numpy as np
import jax.experimental.pallas as pl
import jax.experimental.pallas.tpu as pltpu

S, D, H, DH, N = 2048, 640, 32, 20, 192
WIN, DIL = 8, 2
T = 128
NT = D // T
NB = S // T
HALO = 32
N_COPIES = 28
SINCOS_MAX = 8192.0
QR = 256
RB = 256
IM, SPEC = 144, 280

NA, PA = 1, 8
HEAD, NL = 2, 2
FIRST, EARLY, PER_ROW = 28, 16, 28
LEAD, LAST, LEAD2, LAST2, TAP_LAST = 0.04, 0.98, 0.03, 0.98, 0.8
X_LEAD, X_LAST, X_EVERY, X_GAP, X_LAG = 0.1, 0.95, 32, 1, 8
GEN_EVERY, GEN_GAP, GEN_LAG = 8, 1, 6
PW_EVERY, PW_GAP, PW_LAG, PW_SPLIT = 16, 2, 4, 8
FK_EVERY, KMAT_EVERY, KEEP = 256, 40, 32
MIX_EVERY, MIX_LEAD, MIX_LAST = 64, 0.05, 1.0
NU, NV = 10, 16
GS = 36
KS = 84
F32, BF16, U32 = jnp.float32, jnp.bfloat16, jnp.uint32

_BASES = [0, 1, 2, 3, 4, 5, 6, 7, 256, 258, 260, 262, 512, 516, 768, 772,
          1024, 1280, 1536, 1792]


_TAPS = {2: (2, 0, None), 3: (2, 0, 0),
         4: (3, 0, None), 5: (3, 0, None), 6: (3, T - 4, None), 7: (3, T - 4, 4)}
_TAPS.update({m: (4, (8 - m + m % 2) % T, 2 if m == NB - 1 else None) for m in range(8, NB)})
_SLOT = [0, 1, 2, 3] + [4 + (m - 4) // 2 for m in range(4, NB)]
_SHARE = [0, 0, 1, 2, 3, 4, 3, 4] + [5, 6] * 4


def _pack_rows(a):
    b = a.astype(np.float32).astype(BF16).view(np.uint16).astype(np.uint32)
    return b[..., 0::2, :] | (b[..., 1::2, :] << 16)


def _constants():
    om = 2.0 * np.pi * (np.arange(T) + 0.25) / T
    ph = np.exp(-1j * om[:, None] * np.arange(T)[None, :])
    fx = np.concatenate([ph.real, ph.imag], 0)
    g = np.stack([ph.real.T, ph.imag.T], -1).reshape(T, 2 * T) / T
    lag = np.arange(S).astype(np.float32).astype(BF16).astype(np.float32).astype(np.int64)
    lane = np.arange(T)
    off = 8 * (2 * (lane // 8) + lane % 2)
    tiles = [np.array(_BASES[4 * t:4 * t + 4])[(lane % 8) // 2] + off for t in range(5)]
    lo = lane < T // 2
    vals = [np.where(lo, tiles[0], np.roll(tiles[1], T // 2)),
            np.where(lo, np.roll(tiles[0], T // 2), tiles[1])]
    for m in range(2, NB):
        t, shift, end = _TAPS[m]
        v = np.roll(tiles[t], shift)
        vals.append(v if end is None else np.where(lane == end, (m + 1) * T, v))
    fk = np.zeros((max(_SHARE) + 1, 2 * T, T))
    for m in range(NB):
        blk = lag[m * T:(m + 1) * T]
        e = (blk[:, None] == vals[m][None, :]).astype(np.float64)
        assert (e.sum(1) == 1).all()
        c = np.concatenate([(ph @ e).real, (ph @ e).imag], 0)
        assert _SHARE.index(_SHARE[m]) == m or np.array_equal(fk[_SHARE[m]], c)
        fk[_SHARE[m]] = c
    g = np.stack([g[:, :T], g[:, T:]])
    return _pack_rows(fx), _pack_rows(g), _pack_rows(fk)


def _cmul(a, b):
    return a[0] * b[0] - a[1] * b[1], a[0] * b[1] + a[1] * b[0]


def _times(f, conj=False):
    dif, tot = f[1] - f[0], f[1] + f[0]

    def mul(a):
        k = f[0] * (a[0] + a[1])
        if conj:
            return k + a[1] * dif, k - a[0] * tot
        return k - a[1] * tot, k + a[0] * dif
    return mul


def _csq(a):
    t = a[0] * a[1]
    return a[0] * a[0] - a[1] * a[1], t + t


def _tree(op, xs):
    while len(xs) > 1:
        xs = [op(a, b) for a, b in zip(xs[0::2], xs[1::2])]
    return xs[0]


def _pack(a, b):
    return pltpu.pack_elementwise([a, b], packed_dtype=BF16)


def _words(a):
    return pltpu.bitcast(a.astype(BF16), U32)


def _halves(a):
    return pltpu.bitcast(a, BF16)


def _dot(a, b):
    return jnp.dot(a, b, preferred_element_type=F32)


def _dot_nt(a, b):
    return jax.lax.dot_general(a, b, (((1,), (1,)), ((), ())), preferred_element_type=F32)


def _sincos(x):
    k = jnp.floor(x * (2.0 / np.pi) + 0.5)
    r = ((x - k * 1.5703125) - k * 4.837512969970703125e-4) - k * 7.54978995489188216e-8
    z = r * r
    s = r + r * z * (-1.6666654611e-1 + z * (8.3321608736e-3 + z * -1.9515295891e-4))
    c = 1.0 + z * (-0.5 + z * (4.166664568298827e-2
                               + z * (-1.388731625493765e-3 + z * 2.443315711809948e-5)))
    n = k.astype(jnp.int32)
    odd = (n & 1) == 1
    s, c = jnp.where(odd, c, s), jnp.where(odd, s, c)
    return jnp.where((n & 2) == 2, -s, s), jnp.where(((n + 1) & 2) == 2, -c, c)


def _aligned(i, n):
    return i if isinstance(i, int) else pl.multiple_of(i, n)


def _loop(n, body):
    jax.lax.fori_loop(0, n, lambda i, c: body(i), None)


def _interleave(*streams):
    done = [0] * len(streams)
    live = list(range(len(streams)))
    while live:
        i = min(live, key=lambda n: streams[n][2]
                + (streams[n][3] - streams[n][2]) * done[n] / streams[n][1])
        work = next(streams[i][0], None)
        if work is None:
            live.remove(i)
        else:
            done[i] += work


def _chain(gens):
    for g in gens:
        yield from g


def _kernel(x_hbm, wqkv_hbm, wo_hbm, are_hbm, aim_hbm, bre_hbm, bim_hbm, cre_hbm, cim_hbm,
            ldt_hbm, dsk_hbm, gw_hbm, fx_hbm, g_hbm, fk_hbm, o_hbm,
            x_ref, wqkv_ref, wo_ref, ssm_ref, fx_ref, g_ref, fk_ref, o_ref,
            xs_s, gate_s, wt_s, wp_s, wop_s, par_s, us_s, vs_s, kend_s, ko_s, kt_s,
            kh_s, xh_s, yh_s, tmp_s, q_s, k_s, v_s, at_s, cur_s, y_s, zero_s, vec_s, ldt_in, dsk_in, gw_in,
            sems, xsems, osem):
    lane = jax.lax.broadcasted_iota(jnp.int32, (8, T), 1)
    lo = lane < T // 2

    ldt_ref, dsk_ref, gw_ref = vec_s.at[0], vec_s.at[1], vec_s.at[2]
    ssm_hbm = (are_hbm, aim_hbm, bre_hbm, bim_hbm, cre_hbm, cim_hbm)
    sem_ids = iter(range(N_COPIES))
    copy = lambda a, b: pltpu.make_async_copy(a, b, sems.at[next(sem_ids)])
    cp_ssm = [[copy(h.at[:, a:b], ssm_ref.at[i, :, a:b]) for i, h in enumerate(ssm_hbm)]
              for a, b in ((0, T), (T, 2 * T), (2 * T, D))]
    cp_fx = copy(fx_hbm, fx_ref)
    cp_vec = [copy(ldt_hbm, ldt_in), copy(dsk_hbm, dsk_in), copy(gw_hbm, gw_in)]

    def cp_x(i):
        rows = pl.ds(_aligned(i * (S // 4), S // 4), S // 4)
        return pltpu.make_async_copy(x_hbm.at[rows, :], x_ref.at[rows, :], xsems.at[i])
    cp_w = [copy(wqkv_hbm.at[:, s * D:(s + 1) * D], wqkv_ref.at[:, s * D:(s + 1) * D]) for s in range(3)]
    cp_fk = copy(fk_hbm, fk_ref)
    cp_out = [copy(wo_hbm, wo_ref), copy(g_hbm, g_ref)]
    for c in cp_vec + cp_ssm[0] + [cp_fx, cp_x(0), cp_x(1)]:
        c.start()

    tokens, always = [], []

    def post(a, every):
        tokens[:] = tokens[-KEEP:] + [a[r - 8:r] for r in range(every, a.shape[0] + 1, every)]

    def pace(x):
        always[2] += 1
        if len(tokens) <= always[3] or always[2] < always[1]:
            return x
        always[2] = 0
        head = jnp.where(always[0], x[:8], pltpu.bitcast(tokens.pop(0), x.dtype))
        return head if x.shape[0] == 8 else jnp.concatenate([head, x[8:]], 0)

    def x_block(m):
        r0, h0 = _aligned(m * T, T), _aligned(m * (T // 2), T // 2)
        acc = None
        for t in range(NT):
            x = x_ref[pl.ds(r0, T), t * T:(t + 1) * T]
            xs_s[t, pl.ds(h0, T // 2), :] = pltpu.bitcast(x, U32)
            r = _dot(_halves(fx_ref[...]), x)
            xh_s[t, m, 0:T, :] = r[:T]
            xh_s[t, m, IM:IM + T, :] = r[T:]
            post(r, X_EVERY)
            xg = x.astype(F32) * gw_ref[:, t * T:(t + 1) * T]
            acc = xg if acc is None else acc + xg
            yield 64
        gate = jax.nn.sigmoid(jnp.sum(acc, axis=1, keepdims=True))
        gate_s[pl.ds(r0, T), :] = jnp.broadcast_to(gate, (T, T))

    def regroup(src, t):
        rows = []
        for i in range(2):
            ab = [src[pl.ds(2 * t + i + h * DH // 2, H // 2, stride=DH), :] for h in range(2)]
            ab[0] = pace(ab[0]) if i == 0 else ab[0]
            rows += [_pack(*[pltpu.unpack_elementwise(w, index=e, packed_dtype=BF16, unpacked_dtype=F32)
                             for w in ab]) for e in range(2)]
        return jnp.concatenate(rows, 0)

    def w_qkv(s):
        for c in range(NT):
            for kt in range(NT):
                w = wqkv_ref[kt * T:(kt + 1) * T, s * D + c * T:s * D + (c + 1) * T]
                wt_s[s, kt, c * (T // 2):(c + 1) * (T // 2), :] = pltpu.bitcast(w.T, U32)
                yield 1
        for t in range(NT):
            for kt in range(NT):
                wp_s[t, kt, s * (T // 2):(s + 1) * (T // 2), :] = regroup(wt_s.at[s, kt], t)
                yield 1

    def w_out():
        for ct in range(NT):
            wt_s[0, ct, 0:D // 2, :] = pltpu.bitcast(wo_ref[:, ct * T:(ct + 1) * T], U32)
            for t in range(NT):
                wop_s[ct, t * (T // 2):(t + 1) * (T // 2), :] = regroup(wt_s.at[0, ct], t)
            yield 1

    def put_par(i, a):
        par_s[i, 0:T, :] = a[0:T].T
        hi = a[T:N]
        par_s[i, T:N, :] = jnp.concatenate(
            [hi, pltpu.roll(hi, T // 2, 1)], 0).T[0:T // 2]

    def discretize(j):
        c0 = j * T if isinstance(j, int) else pl.multiple_of(j * T, T)
        dt = jnp.exp(ldt_ref[:, pl.ds(c0, T)].astype(F32)).astype(BF16).astype(F32)
        load = lambda i: ssm_ref[i, :, pl.ds(c0, T)].astype(F32)
        return dt, load, jnp.exp(dt * load(0)), dt * load(1)

    def prep(j):
        dt, load, mag, ang = discretize(j)
        sin, cos = _sincos(ang)
        w = _cmul((load(4), load(5)), (dt * load(2), dt * load(3)))
        for i, a in enumerate((mag * cos, mag * sin, w[0], -w[1])):
            put_par(i, a)
        return jnp.max(jnp.abs(ang))

    def prep_wide(j, ang_max):
        def redo(_):
            _, _, mag, ang = discretize(j)
            put_par(0, mag * jnp.cos(ang))
            put_par(1, mag * jnp.sin(ang))
        _loop(jnp.where(ang_max <= SINCOS_MAX, 0, 1), redo)

    GEN_STEPS = 28

    def gen(r, hi):
        r0 = r * 8 if isinstance(r, int) else pl.multiple_of(r * 8, 8)
        d0 = (r // 4) * GS + (r % 4) * 8
        s0 = T + r0 if hi else r0

        def put(dst, i, a, b):
            re, im = _pack(a[0], b[0]), _pack(a[1], b[1])
            if hi:
                t = pltpu.roll(jnp.where(lo, im, re), T // 2, 1)
                dst[2, pl.ds(i * 4 * GS + d0, 8), :] = jnp.where(lo, re, t)
                dst[2, pl.ds(i * 4 * GS + 2 * GS + d0, 8), :] = jnp.where(lo, t, im)
            else:
                dst[0, pl.ds(i * 4 * GS + d0, 8), :] = re
                dst[1, pl.ds(i * 4 * GS + d0, 8), :] = im

        p = (par_s[0, pl.ds(s0, 8), :], par_s[1, pl.ds(s0, 8), :])
        p2 = _csq(p)
        p4 = _csq(p2)
        q = _csq(p4)
        q2 = _csq(q)
        q4 = _csq(q2)
        yield 1
        v = [(jnp.ones_like(q[0]), jnp.zeros_like(q[0])), q, q2, _cmul(q, q2)]
        by_q4 = _times(q4)
        for i in range(NV // 2):
            put(vs_s, 2 * i, v[0], v[1])
            yield 1
            put(vs_s, 2 * i + 1, v[2], v[3])
            if i == 0:
                v = [q4] + [by_q4(a) for a in v[1:]]
            elif i < NV // 2 - 1:
                v = [by_q4((pace(v[0][0]), v[0][1]))] + [by_q4(a) for a in v[1:]]
            yield 1
        b1 = by_q4(v[0])
        u = [(par_s[2, pl.ds(s0, 8), :], par_s[3, pl.ds(s0, 8), :])]
        u += [_times(p, True)(u[0])]
        put(us_s, 0, u[0], u[1])
        yield 1
        fs, by = [p2, p4, b1], []
        for i, (a, b, f) in enumerate(((0, 1, 0), (0, 1, 1), (2, 3, 1), (0, 2, 2), (4, 6, 2),
                                       (0, 4, 3), (8, 10, 3), (0, 8, 4), (12, 14, 4))):
            if f == len(fs):
                fs.append(_csq(fs[-1]))
            if f == len(by):
                by.append(_times(fs[f], True))
            u += [by[f]((pace(u[a][0]), u[a][1])), by[f](u[b])]
            put(us_s, 1 + i, u[-2], u[-1])
            yield 1
        last = u[16][0] * fs[4][0] + u[16][1] * fs[4][1]
        if hi:
            kend_s[1, pl.ds(r0, 8), :] = jnp.where(lo, last, 0.0)
            kend_s[1, pl.ds(T // 2 + r0, 8), :] = jnp.where(lo, 0.0, last)
        else:
            kend_s[0, pl.ds(r0, 8), :] = last
        yield 1

    def kmat(g):
        u = jnp.concatenate([_halves(us_s[t, pl.ds(g, 4 * NU, stride=GS), :]) for t in range(3)], 1)
        v = jnp.concatenate([_halves(vs_s[t, pl.ds(g, 4 * NV, stride=GS), :]) for t in range(3)], 1)
        r = _dot_nt(u, v)
        ko_s[pl.ds(g * KS, 8 * NU), :] = r
        post(r, KMAT_EVERY)

    def taps(j):
        lane32 = jax.lax.broadcasted_iota(jnp.int32, (32, T), 1)
        slot = (lane32 % 8) // 2

        def gather(t):
            parts = []
            for c in range(4):
                acc = None
                for jj in range(4):
                    k = 4 * t + jj
                    a = ko_s[pl.ds((k // 2) * 8 + 2 * c + k % 2, 32, stride=KS), :]
                    if jj != c:
                        a = pltpu.roll(a, (2 * (jj - c)) % T, 1)
                    acc = a if acc is None else jnp.where(slot == jj, a, acc)
                parts.append(acc)
            return jnp.concatenate(parts, 0)

        def emit(ms, taps):
            kt_s[_SLOT[ms[0]]] = _words(taps)

        lane_t = jax.lax.broadcasted_iota(jnp.int32, (T, T), 1)
        lo_t, first = lane_t < T // 2, lane_t == 0
        t4 = gather(4)
        emit([8, 9], t4)
        for m in (10, 12):
            emit([m, m + 1], pltpu.roll(t4, _TAPS[m][1], 1))
        kend = jnp.sum(kend_s[0] + kend_s[1], axis=1, keepdims=True)
        emit([14, 15], jnp.where(lane_t == 2, kend, pltpu.roll(t4, _TAPS[14][1], 1)))
        yield 1
        t3 = gather(3)
        emit([4, 5], t3)
        emit([6, 7], jnp.where(lane_t == 4, pltpu.roll(t4, 4, 1), pltpu.roll(t3, _TAPS[6][1], 1)))
        yield 1
        t2 = gather(2)
        emit([2], t2)
        emit([3], jnp.where(first, t3, t2))
        yield 1
        t1 = gather(1)
        yield 1
        t0 = gather(0)
        x = pltpu.roll(jnp.where(lo_t, t1, t0), T // 2, 1)
        emit([1], jnp.where(lo_t, x, t1))
        skip = dsk_ref[:, pl.ds(j * T if isinstance(j, int) else pl.multiple_of(j * T, T), T)].astype(F32)
        skip = jnp.broadcast_to(skip, (T, T)).T
        emit([0], jnp.where(lo_t, t0, x) + jnp.where(first, skip, 0.0))
        yield 1

    def spectrum_k():
        for m in range(NB):
            r = _dot_nt(_halves(fk_ref[_SHARE[m]]), _halves(kt_s[_SLOT[m]]))
            kh_s[m, 0:T, :] = r[:T]
            kh_s[m, IM:IM + T, :] = r[T:]
            post(r, FK_EVERY)
            yield 64

    PW_STEPS = 3 * NB * (NB + 1) // 2

    def pointwise(j, i):
        r0 = _aligned(i * 8, 8)

        def part(ref, m, c):
            if c < 2:
                return ref[m, pl.ds(c * IM + r0, 8), :]
            return part(ref, m, 0) + part(ref, m, 1)

        prev = None
        for c in range(3):
            for p0 in range(0, NB, PW_SPLIT):
                ps = range(p0, p0 + PW_SPLIT)
                xs, acc = {}, {}
                for m in range(p0 + PW_SPLIT):
                    k = part(kh_s, m, c)
                    if m % 2 == 0:
                        k = pace(k)
                    for p in ps:
                        if p >= m:
                            if p - m not in xs:
                                xs[p - m] = part(xh_s.at[j], p - m, c)
                            kx = k * xs[p - m]
                            acc[p] = kx + acc[p] if m else kx - tmp_s[p] if c == 2 else kx
                    yield min(p0 + PW_SPLIT - m, PW_SPLIT)
                for p in ps:
                    if c == 0:
                        tmp_s[p] = acc[p]
                    elif c == 1:
                        rr = tmp_s[p]
                        tmp_s[NB + p] = rr - acc[p]
                        tmp_s[p] = rr + acc[p]
                    else:
                        y = (tmp_s[NB + p], acc[p])
                        z = y if prev is None else (y[0] - prev[1], y[1] + prev[0])
                        yh_s[j, p, pl.ds(r0, 8), :] = _pack(*z)
                        prev = y

    qscale = float(DH ** -0.5 * np.log2(np.e))

    def qkv(j, i, every):
        r0, h0 = i * QR, i * (QR // 2)
        if not isinstance(i, int):
            r0, h0 = pl.multiple_of(r0, QR), pl.multiple_of(h0, QR // 2)
        for s in range(3):
            x = jnp.concatenate([_halves(xs_s[t, pl.ds(h0, QR // 2), :]) for t in range(NT)], 1)
            w = jnp.concatenate([_halves(wp_s[j, t, s * (T // 2):(s + 1) * (T // 2), :])
                                 for t in range(NT)], 1)
            acc = _dot_nt(x, w)
            if s == 0:
                q_s[j, pl.ds(r0, QR), :] = acc * qscale
            else:
                (k_s, v_s)[s - 1][j, pl.ds(HALO + r0, QR), :] = acc
            post(acc, every)
            yield QR * 5 // 4

    def window(r0, masked):
        rows = lambda r: pl.ds(r, 8)
        qs = [q_s[t, rows(r0), :] for t in range(NT)]
        ls = []
        for w in range(WIN):
            a = None
            for t in range(NT):
                k = k_s[t, rows(r0 + HALO - DIL * w), :]
                kq = qs[t] * k
                a = kq if a is None else a + kq
            ls.append((a, pltpu.roll(a, 64, 1)))
        yield 1
        ls = [a + b for a, b in ls]
        ls = [(a, pltpu.roll(a, 32, 1)) for a in ls]
        yield 1
        ls = [a + b for a, b in ls]
        if masked:
            row = jax.lax.broadcasted_iota(jnp.int32, (8, T), 0) + r0
            ls = [jnp.where(row >= DIL * w, a, -1e9 * np.log2(np.e)) for w, a in enumerate(ls)]
        mx = _tree(jnp.maximum, ls)
        es = [jnp.exp2(a - mx) for a in ls]
        yield 1
        inv = gate_s[rows(r0), :] * pl.reciprocal(_tree(jnp.add, es), full_range=False)
        outs = []
        for t in range(NT):
            a = None
            for w in range(WIN):
                v = v_s[t, rows(r0 + HALO - DIL * w), :]
                pv = es[w] * (pace(v) if w == 0 and t == 0 else v)
                a = pv if a is None else a + pv
            outs.append(a)
        for t in range(NT):
            at_s[t, rows(r0), :] = outs[t] * inv
        yield 1

    def attend(r0, n, first=False):
        gens = [window(r0 + 8 * c, first and 8 * c < DIL * WIN) for c in range(n)]
        for step in range(n + 3):
            for c in range(step, step - 4, -1):
                if 0 <= c < n:
                    next(gens[c])
            yield 1

    def stage(i):
        r0 = _aligned(i * RB, RB)
        for t in range(NT):
            cur_s[t] = _pack(*[at_s[t, pl.ds(r0 + e, RB // 2, stride=2), :] for e in range(2)])

    def out_copy(i):
        r0 = _aligned(i * RB, RB)
        return pltpu.make_async_copy(o_ref.at[pl.ds(r0, RB), :], o_hbm.at[pl.ds(r0, RB), :], osem)

    def tail_copy(ct):
        part = (slice(S - RB, S), slice(ct * T, (ct + 1) * T))
        return pltpu.make_async_copy(o_ref.at[part], o_hbm.at[part], osem)

    def mix(i):
        r0 = _aligned(i * RB, RB)
        for ct in range(NT):
            for h in range(RB // T):
                y = _dot(jnp.concatenate([_halves(g_ref[b]) for b in range(2)], 1),
                         _halves(yh_s[ct, i * (RB // T) + h]))
                y_s[ct, h * T:(h + 1) * T, :] = (1.0 - gate_s[pl.ds(r0 + h * T, T), :]) * y
                post(y, T)
                yield 64
        for ct in range(NT):
            yield from project(r0, ct)

    def project(r0, ct):
        a = _dot(jnp.concatenate([_halves(cur_s[t]) for t in range(NT)], 1), _halves(wop_s[ct]))
        acc = a + y_s[ct]
        o_ref[pl.ds(r0, RB), ct * T:(ct + 1) * T] = acc.astype(BF16)
        if isinstance(r0, int):
            tail_copy(ct).start()
        post(acc, MIX_EVERY)
        yield RB * 5 // 4

    def gen_stream(i0, n):
        units = [u for i in range(2 * n)
                 for u in (gen(4 * i0 + 2 * i, False), gen(4 * i0 + 2 * i + 1, False), gen(2 * i0 + i, True))]
        return _chain(units), len(units) * GEN_STEPS, 0.0, 1.0

    def qkvs(j, i0, n, every):
        return _chain([qkv(j, i0 + u, every) for u in range(n)])

    def kmats(g0, n):
        for u in range(n):
            kmat(g0 + u)
            yield 60

    def overlap(*streams, gap=1, lag=0):
        always[:] = [zero_s[...] == 0.0, gap, 0, lag]
        _interleave(*streams)
        tokens.clear()
        always.clear()

    nq, cq = S // QR, QR * 15 // 4

    for t in range(NT):
        k_s[t, 0:HALO, :] = jnp.zeros((HALO, T), F32)
        v_s[t, 0:HALO, :] = jnp.zeros((HALO, T), F32)
    zero_s[...] = jnp.zeros((8, T), F32)
    for c in cp_vec + cp_ssm[0]:
        c.wait()
    for i, ref in enumerate((ldt_in, dsk_in, gw_in)):
        vec_s[i] = ref[...].astype(F32).reshape(1, D)
    cp_x(2).start()
    prep_wide(0, prep(0))
    cp_fx.wait()

    def first(i):
        for when, cs in enumerate(([cp_w[0]], [cp_x(3), cp_w[1]], [cp_w[2]], [cp_fk] + cp_ssm[1])):
            @pl.when(i == when)
            def _():
                for c in cs:
                    c.start()

        @pl.when(i % 2 == 0)
        def _():
            cp_x(i // 2).wait()
        xs = (_chain([x_block(2 * i + u) for u in range(2)]), 128 * NT, X_LEAD, X_LAST)
        overlap(xs, gen_stream(i, 1), gap=X_GAP, lag=X_LAG)
    _loop(4, first)
    late = (cp_ssm[2], cp_out, [])
    for s, (g0, g1, m0, m1) in enumerate(((0, 16, 8, 10), (16, 32, 10, 12), (32, 32, 12, NB))):
        for c in late[s]:
            c.start()
        cp_w[s].wait()
        if m0 % 4 == 0:
            cp_x(m0 // 4).wait()
        mxu = _chain([kmats(g0, g1 - g0)] + [x_block(m) for m in range(m0, m1)])
        overlap((mxu, 60 * (g1 - g0) + 64 * NT * (m1 - m0), LEAD, LAST),
                (w_qkv(s), 2 * NT * NT, 0.0, 1.0), lag=PW_LAG)
    overlap((qkv(0, 0, QR), cq, 0.0, 1.0), (taps(0), 5, 0.0, 1.0))
    for c in [cp_fk] + cp_ssm[1]:
        c.wait()

    def pws(j, i0, n):
        return (_chain([pointwise(j, i0 + u) for u in range(n)]), n * PW_STEPS, 0.0, 1.0)

    def tile(j):
        @pl.when(j == 1)
        def _():
            for c in cp_ssm[2]:
                c.wait()
        overlap((spectrum_k(), 1024, 0.0, 1.0))
        prep_wide(j + 1, prep(j + 1))
        overlap((qkvs(j, 1, 4, GEN_EVERY), 4 * cq, LEAD2, LAST2), gen_stream(0, 4),
                gap=GEN_GAP, lag=GEN_LAG)
        mxu = _chain([kmats(0, 32), qkvs(j, 5, NA, PW_EVERY)])
        overlap((mxu, 1920 + NA * cq, LEAD, LAST), pws(j, 0, PA), gap=PW_GAP, lag=PW_LAG)
        n = nq - 4 - NA
        mxu = _chain([qkvs(j, NA + 5, n - 1, PW_EVERY), qkv(j + 1, 0, PW_EVERY)])
        st = [(mxu, n * cq, LEAD, LAST), pws(j, PA, 16 - PA)]
        overlap(*st, (taps(j + 1), 5, 0.0, TAP_LAST), gap=PW_GAP, lag=PW_LAG)
    _loop(NT - 1, tile)

    j = NT - 1
    for c in cp_out:
        c.wait()
    mxu = _chain([spectrum_k(), qkvs(j, 1, HEAD - 1, 64)])
    st = [(mxu, 1024 + cq * (HEAD - 1), LEAD, LAST), (attend(0, FIRST, True), FIRST + 3, 0.0, 1.0)]
    overlap(*st, (w_out(), NT, 0.0, 1.0), lag=PW_LAG)
    n = (nq - HEAD) // NL

    def last_conv(i):
        r0 = pl.multiple_of(8 * (FIRST + i * EARLY), 16)
        st = [(qkvs(j, HEAD + n * i, n, PW_EVERY), cq * n, LEAD, LAST), pws(j, 16 // NL * i, 16 // NL)]
        overlap(*st, (attend(r0, EARLY), EARLY + 3, 0.0, 1.0), gap=PW_GAP, lag=PW_LAG)
    _loop(NL, last_conv)

    done, nr = FIRST + NL * EARLY, S // RB
    n_mixed = (S // 8 - done) // PER_ROW
    assert n * NL + HEAD == nq and done + n_mixed * PER_ROW == S // 8 and n_mixed == nr - 1
    assert 8 * FIRST <= QR and FIRST % 2 == EARLY % 2 == PER_ROW % 2 == 0
    assert all(8 * (FIRST + EARLY * (i + 1)) <= (HEAD + n * i) * QR for i in range(NL))
    assert all(8 * (done + PER_ROW * i) >= (i + 1) * RB for i in range(n_mixed + 1))
    stage(0)

    def rows(i):
        r0 = pl.multiple_of(8 * (done + PER_ROW * i), 16)
        overlap((mix(i), NT * RB * 7 // 4, MIX_LEAD, MIX_LAST),
                (attend(r0, PER_ROW), 100 * PER_ROW + 300, 0.0, 1.0), lag=1)
        stage(i + 1)
        out_copy(i).start()
    _loop(nr - 1, rows)
    overlap((mix(nr - 1), 1, 0.0, 1.0))
    for i in range(nr - 1):
        out_copy(i).wait()
    for ct in range(NT):
        tail_copy(ct).wait()


@jax.jit
def pallas_gated_mix__sliding_local_dilated__ssm_conv_s4__prompt_kernel(
    A_x: jax.Array,
    A_wqkv: jax.Array,
    A_wo: jax.Array,
    B_u: jax.Array,
    B_A_re: jax.Array,
    B_A_im: jax.Array,
    B_B_re: jax.Array,
    B_B_im: jax.Array,
    B_C_re: jax.Array,
    B_C_im: jax.Array,
    B_log_dt: jax.Array,
    B_Dskip: jax.Array,
    gate_w: jax.Array,
):
    del B_u
    fx, g, fk = _constants()
    vm = pltpu.VMEM
    hbm = pl.BlockSpec(memory_space=pl.ANY)
    out = pl.pallas_call(
        _kernel,
        out_shape=jax.ShapeDtypeStruct((S, D), BF16),
        in_specs=[hbm] * 15,
        out_specs=hbm,
        scratch_shapes=[
            vm((S, D), BF16), vm((D, 3 * D), BF16), vm((D, D), BF16), vm((6, N, D), BF16),
            vm(fx.shape, U32), vm(g.shape, U32), vm(fk.shape, U32), vm((S, D), BF16),
            vm((NT, S // 2, T), U32), vm((S, T), F32),
            vm((3, NT, D // 2 + 32, T), U32), vm((NT, NT, 3 * T // 2, T), U32), vm((NT, D // 2, T), U32),
            vm((4, N, T), F32), vm((3, NU * 4 * GS + 64, T), U32), vm((3, NV * 4 * GS + 64, T), U32),
            vm((2, T, T), F32), vm((32 * KS + 96, T), F32), vm((max(_SLOT) + 1, T // 2, T), U32),
            vm((NB, SPEC, T), F32), vm((NT, NB, SPEC, T), F32), vm((NT, NB, T, T), U32),
            vm((2 * NB, 8, T), F32),
            vm((NT, S, T), F32), vm((NT, S + HALO, T), F32), vm((NT, S + HALO, T), F32),
            vm((NT, S + 32, T), F32), vm((NT, RB // 2, T), U32), vm((NT, RB, T), F32), vm((8, T), F32),
            vm((3, 1, D), F32), vm((D,), BF16), vm((D,), BF16), vm((D,), BF16),
            pltpu.SemaphoreType.DMA((N_COPIES,)), pltpu.SemaphoreType.DMA((4,)),
             pltpu.SemaphoreType.DMA(()),
        ],
        compiler_params=pltpu.CompilerParams(vmem_limit_bytes=100 * 1024 * 1024),
    )(A_x.reshape(S, D), A_wqkv, A_wo, B_A_re.T, B_A_im.T, B_B_re.T, B_B_im.T, B_C_re.T, B_C_im.T,
      B_log_dt, B_Dskip, gate_w, fx, g, fk)
    return out.reshape(1, S, D)
```

```python
import jax
import jax.numpy as jnp
import numpy as np
import jax.experimental.pallas as pl
import jax.experimental.pallas.tpu as pltpu

S, D, H, DH, N = 2048, 640, 32, 20, 192
WIN, DIL = 8, 2
T = 128
NT = D // T
NB = S // T
HALO = 32
N_COPIES = 28
SINCOS_MAX = 8192.0
QR = 256
RB = 256
IM, SPEC = 144, 280

NA, PA = 1, 8
HEAD, NL = 2, 2
FIRST, EARLY, PER_ROW = 28, 16, 28
LEAD, LAST, LEAD2, LAST2, TAP_LAST = 0.04, 0.98, 0.03, 0.98, 0.8
X_LEAD, X_LAST, X_EVERY, X_GAP, X_LAG = 0.1, 0.95, 32, 1, 8
GEN_EVERY, GEN_GAP, GEN_LAG = 8, 1, 6
PW_EVERY, PW_GAP, PW_LAG, PW_SPLIT = 16, 2, 4, 8
FK_EVERY, KMAT_EVERY, KEEP = 256, 40, 32
MIX_EVERY, MIX_LEAD, MIX_LAST = 64, 0.05, 1.0
NU, NV = 10, 16
GS = 36
KS = 84
F32, BF16, U32 = jnp.float32, jnp.bfloat16, jnp.uint32

_BASES = [0, 1, 2, 3, 4, 5, 6, 7, 256, 258, 260, 262, 512, 516, 768, 772,
          1024, 1280, 1536, 1792]


_TAPS = {2: (2, 0, None), 3: (2, 0, 0),
         4: (3, 0, None), 5: (3, 0, None), 6: (3, T - 4, None), 7: (3, T - 4, 4)}
_TAPS.update({m: (4, (8 - m + m % 2) % T, 2 if m == NB - 1 else None) for m in range(8, NB)})
_SLOT = [0, 1, 2, 3] + [4 + (m - 4) // 2 for m in range(4, NB)]
_SHARE = [0, 0, 1, 2, 3, 4, 3, 4] + [5, 6] * 4


def _pack_rows(a):
    b = a.astype(np.float32).astype(BF16).view(np.uint16).astype(np.uint32)
    return b[..., 0::2, :] | (b[..., 1::2, :] << 16)


def _constants():
    om = 2.0 * np.pi * (np.arange(T) + 0.25) / T
    ph = np.exp(-1j * om[:, None] * np.arange(T)[None, :])
    fx = np.concatenate([ph.real, ph.imag], 0)
    g = np.stack([ph.real.T, ph.imag.T], -1).reshape(T, 2 * T) / T
    lag = np.arange(S).astype(np.float32).astype(BF16).astype(np.float32).astype(np.int64)
    lane = np.arange(T)
    off = 8 * (2 * (lane // 8) + lane % 2)
    tiles = [np.array(_BASES[4 * t:4 * t + 4])[(lane % 8) // 2] + off for t in range(5)]
    lo = lane < T // 2
    vals = [np.where(lo, tiles[0], np.roll(tiles[1], T // 2)),
            np.where(lo, np.roll(tiles[0], T // 2), tiles[1])]
    for m in range(2, NB):
        t, shift, end = _TAPS[m]
        v = np.roll(tiles[t], shift)
        vals.append(v if end is None else np.where(lane == end, (m + 1) * T, v))
    fk = np.zeros((max(_SHARE) + 1, 2 * T, T))
    for m in range(NB):
        blk = lag[m * T:(m + 1) * T]
        e = (blk[:, None] == vals[m][None, :]).astype(np.float64)
        assert (e.sum(1) == 1).all()
        c = np.concatenate([(ph @ e).real, (ph @ e).imag], 0)
        assert _SHARE.index(_SHARE[m]) == m or np.array_equal(fk[_SHARE[m]], c)
        fk[_SHARE[m]] = c
    g = np.stack([g[:, :T], g[:, T:]])
    return _pack_rows(fx), _pack_rows(g), _pack_rows(fk)


def _cmul(a, b):
    return a[0] * b[0] - a[1] * b[1], a[0] * b[1] + a[1] * b[0]


def _times(f, conj=False):
    dif, tot = f[1] - f[0], f[1] + f[0]

    def mul(a):
        k = f[0] * (a[0] + a[1])
        if conj:
            return k + a[1] * dif, k - a[0] * tot
        return k - a[1] * tot, k + a[0] * dif
    return mul


def _csq(a):
    t = a[0] * a[1]
    return a[0] * a[0] - a[1] * a[1], t + t


def _tree(op, xs):
    while len(xs) > 1:
        xs = [op(a, b) for a, b in zip(xs[0::2], xs[1::2])]
    return xs[0]


def _pack(a, b):
    return pltpu.pack_elementwise([a, b], packed_dtype=BF16)


def _words(a):
    return pltpu.bitcast(a.astype(BF16), U32)


def _halves(a):
    return pltpu.bitcast(a, BF16)


def _dot(a, b):
    return jnp.dot(a, b, preferred_element_type=F32)


def _dot_nt(a, b):
    return jax.lax.dot_general(a, b, (((1,), (1,)), ((), ())), preferred_element_type=F32)


def _sincos(x):
    k = jnp.floor(x * (2.0 / np.pi) + 0.5)
    r = ((x - k * 1.5703125) - k * 4.837512969970703125e-4) - k * 7.54978995489188216e-8
    z = r * r
    s = r + r * z * (-1.6666654611e-1 + z * (8.3321608736e-3 + z * -1.9515295891e-4))
    c = 1.0 + z * (-0.5 + z * (4.166664568298827e-2
                               + z * (-1.388731625493765e-3 + z * 2.443315711809948e-5)))
    n = k.astype(jnp.int32)
    odd = (n & 1) == 1
    s, c = jnp.where(odd, c, s), jnp.where(odd, s, c)
    return jnp.where((n & 2) == 2, -s, s), jnp.where(((n + 1) & 2) == 2, -c, c)


def _aligned(i, n):
    return i if isinstance(i, int) else pl.multiple_of(i, n)


def _loop(n, body):
    jax.lax.fori_loop(0, n, lambda i, c: body(i), None)


def _interleave(*streams):
    done = [0] * len(streams)
    live = list(range(len(streams)))
    while live:
        i = min(live, key=lambda n: streams[n][2]
                + (streams[n][3] - streams[n][2]) * done[n] / streams[n][1])
        work = next(streams[i][0], None)
        if work is None:
            live.remove(i)
        else:
            done[i] += work


def _chain(gens):
    for g in gens:
        yield from g


def _kernel(x_hbm, wqkv_hbm, wo_hbm, are_hbm, aim_hbm, bre_hbm, bim_hbm, cre_hbm, cim_hbm,
            ldt_hbm, dsk_hbm, gw_hbm, fx_hbm, g_hbm, fk_hbm, o_hbm,
            x_ref, wqkv_ref, wo_ref, ssm_ref, fx_ref, g_ref, fk_ref, o_ref,
            xs_s, gate_s, wt_s, wp_s, wop_s, par_s, us_s, vs_s, kend_s, ko_s, kt_s,
            kh_s, xh_s, yh_s, tmp_s, q_s, k_s, v_s, at_s, cur_s, y_s, zero_s, vec_s, ldt_in, dsk_in, gw_in,
            sems, xsems, osem):
    lane = jax.lax.broadcasted_iota(jnp.int32, (8, T), 1)
    lo = lane < T // 2

    ldt_ref, dsk_ref, gw_ref = vec_s.at[0], vec_s.at[1], vec_s.at[2]
    ssm_hbm = (are_hbm, aim_hbm, bre_hbm, bim_hbm, cre_hbm, cim_hbm)
    sem_ids = iter(range(N_COPIES))
    copy = lambda a, b: pltpu.make_async_copy(a, b, sems.at[next(sem_ids)])
    cp_ssm = [[copy(h.at[:, a:b], ssm_ref.at[i, :, a:b]) for i, h in enumerate(ssm_hbm)]
              for a, b in ((0, T), (T, 2 * T), (2 * T, D))]
    cp_fx = copy(fx_hbm, fx_ref)
    cp_vec = [copy(ldt_hbm, ldt_in), copy(dsk_hbm, dsk_in), copy(gw_hbm, gw_in)]

    def cp_x(i):
        rows = pl.ds(_aligned(i * (S // 4), S // 4), S // 4)
        return pltpu.make_async_copy(x_hbm.at[rows, :], x_ref.at[rows, :], xsems.at[i])
    cp_w = [copy(wqkv_hbm.at[:, s * D:(s + 1) * D], wqkv_ref.at[:, s * D:(s + 1) * D]) for s in range(3)]
    cp_fk = copy(fk_hbm, fk_ref)
    cp_out = [copy(wo_hbm, wo_ref), copy(g_hbm, g_ref)]
    for c in cp_vec + cp_ssm[0] + [cp_fx, cp_x(0), cp_x(1)]:
        c.start()

    tokens, always = [], []

    def post(a, every):
        tokens[:] = tokens[-KEEP:] + [a[r - 8:r] for r in range(every, a.shape[0] + 1, every)]

    def pace(x):
        always[2] += 1
        if len(tokens) <= always[3] or always[2] < always[1]:
            return x
        always[2] = 0
        head = jnp.where(always[0], x[:8], pltpu.bitcast(tokens.pop(0), x.dtype))
        return head if x.shape[0] == 8 else jnp.concatenate([head, x[8:]], 0)

    def x_block(m):
        r0, h0 = _aligned(m * T, T), _aligned(m * (T // 2), T // 2)
        acc = None
        for t in range(NT):
            x = x_ref[pl.ds(r0, T), t * T:(t + 1) * T]
            xs_s[t, pl.ds(h0, T // 2), :] = pltpu.bitcast(x, U32)
            r = _dot(_halves(fx_ref[...]), x)
            xh_s[t, m, 0:T, :] = r[:T]
            xh_s[t, m, IM:IM + T, :] = r[T:]
            post(r, X_EVERY)
            xg = x.astype(F32) * gw_ref[:, t * T:(t + 1) * T]
            acc = xg if acc is None else acc + xg
            yield 64
        gate = jax.nn.sigmoid(jnp.sum(acc, axis=1, keepdims=True))
        gate_s[pl.ds(r0, T), :] = jnp.broadcast_to(gate, (T, T))

    def regroup(src, t):
        rows = []
        for i in range(2):
            ab = [src[pl.ds(2 * t + i + h * DH // 2, H // 2, stride=DH), :] for h in range(2)]
            ab[0] = pace(ab[0]) if i == 0 else ab[0]
            rows += [_pack(*[pltpu.unpack_elementwise(w, index=e, packed_dtype=BF16, unpacked_dtype=F32)
                             for w in ab]) for e in range(2)]
        return jnp.concatenate(rows, 0)

    def w_qkv(s):
        for c in range(NT):
            for kt in range(NT):
                w = wqkv_ref[kt * T:(kt + 1) * T, s * D + c * T:s * D + (c + 1) * T]
                wt_s[s, kt, c * (T // 2):(c + 1) * (T // 2), :] = pltpu.bitcast(w.T, U32)
                yield 1
        for t in range(NT):
            for kt in range(NT):
                wp_s[t, kt, s * (T // 2):(s + 1) * (T // 2), :] = regroup(wt_s.at[s, kt], t)
                yield 1

    def w_out():
        for ct in range(NT):
            wt_s[0, ct, 0:D // 2, :] = pltpu.bitcast(wo_ref[:, ct * T:(ct + 1) * T], U32)
            for t in range(NT):
                wop_s[ct, t * (T // 2):(t + 1) * (T // 2), :] = regroup(wt_s.at[0, ct], t)
            yield 1

    def put_par(i, a):
        par_s[i, 0:T, :] = a[0:T].T
        hi = a[T:N]
        par_s[i, T:N, :] = jnp.concatenate(
            [hi, pltpu.roll(hi, T // 2, 1)], 0).T[0:T // 2]

    def discretize(j):
        c0 = j * T if isinstance(j, int) else pl.multiple_of(j * T, T)
        dt = jnp.exp(ldt_ref[:, pl.ds(c0, T)].astype(F32)).astype(BF16).astype(F32)
        load = lambda i: ssm_ref[i, :, pl.ds(c0, T)].astype(F32)
        return dt, load, jnp.exp(dt * load(0)), dt * load(1)

    def prep(j):
        dt, load, mag, ang = discretize(j)
        sin, cos = _sincos(ang)
        w = _cmul((load(4), load(5)), (dt * load(2), dt * load(3)))
        for i, a in enumerate((mag * cos, mag * sin, w[0], -w[1])):
            put_par(i, a)
        return jnp.max(jnp.abs(ang))

    def prep_wide(j, ang_max):
        def redo(_):
            _, _, mag, ang = discretize(j)
            put_par(0, mag * jnp.cos(ang))
            put_par(1, mag * jnp.sin(ang))
        _loop(jnp.where(ang_max <= SINCOS_MAX, 0, 1), redo)

    GEN_STEPS = 28

    def gen(r, hi):
        r0 = r * 8 if isinstance(r, int) else pl.multiple_of(r * 8, 8)
        d0 = (r // 4) * GS + (r % 4) * 8
        s0 = T + r0 if hi else r0

        def put(dst, i, a, b):
            re, im = _pack(a[0], b[0]), _pack(a[1], b[1])
            if hi:
                t = pltpu.roll(jnp.where(lo, im, re), T // 2, 1)
                dst[2, pl.ds(i * 4 * GS + d0, 8), :] = jnp.where(lo, re, t)
                dst[2, pl.ds(i * 4 * GS + 2 * GS + d0, 8), :] = jnp.where(lo, t, im)
            else:
                dst[0, pl.ds(i * 4 * GS + d0, 8), :] = re
                dst[1, pl.ds(i * 4 * GS + d0, 8), :] = im

        p = (par_s[0, pl.ds(s0, 8), :], par_s[1, pl.ds(s0, 8), :])
        p2 = _csq(p)
        p4 = _csq(p2)
        q = _csq(p4)
        q2 = _csq(q)
        q4 = _csq(q2)
        yield 1
        v = [(jnp.ones_like(q[0]), jnp.zeros_like(q[0])), q, q2, _cmul(q, q2)]
        by_q4 = _times(q4)
        for i in range(NV // 2):
            put(vs_s, 2 * i, v[0], v[1])
            yield 1
            put(vs_s, 2 * i + 1, v[2], v[3])
            if i == 0:
                v = [q4] + [by_q4(a) for a in v[1:]]
            elif i < NV // 2 - 1:
                v = [by_q4((pace(v[0][0]), v[0][1]))] + [by_q4(a) for a in v[1:]]
            yield 1
        b1 = by_q4(v[0])
        u = [(par_s[2, pl.ds(s0, 8), :], par_s[3, pl.ds(s0, 8), :])]
        u += [_times(p, True)(u[0])]
        put(us_s, 0, u[0], u[1])
        yield 1
        fs, by = [p2, p4, b1], []
        for i, (a, b, f) in enumerate(((0, 1, 0), (0, 1, 1), (2, 3, 1), (0, 2, 2), (4, 6, 2),
                                       (0, 4, 3), (8, 10, 3), (0, 8, 4), (12, 14, 4))):
            if f == len(fs):
                fs.append(_csq(fs[-1]))
            if f == len(by):
                by.append(_times(fs[f], True))
            u += [by[f]((pace(u[a][0]), u[a][1])), by[f](u[b])]
            put(us_s, 1 + i, u[-2], u[-1])
            yield 1
        last = u[16][0] * fs[4][0] + u[16][1] * fs[4][1]
        if hi:
            kend_s[1, pl.ds(r0, 8), :] = jnp.where(lo, last, 0.0)
            kend_s[1, pl.ds(T // 2 + r0, 8), :] = jnp.where(lo, 0.0, last)
        else:
            kend_s[0, pl.ds(r0, 8), :] = last
        yield 1

    def kmat(g):
        u = jnp.concatenate([_halves(us_s[t, pl.ds(g, 4 * NU, stride=GS), :]) for t in range(3)], 1)
        v = jnp.concatenate([_halves(vs_s[t, pl.ds(g, 4 * NV, stride=GS), :]) for t in range(3)], 1)
        r = _dot_nt(u, v)
        ko_s[pl.ds(g * KS, 8 * NU), :] = r
        post(r, KMAT_EVERY)

    def taps(j):
        lane32 = jax.lax.broadcasted_iota(jnp.int32, (32, T), 1)
        slot = (lane32 % 8) // 2

        def gather(t):
            parts = []
            for c in range(4):
                acc = None
                for jj in range(4):
                    k = 4 * t + jj
                    a = ko_s[pl.ds((k // 2) * 8 + 2 * c + k % 2, 32, stride=KS), :]
                    if jj != c:
                        a = pltpu.roll(a, (2 * (jj - c)) % T, 1)
                    acc = a if acc is None else jnp.where(slot == jj, a, acc)
                parts.append(acc)
            return jnp.concatenate(parts, 0)

        def emit(ms, taps):
            kt_s[_SLOT[ms[0]]] = _words(taps)

        lane_t = jax.lax.broadcasted_iota(jnp.int32, (T, T), 1)
        lo_t, first = lane_t < T // 2, lane_t == 0
        t4 = gather(4)
        emit([8, 9], t4)
        for m in (10, 12):
            emit([m, m + 1], pltpu.roll(t4, _TAPS[m][1], 1))
        kend = jnp.sum(kend_s[0] + kend_s[1], axis=1, keepdims=True)
        emit([14, 15], jnp.where(lane_t == 2, kend, pltpu.roll(t4, _TAPS[14][1], 1)))
        yield 1
        t3 = gather(3)
        emit([4, 5], t3)
        emit([6, 7], jnp.where(lane_t == 4, pltpu.roll(t4, 4, 1), pltpu.roll(t3, _TAPS[6][1], 1)))
        yield 1
        t2 = gather(2)
        emit([2], t2)
        emit([3], jnp.where(first, t3, t2))
        yield 1
        t1 = gather(1)
        yield 1
        t0 = gather(0)
        x = pltpu.roll(jnp.where(lo_t, t1, t0), T // 2, 1)
        emit([1], jnp.where(lo_t, x, t1))
        skip = dsk_ref[:, pl.ds(j * T if isinstance(j, int) else pl.multiple_of(j * T, T), T)].astype(F32)
        skip = jnp.broadcast_to(skip, (T, T)).T
        emit([0], jnp.where(lo_t, t0, x) + jnp.where(first, skip, 0.0))
        yield 1

    def spectrum_k():
        for m in range(NB):
            r = _dot_nt(_halves(fk_ref[_SHARE[m]]), _halves(kt_s[_SLOT[m]]))
            kh_s[m, 0:T, :] = r[:T]
            kh_s[m, IM:IM + T, :] = r[T:]
            post(r, FK_EVERY)
            yield 64

    PW_STEPS = 3 * NB * (NB + 1) // 2

    def pointwise(j, i):
        r0 = _aligned(i * 8, 8)

        def part(ref, m, c):
            if c < 2:
                return ref[m, pl.ds(c * IM + r0, 8), :]
            return part(ref, m, 0) + part(ref, m, 1)

        prev = None
        for c in range(3):
            for p0 in range(0, NB, PW_SPLIT):
                ps = range(p0, p0 + PW_SPLIT)
                xs, acc = {}, {}
                for m in range(p0 + PW_SPLIT):
                    k = part(kh_s, m, c)
                    if m % 2 == 0:
                        k = pace(k)
                    for p in ps:
                        if p >= m:
                            if p - m not in xs:
                                xs[p - m] = part(xh_s.at[j], p - m, c)
                            kx = k * xs[p - m]
                            acc[p] = kx + acc[p] if m else kx - tmp_s[p] if c == 2 else kx
                    yield min(p0 + PW_SPLIT - m, PW_SPLIT)
                for p in ps:
                    if c == 0:
                        tmp_s[p] = acc[p]
                    elif c == 1:
                        rr = tmp_s[p]
                        tmp_s[NB + p] = rr - acc[p]
                        tmp_s[p] = rr + acc[p]
                    else:
                        y = (tmp_s[NB + p], acc[p])
                        z = y if prev is None else (y[0] - prev[1], y[1] + prev[0])
                        yh_s[j, p, pl.ds(r0, 8), :] = _pack(*z)
                        prev = y

    qscale = float(DH ** -0.5 * np.log2(np.e))

    def qkv(j, i, every):
        r0, h0 = i * QR, i * (QR // 2)
        if not isinstance(i, int):
            r0, h0 = pl.multiple_of(r0, QR), pl.multiple_of(h0, QR // 2)
        for s in range(3):
            x = jnp.concatenate([_halves(xs_s[t, pl.ds(h0, QR // 2), :]) for t in range(NT)], 1)
            w = jnp.concatenate([_halves(wp_s[j, t, s * (T // 2):(s + 1) * (T // 2), :])
                                 for t in range(NT)], 1)
            acc = _dot_nt(x, w)
            if s == 0:
                q_s[j, pl.ds(r0, QR), :] = acc * qscale
            else:
                (k_s, v_s)[s - 1][j, pl.ds(HALO + r0, QR), :] = acc
            post(acc, every)
            yield QR * 5 // 4

    def window(r0, masked):
        rows = lambda r: pl.ds(r, 8)
        qs = [q_s[t, rows(r0), :] for t in range(NT)]
        ls = []
        for w in range(WIN):
            a = None
            for t in range(NT):
                k = k_s[t, rows(r0 + HALO - DIL * w), :]
                kq = qs[t] * k
                a = kq if a is None else a + kq
            ls.append((a, pltpu.roll(a, 64, 1)))
        yield 1
        ls = [a + b for a, b in ls]
        ls = [(a, pltpu.roll(a, 32, 1)) for a in ls]
        yield 1
        ls = [a + b for a, b in ls]
        if masked:
            row = jax.lax.broadcasted_iota(jnp.int32, (8, T), 0) + r0
            ls = [jnp.where(row >= DIL * w, a, -1e9 * np.log2(np.e)) for w, a in enumerate(ls)]
        mx = _tree(jnp.maximum, ls)
        es = [jnp.exp2(a - mx) for a in ls]
        yield 1
        inv = gate_s[rows(r0), :] * pl.reciprocal(_tree(jnp.add, es), full_range=False)
        outs = []
        for t in range(NT):
            a = None
            for w in range(WIN):
                v = v_s[t, rows(r0 + HALO - DIL * w), :]
                pv = es[w] * (pace(v) if w == 0 and t == 0 else v)
                a = pv if a is None else a + pv
            outs.append(a)
        for t in range(NT):
            at_s[t, rows(r0), :] = outs[t] * inv
        yield 1

    def attend(r0, n, first=False):
        gens = [window(r0 + 8 * c, first and 8 * c < DIL * WIN) for c in range(n)]
        for step in range(n + 3):
            for c in range(step, step - 4, -1):
                if 0 <= c < n:
                    next(gens[c])
            yield 1

    def stage(i):
        r0 = _aligned(i * RB, RB)
        for t in range(NT):
            cur_s[t] = _pack(*[at_s[t, pl.ds(r0 + e, RB // 2, stride=2), :] for e in range(2)])

    def out_copy(i):
        r0 = _aligned(i * RB, RB)
        return pltpu.make_async_copy(o_ref.at[pl.ds(r0, RB), :], o_hbm.at[pl.ds(r0, RB), :], osem)

    def tail_copy(ct):
        part = (slice(S - RB, S), slice(ct * T, (ct + 1) * T))
        return pltpu.make_async_copy(o_ref.at[part], o_hbm.at[part], osem)

    def mix(i):
        r0 = _aligned(i * RB, RB)
        for ct in range(NT):
            for h in range(RB // T):
                y = _dot(jnp.concatenate([_halves(g_ref[b]) for b in range(2)], 1),
                         _halves(yh_s[ct, i * (RB // T) + h]))
                y_s[ct, h * T:(h + 1) * T, :] = (1.0 - gate_s[pl.ds(r0 + h * T, T), :]) * y
                post(y, T)
                yield 64
        for ct in range(NT):
            yield from project(r0, ct)

    def project(r0, ct):
        a = _dot(jnp.concatenate([_halves(cur_s[t]) for t in range(NT)], 1), _halves(wop_s[ct]))
        acc = a + y_s[ct]
        o_ref[pl.ds(r0, RB), ct * T:(ct + 1) * T] = acc.astype(BF16)
        if isinstance(r0, int):
            tail_copy(ct).start()
        post(acc, MIX_EVERY)
        yield RB * 5 // 4

    def gen_stream(i0, n):
        units = [u for i in range(2 * n)
                 for u in (gen(4 * i0 + 2 * i, False), gen(4 * i0 + 2 * i + 1, False), gen(2 * i0 + i, True))]
        return _chain(units), len(units) * GEN_STEPS, 0.0, 1.0

    def qkvs(j, i0, n, every):
        return _chain([qkv(j, i0 + u, every) for u in range(n)])

    def kmats(g0, n):
        for u in range(n):
            kmat(g0 + u)
            yield 60

    def overlap(*streams, gap=1, lag=0):
        always[:] = [zero_s[...] == 0.0, gap, 0, lag]
        _interleave(*streams)
        tokens.clear()
        always.clear()

    nq, cq = S // QR, QR * 15 // 4

    for t in range(NT):
        k_s[t, 0:HALO, :] = jnp.zeros((HALO, T), F32)
        v_s[t, 0:HALO, :] = jnp.zeros((HALO, T), F32)
    zero_s[...] = jnp.zeros((8, T), F32)
    for c in cp_vec + cp_ssm[0]:
        c.wait()
    for i, ref in enumerate((ldt_in, dsk_in, gw_in)):
        vec_s[i] = ref[...].astype(F32).reshape(1, D)
    cp_x(2).start()
    prep_wide(0, prep(0))
    cp_fx.wait()

    def first(i):
        for when, cs in enumerate(([cp_w[0]], [cp_x(3), cp_w[1]], [cp_w[2]])):
            @pl.when(i == when)
            def _():
                for c in cs:
                    c.start()

        @pl.when(i % 2 == 0)
        def _():
            cp_x(i // 2).wait()
        xs = (_chain([x_block(2 * i + u) for u in range(2)]), 128 * NT, X_LEAD, X_LAST)
        overlap(xs, gen_stream(i, 1), gap=X_GAP, lag=X_LAG)
    _loop(4, first)
    late = ([], [cp_fk] + cp_ssm[1], cp_ssm[2] + cp_out)
    for s, (g0, g1, m0, m1) in enumerate(((0, 8, 8, 12), (8, 16, 12, NB), (16, 32, NB, NB))):
        for c in late[s]:
            c.start()
        cp_w[s].wait()
        if s < 2:
            cp_x(2 + s).wait()
        mxu = _chain([kmats(g0, g1 - g0)] + [x_block(m) for m in range(m0, m1)])
        overlap((mxu, 60 * (g1 - g0) + 64 * NT * (m1 - m0), LEAD, LAST),
                (w_qkv(s), 2 * NT * NT, 0.0, 1.0), lag=PW_LAG)
    overlap((qkv(0, 0, QR), cq, 0.0, 1.0), (taps(0), 5, 0.0, 1.0))
    for c in [cp_fk] + cp_ssm[1]:
        c.wait()

    def pws(j, i0, n):
        return (_chain([pointwise(j, i0 + u) for u in range(n)]), n * PW_STEPS, 0.0, 1.0)

    def tile(j):
        @pl.when(j == 1)
        def _():
            for c in cp_ssm[2]:
                c.wait()
        overlap((spectrum_k(), 1024, 0.0, 1.0))
        prep_wide(j + 1, prep(j + 1))
        overlap((qkvs(j, 1, 4, GEN_EVERY), 4 * cq, LEAD2, LAST2), gen_stream(0, 4),
                gap=GEN_GAP, lag=GEN_LAG)
        mxu = _chain([kmats(0, 32), qkvs(j, 5, NA, PW_EVERY)])
        overlap((mxu, 1920 + NA * cq, LEAD, LAST), pws(j, 0, PA), gap=PW_GAP, lag=PW_LAG)
        n = nq - 4 - NA
        mxu = _chain([qkvs(j, NA + 5, n - 1, PW_EVERY), qkv(j + 1, 0, PW_EVERY)])
        st = [(mxu, n * cq, LEAD, LAST), pws(j, PA, 16 - PA)]
        overlap(*st, (taps(j + 1), 5, 0.0, TAP_LAST), gap=PW_GAP, lag=PW_LAG)
    _loop(NT - 1, tile)

    j = NT - 1
    for c in cp_out:
        c.wait()
    mxu = _chain([spectrum_k(), qkvs(j, 1, HEAD - 1, 64)])
    st = [(mxu, 1024 + cq * (HEAD - 1), LEAD, LAST), (attend(0, FIRST, True), FIRST + 3, 0.0, 1.0)]
    overlap(*st, (w_out(), NT, 0.0, 1.0), lag=PW_LAG)
    n = (nq - HEAD) // NL

    def last_conv(i):
        r0 = pl.multiple_of(8 * (FIRST + i * EARLY), 16)
        st = [(qkvs(j, HEAD + n * i, n, PW_EVERY), cq * n, LEAD, LAST), pws(j, 16 // NL * i, 16 // NL)]
        overlap(*st, (attend(r0, EARLY), EARLY + 3, 0.0, 1.0), gap=PW_GAP, lag=PW_LAG)
    _loop(NL, last_conv)

    done, nr = FIRST + NL * EARLY, S // RB
    n_mixed = (S // 8 - done) // PER_ROW
    assert n * NL + HEAD == nq and done + n_mixed * PER_ROW == S // 8 and n_mixed == nr - 1
    assert 8 * FIRST <= QR and FIRST % 2 == EARLY % 2 == PER_ROW % 2 == 0
    assert all(8 * (FIRST + EARLY * (i + 1)) <= (HEAD + n * i) * QR for i in range(NL))
    assert all(8 * (done + PER_ROW * i) >= (i + 1) * RB for i in range(n_mixed + 1))
    stage(0)

    def rows(i):
        r0 = pl.multiple_of(8 * (done + PER_ROW * i), 16)
        overlap((mix(i), NT * RB * 7 // 4, MIX_LEAD, MIX_LAST),
                (attend(r0, PER_ROW), 100 * PER_ROW + 300, 0.0, 1.0), lag=1)
        stage(i + 1)
        out_copy(i).start()
    _loop(nr - 1, rows)
    overlap((mix(nr - 1), 1, 0.0, 1.0))
    for i in range(nr - 1):
        out_copy(i).wait()
    for ct in range(NT):
        tail_copy(ct).wait()


@jax.jit
def pallas_gated_mix__sliding_local_dilated__ssm_conv_s4__prompt_kernel(
    A_x: jax.Array,
    A_wqkv: jax.Array,
    A_wo: jax.Array,
    B_u: jax.Array,
    B_A_re: jax.Array,
    B_A_im: jax.Array,
    B_B_re: jax.Array,
    B_B_im: jax.Array,
    B_C_re: jax.Array,
    B_C_im: jax.Array,
    B_log_dt: jax.Array,
    B_Dskip: jax.Array,
    gate_w: jax.Array,
):
    del B_u
    fx, g, fk = _constants()
    vm = pltpu.VMEM
    hbm = pl.BlockSpec(memory_space=pl.ANY)
    out = pl.pallas_call(
        _kernel,
        out_shape=jax.ShapeDtypeStruct((S, D), BF16),
        in_specs=[hbm] * 15,
        out_specs=hbm,
        scratch_shapes=[
            vm((S, D), BF16), vm((D, 3 * D), BF16), vm((D, D), BF16), vm((6, N, D), BF16),
            vm(fx.shape, U32), vm(g.shape, U32), vm(fk.shape, U32), vm((S, D), BF16),
            vm((NT, S // 2, T), U32), vm((S, T), F32),
            vm((3, NT, D // 2 + 32, T), U32), vm((NT, NT, 3 * T // 2, T), U32), vm((NT, D // 2, T), U32),
            vm((4, N, T), F32), vm((3, NU * 4 * GS + 64, T), U32), vm((3, NV * 4 * GS + 64, T), U32),
            vm((2, T, T), F32), vm((32 * KS + 96, T), F32), vm((max(_SLOT) + 1, T // 2, T), U32),
            vm((NB, SPEC, T), F32), vm((NT, NB, SPEC, T), F32), vm((NT, NB, T, T), U32),
            vm((2 * NB, 8, T), F32),
            vm((NT, S, T), F32), vm((NT, S + HALO, T), F32), vm((NT, S + HALO, T), F32),
            vm((NT, S + 32, T), F32), vm((NT, RB // 2, T), U32), vm((NT, RB, T), F32), vm((8, T), F32),
            vm((3, 1, D), F32), vm((D,), BF16), vm((D,), BF16), vm((D,), BF16),
            pltpu.SemaphoreType.DMA((N_COPIES,)), pltpu.SemaphoreType.DMA((4,)),
             pltpu.SemaphoreType.DMA(()),
        ],
        compiler_params=pltpu.CompilerParams(vmem_limit_bytes=100 * 1024 * 1024),
    )(A_x.reshape(S, D), A_wqkv, A_wo, B_A_re.T, B_A_im.T, B_B_re.T, B_B_im.T, B_C_re.T, B_C_im.T,
      B_log_dt, B_Dskip, gate_w, fx, g, fk)
    return out.reshape(1, S, D)
```
